```python
import jax
import jax.numpy as jnp

def _softmax(x, axis=-1):
    return jax.nn.softmax(x, axis=axis)
def _gelu(x):
    return jax.nn.gelu(x, approximate=True)
def _silu(x):
    return jax.nn.silu(x)
def _sigmoid(x):
    return jax.nn.sigmoid(x)
def _layernorm(x, axis=-1, eps=1e-5):
    m = jnp.mean(x, axis=axis, keepdims=True)
    v = jnp.var(x, axis=axis, keepdims=True)
    return (x - m) / jnp.sqrt(v + eps)
def _scatter_add(tgt, idx, src, axis=0):
    return tgt.at[idx].add(src)
def _segment_sum(src, seg, n):
    return jax.ops.segment_sum(src, seg, n)
class _Rng:
    def __init__(self, key):
        self._k = key
    def _next(self):
        self._k, sub = jax.random.split(self._k)
        return sub
    def normal(self, shape):
        return jax.random.normal(self._next(), shape, dtype=jnp.bfloat16)
    def randint(self, lo, hi, shape):
        return jax.random.randint(self._next(), shape, lo, hi, dtype=jnp.int32)
    def uniform(self, shape, lo=0.0, hi=1.0):
        return jax.random.uniform(self._next(), shape, jnp.bfloat16, lo, hi)
    def permutation(self, n):
        return jax.random.permutation(self._next(), n)


kernel_name = 'concat_heads__spectral_gfnet__compressed_kv_cla__prompt'

def setup_inputs():
    _rng = _Rng(jax.random.key(int.from_bytes(__import__("os").urandom(4), "little")))
    _w = (lambda a: (lambda t: t.astype(jnp.bfloat16) if jnp.issubdtype(t.dtype, jnp.floating) else t)(jnp.asarray(a)))
    def _A_setup():
        B, S, D = 1, 2048, 448
        Df = D // 2 + 1
        return {
            "x": _w((lambda *s: _rng.normal(s) * 0.05)(B, S, D)),
            "w_r": _w((lambda *s: _rng.normal(s) * 0.05)(S, Df) * 0.02),
            "w_i": _w((lambda *s: _rng.normal(s) * 0.05)(S, Df) * 0.02),
        }
    _A_in = _A_setup()

    def _B_setup():
        B, H, Sq, Sk, D, M = 1, 16, 2048, 2048, 256, 448
        Dc = 4 * D
        return {
            "x": _w((lambda *s: _rng.normal(s) * 0.05)(B, Sq, M)),
            "c_kv": _w((lambda *s: _rng.normal(s) * 0.05)(B, Sk, Dc)),
            "w_q": _w((lambda *s: _rng.normal(s) * 0.05)(M, H, D) * (M ** -0.5)),
            "w_uk": _w((lambda *s: _rng.normal(s) * 0.05)(Dc, H, D) * (Dc ** -0.5)),
            "w_uv": _w((lambda *s: _rng.normal(s) * 0.05)(Dc, H, D) * (Dc ** -0.5)),
            "w_o": _w((lambda *s: _rng.normal(s) * 0.05)(H, D, M) * ((H * D) ** -0.5)),
        }
    _B_in = _B_setup()

    return {
        "A_x": _A_in["x"],
        "A_w_r": _A_in["w_r"],
        "A_w_i": _A_in["w_i"],
        "B_x": _B_in["x"],
        "B_c_kv": _B_in["c_kv"],
        "B_w_q": _B_in["w_q"],
        "B_w_uk": _B_in["w_uk"],
        "B_w_uv": _B_in["w_uv"],
        "B_w_o": _B_in["w_o"],
    }

def reference(A_x, A_w_r, A_w_i, B_x, B_c_kv, B_w_q, B_w_uk, B_w_uv, B_w_o):
    def _A_ref(x, w_r, w_i):
        B, S, D = x.shape
        X = (lambda x, axes=(-2,-1): jnp.fft.rfft2(x.astype(jnp.float32), axes=axes))(x, axes=(-2, -1))
        W = w_r + 1j * w_i
        X = X * W
        y = (lambda x, s, axes=(-2,-1): jnp.fft.irfft2(x, s=s, axes=axes).astype(jnp.bfloat16))(X, (S, D), axes=(-2, -1))
        return y

    def _B_ref(x, c_kv, w_q, w_uk, w_uv, w_o):
        B, Sq, M = x.shape[0], x.shape[1], x.shape[2]
        Sk = c_kv.shape[1]
        H, D = w_q.shape[1], w_q.shape[2]
        q = jnp.einsum("bqm,mhd->bhqd", x, w_q)
        k = jnp.einsum("bkc,chd->bhkd", c_kv, w_uk)
        v = jnp.einsum("bkc,chd->bhkd", c_kv, w_uv)
        scores = jnp.einsum("bhqd,bhkd->bhqk", q, k) * (D ** -0.5)
        off = Sk - Sq
        qi = jnp.arange(Sq)[:, None]
        kj = jnp.arange(Sk)[None, :]
        cmask = kj <= (qi + off)
        scores = jnp.where(cmask[None, None], scores, -1e9)
        p = _softmax(scores, axis=-1)
        ctx = jnp.einsum("bhqk,bhkd->bhqd", p, v)
        return jnp.einsum("bhqd,hdm->bqm", ctx, w_o)

    a = _A_ref(A_x, A_w_r, A_w_i)
    b = _B_ref(B_x, B_c_kv, B_w_q, B_w_uk, B_w_uv, B_w_o)
    return jnp.concatenate([a, b], axis=-1)
```

```python
import numpy as np
import jax
import jax.numpy as jnp
from jax import lax
import jax.experimental.pallas as pl
import jax.experimental.pallas.tpu as pltpu

S = 2048
DA = 448
DF = DA // 2 + 1
FP = 240
H = 16
D = 256
C = 1024
N1 = 16
N2 = 128
TQ = 256
LOG2E = 1.4426950408889634
MASK_VAL = -1e9 * LOG2E
BF = jnp.bfloat16
F32 = jnp.float32
NT = (((1,), (1,)), ((), ()))


def _tables():
    f = np.arange(FP)[:, None].astype(np.float64)
    d = np.arange(DA)[None, :].astype(np.float64)
    valid = (np.arange(FP) < DF)[:, None]
    ang = 2 * np.pi * ((f * d) % DA) / DA
    g1 = np.concatenate([np.cos(ang) * valid, -np.sin(ang) * valid], axis=0)
    k2 = np.arange(N2)[:, None]
    s2 = np.arange(N2)[None, :]
    rt = np.zeros((N1, 2 * N2, 2 * N2))
    for k1 in range(N1):
        a = 2 * np.pi * ((s2 * (k1 + N1 * k2)) % S) / S
        mr, mi = np.cos(a), -np.sin(a)
        rt[k1] = np.block([[mr, -mi], [mi, mr]])
    rtt = np.transpose(rt, (0, 2, 1))
    f2 = np.arange(256)[:, None].astype(np.float64)
    cf = np.where((f2 == 0) | (f2 == DA // 2), 1.0, 2.0) * (f2 < DF) / (S * DA)
    ang2 = 2 * np.pi * ((f2 * d) % DA) / DA
    g2 = np.concatenate([np.cos(ang2) * cf, -np.sin(ang2) * cf], axis=0)
    perm = np.zeros((128, 128))
    for k1 in range(N1):
        for j in range(8):
            perm[8 * k1 + j, k1 + 16 * j] = 1.0
    cast = lambda a: jnp.asarray(a.astype(np.float32), dtype=BF)
    return cast(g1), cast(rt), cast(rtt), cast(g2), cast(perm)


def _fft4(xs, sign):
    (ar, ai), (br, bi), (cr, ci), (dr, di) = xs
    s0r, s0i = ar + cr, ai + ci
    s1r, s1i = ar - cr, ai - ci
    s2r, s2i = br + dr, bi + di
    s3r, s3i = br - dr, bi - di
    y0 = (s0r + s2r, s0i + s2i)
    y2 = (s0r - s2r, s0i - s2i)
    if sign < 0:
        y1 = (s1r + s3i, s1i - s3r)
        y3 = (s1r - s3i, s1i + s3r)
    else:
        y1 = (s1r - s3i, s1i + s3r)
        y3 = (s1r + s3i, s1i - s3r)
    return [y0, y1, y2, y3]


def _twiddle(z, e, sign):
    zr, zi = z
    e = e % 16
    if e == 0:
        return z
    if (e * sign) % 16 == 12:
        return (zi, -zr)
    if (e * sign) % 16 == 4:
        return (-zi, zr)
    c = float(np.cos(2 * np.pi * e / 16))
    s = float(sign * np.sin(2 * np.pi * e / 16))
    if abs(abs(c) - abs(s)) < 1e-12:
        r = abs(c)
        u = zr - zi if (c > 0) == (s > 0) else zr + zi
        v = zi + zr if (c > 0) == (s > 0) else zi - zr
        return (u * c, v * c)
    return (zr * c - zi * s, zi * c + zr * s)


def _fft16(xs, sign):
    t = [None] * 16
    for b in range(4):
        col = _fft4([xs[4 * a + b] for a in range(4)], sign)
        for c in range(4):
            t[4 * c + b] = _twiddle(col[c], b * c, sign)
    out = [None] * 16
    for c in range(4):
        col = _fft4([t[4 * c + b] for b in range(4)], sign)
        for e in range(4):
            out[c + 4 * e] = col[e]
    return out


def _kernel(axt_hbm, wrt_hbm, wit_hbm, bxt_hbm, ckv_hbm, wq_hbm, wuk_hbm, wuv_hbm, wot_hbm,
            g1_hbm, rt_hbm, rtt_hbm, g2_hbm, perm_hbm,
            out_hbm,
            axt, wrt, wit, bxt, ckv, wq_w, wuk_w, wuv_w, wot, g1, rt, rtt, g2, perm,
            x1_s, a_s, wr_s, wi_s, b_s, y1_s,
            qt_s, k_s, vt_s, acc_s, o_s,
            sem, wsem, osem):
    h = pl.program_id(0)

    simple = [(axt_hbm, axt), (g1_hbm, g1), (wrt_hbm, wrt), (wit_hbm, wit), (perm_hbm, perm),
              (rt_hbm, rt), (rtt_hbm, rtt), (g2_hbm, g2), (bxt_hbm, bxt), (ckv_hbm, ckv),
              (wot_hbm, wot)]
    cps = [pltpu.make_async_copy(s, d, sem.at[i]) for i, (s, d) in enumerate(simple)]
    (cp_axt, cp_g1, cp_wrt, cp_wit, cp_perm, cp_rt, cp_rtt, cp_g2, cp_bxt, cp_ckv, cp_wot) = cps

    def wcopies(widx, w_hbm, w_buf, g):
        src = w_hbm.bitcast(jnp.uint32)
        return [pltpu.make_async_copy(
            src.at[:, p, pl.ds(4 * g, 4), pl.ds(128 * t, 128)],
            w_buf.at[g, t, :, pl.ds(4 * p, 4), :],
            wsem.at[widx, g, 2 * t + p]) for t in range(2) for p in range(2)]

    wlist = [(0, wq_hbm, wq_w), (1, wuk_hbm, wuk_w), (2, wuv_hbm, wuv_w)]

    @pl.when(h == 0)
    def _prologue():
        for cp in (cp_axt, cp_g1, cp_wrt, cp_wit, cp_perm, cp_rt, cp_rtt, cp_g2, cp_bxt):
            cp.start()
        for cp in wcopies(*wlist[0], 0):
            cp.start()
        cp_ckv.start()
        for cp in wcopies(*wlist[1], 0) + wcopies(*wlist[2], 0):
            cp.start()
        cp_wot.start()
        for w in wlist:
            for cp in wcopies(*w, 1):
                cp.start()

        acc_s[...] = jnp.zeros_like(acc_s)

        cp_axt.wait()
        cp_g1.wait()
        x1_s[...] = jnp.dot(g1[...], axt[...], preferred_element_type=F32)
        for r in range(0, FP, 8):
            xs = [(x1_s[r:r + 8, 128 * s1:128 * (s1 + 1)],
                   x1_s[FP + r:FP + r + 8, 128 * s1:128 * (s1 + 1)]) for s1 in range(N1)]
            ys = _fft16(xs, -1)
            for k1 in range(N1):
                a_s[k1, r:r + 8, 0:128] = ys[k1][0]
                a_s[k1, r:r + 8, 128:256] = ys[k1][1]
        a_s[:, FP:256, :] = jnp.zeros((N1, 256 - FP, 256), F32)

        cp_wrt.wait()
        cp_wit.wait()
        cp_perm.wait()
        zpad = jnp.zeros((128, 256 - DF), F32)
        for a in range(N1):
            for (src, dst) in ((wrt, wr_s), (wit, wi_s)):
                t = lax.dot_general(perm[...], src[:, 128 * a:128 * (a + 1)], NT,
                                    preferred_element_type=F32)
                t = jnp.concatenate([t, zpad], axis=1)
                for k1 in range(N1):
                    dst[k1, 8 * a:8 * (a + 1), :] = t[8 * k1:8 * (k1 + 1), :]

        cp_rt.wait()
        cp_rtt.wait()
        for k1 in range(N1):
            z = lax.dot_general(rt[k1], a_s[k1].astype(BF), NT, preferred_element_type=F32)
            zr, zi = z[0:128], z[128:256]
            wr, wi = wr_s[k1], wi_s[k1]
            y = jnp.concatenate([zr * wr - zi * wi, zr * wi + zi * wr], axis=0).astype(BF)
            b_s[k1] = jnp.dot(rtt[k1], y, preferred_element_type=F32)

        for g in range(N2 // 8):
            for t in range(2):
                xs = [(b_s[k1, 8 * g:8 * g + 8, 128 * t:128 * (t + 1)],
                       b_s[k1, 128 + 8 * g:128 + 8 * g + 8, 128 * t:128 * (t + 1)]) for k1 in range(N1)]
                ys = _fft16(xs, +1)
                for s1 in range(N1):
                    r0 = 128 * s1 + 8 * g
                    y1_s[r0:r0 + 8, 128 * t:128 * (t + 1)] = ys[s1][0]
                    y1_s[r0:r0 + 8, 256 + 128 * t:256 + 128 * (t + 1)] = ys[s1][1]
        cp_g2.wait()
        ya = jnp.dot(y1_s[...].astype(BF), g2[...], preferred_element_type=F32)
        o_s[:, 0:DA] = ya.astype(BF)

        cp_bxt.wait()
        for cp in wcopies(*wlist[0], 0):
            cp.wait()
        cp_ckv.wait()
        for cp in wcopies(*wlist[1], 0) + wcopies(*wlist[2], 0):
            cp.wait()
        cp_wot.wait()

    @pl.when(h == 8)
    def _():
        for w in wlist:
            for cp in wcopies(*w, 1):
                cp.wait()

    g = lax.shift_right_logical(h, 3)
    j = lax.shift_right_logical(h, 1) & 3
    sh = ((h & 1) * 16).astype(jnp.uint32)

    def head_weight(w_buf, rows):
        halves = []
        for t in range(2):
            w2 = w_buf.at[g, t].reshape(rows * 4, 128)
            a = w2[pl.ds(j, rows, stride=4), :]
            halves.append(pltpu.bitcast((a >> sh) << 16, F32))
        return jnp.concatenate(halves, axis=1)

    wq_t = head_weight(wq_w, DA).T.astype(BF)
    qt = jnp.dot(wq_t, bxt[...], preferred_element_type=F32) * (D ** -0.5 * LOG2E)
    qt_s[...] = qt.astype(BF)
    wk = head_weight(wuk_w, C).astype(BF)
    k_s[...] = jnp.dot(ckv[...], wk, preferred_element_type=F32).astype(BF)
    wv_t = head_weight(wuv_w, C).T.astype(BF)
    vt_s[...] = lax.dot_general(wv_t, ckv[...], NT, preferred_element_type=F32).astype(BF)

    wo_t = wot[h]
    key = lax.broadcasted_iota(jnp.int32, (TQ, TQ), 0)
    qry = lax.broadcasted_iota(jnp.int32, (TQ, TQ), 1)
    causal = key <= qry
    for i in range(S // TQ):
        L = (i + 1) * TQ
        st = jnp.dot(k_s[0:L, :], qt_s[:, i * TQ:(i + 1) * TQ], preferred_element_type=F32)
        sd = jnp.where(causal, st[L - TQ:, :], MASK_VAL)
        st = jnp.concatenate([st[:L - TQ, :], sd], axis=0) if L > TQ else sd
        m = jnp.max(st, axis=0, keepdims=True)
        p = jnp.exp2(st - m)
        l = jnp.sum(p, axis=0, keepdims=True)
        ot = jnp.dot(vt_s[:, 0:L], p.astype(BF), preferred_element_type=F32)
        ot = (ot * (1.0 / l)).astype(BF)
        acc_s[64:512, i * TQ:(i + 1) * TQ] += jnp.dot(wo_t, ot, preferred_element_type=F32)

    @pl.when(h == H - 1)
    def _epilogue():
        lane = lax.broadcasted_iota(jnp.int32, (TQ, 128), 1)
        outs = []
        for i in range(S // TQ):
            rows = slice(i * TQ, (i + 1) * TQ)
            bt = acc_s[:, rows].T.astype(BF)
            first = jnp.where(lane < 64, o_s[rows, 384:512], bt[:, 0:128])
            o_s[rows, 384:512] = first
            o_s[rows, 512:896] = bt[:, 128:512]
            cp = pltpu.make_async_copy(o_s.at[rows], out_hbm.at[rows], osem.at[i])
            cp.start()
            outs.append(cp)
        for cp in outs:
            cp.wait()


@jax.jit
def pallas_concat_heads__spectral_gfnet__compressed_kv_cla__prompt_kernel(
    A_x, A_w_r, A_w_i, B_x, B_c_kv, B_w_q, B_w_uk, B_w_uv, B_w_o,
):
    g1, rt, rtt, g2, perm = _tables()
    axt = jnp.swapaxes(A_x, 1, 2).reshape(DA, S)
    bxt = jnp.swapaxes(B_x, 1, 2).reshape(DA, S)
    wrt = A_w_r.T
    wit = A_w_i.T
    ckv = B_c_kv.reshape(S, C)
    wq = B_w_q.reshape(DA // 2, 2, H, D)
    wuk = B_w_uk.reshape(C // 2, 2, H, D)
    wuv = B_w_uv.reshape(C // 2, 2, H, D)
    wot = jnp.swapaxes(B_w_o, 1, 2)

    any_spec = pl.BlockSpec(memory_space=pl.ANY)
    V = pltpu.VMEM
    out = pl.pallas_call(
        _kernel,
        grid=(H,),
        in_specs=[any_spec] * 14,
        out_specs=any_spec,
        out_shape=jax.ShapeDtypeStruct((S, 2 * DA), BF),
        scratch_shapes=[
            V((DA, S), BF), V((DF, S), BF), V((DF, S), BF), V((DA, S), BF), V((S, C), BF),
            V((2, 2, DA // 2, 8, 128), jnp.uint32),
            V((2, 2, C // 2, 8, 128), jnp.uint32),
            V((2, 2, C // 2, 8, 128), jnp.uint32),
            V((H, DA, D), BF),
            V((2 * FP, DA), BF), V((N1, 256, 256), BF), V((N1, 256, 256), BF), V((512, DA), BF),
            V((128, 128), BF),
            V((2 * FP, S), F32), V((N1, 256, 256), F32), V((N1, 128, 256), F32),
            V((N1, 128, 256), F32), V((N1, 256, 256), F32), V((S, 512), F32),
            V((D, S), BF), V((S, D), BF), V((D, S), BF), V((512, S), F32), V((S, 2 * DA), BF),
            pltpu.SemaphoreType.DMA((11,)),
            pltpu.SemaphoreType.DMA((3, 2, 4)),
            pltpu.SemaphoreType.DMA((S // TQ,)),
        ],
        compiler_params=pltpu.CompilerParams(
            dimension_semantics=("arbitrary",),
            vmem_limit_bytes=120 * 2**20),
    )(axt, wrt, wit, bxt, ckv, wq, wuk, wuv, wot, g1, rt, rtt, g2, perm)
    return out.reshape(1, S, 2 * DA)
```

```python
import numpy as np
import jax
import jax.numpy as jnp
from jax import lax
import jax.experimental.pallas as pl
import jax.experimental.pallas.tpu as pltpu

S = 2048
DA = 448
DF = DA // 2 + 1
FP = 240
H = 16
D = 256
C = 1024
N1 = 16
N2 = 128
TQ = 256
PIN = 1
LOG2E = 1.4426950408889634
MASK_VAL = -1e9 * LOG2E
BF = jnp.bfloat16
F32 = jnp.float32
NT = (((1,), (1,)), ((), ()))


def _tables():
    f = np.arange(FP)[:, None].astype(np.float64)
    d = np.arange(DA)[None, :].astype(np.float64)
    valid = (np.arange(FP) < DF)[:, None]
    ang = 2 * np.pi * ((f * d) % DA) / DA
    g1 = np.concatenate([np.cos(ang) * valid, -np.sin(ang) * valid], axis=0)
    k2 = np.arange(N2)[:, None]
    s2 = np.arange(N2)[None, :]
    rt = np.zeros((N1, 2 * N2, 2 * N2))
    for k1 in range(N1):
        a = 2 * np.pi * ((s2 * (k1 + N1 * k2)) % S) / S
        mr, mi = np.cos(a), -np.sin(a)
        rt[k1] = np.block([[mr, -mi], [mi, mr]])
    rtt = np.transpose(rt, (0, 2, 1))
    f2 = np.arange(256)[:, None].astype(np.float64)
    cf = np.where((f2 == 0) | (f2 == DA // 2), 1.0, 2.0) * (f2 < DF) / (S * DA)
    ang2 = 2 * np.pi * ((f2 * d) % DA) / DA
    g2 = np.concatenate([np.cos(ang2) * cf, -np.sin(ang2) * cf], axis=0)
    perm = np.zeros((128, 128))
    for k1 in range(N1):
        for j in range(8):
            perm[8 * k1 + j, k1 + 16 * j] = 1.0
    cast = lambda a: jnp.asarray(a.astype(np.float32), dtype=BF)
    return cast(g1), cast(rt), cast(rtt), cast(g2), cast(perm)


def _fft4(xs, sign):
    (ar, ai), (br, bi), (cr, ci), (dr, di) = xs
    s0r, s0i = ar + cr, ai + ci
    s1r, s1i = ar - cr, ai - ci
    s2r, s2i = br + dr, bi + di
    s3r, s3i = br - dr, bi - di
    y0 = (s0r + s2r, s0i + s2i)
    y2 = (s0r - s2r, s0i - s2i)
    if sign < 0:
        y1 = (s1r + s3i, s1i - s3r)
        y3 = (s1r - s3i, s1i + s3r)
    else:
        y1 = (s1r - s3i, s1i + s3r)
        y3 = (s1r + s3i, s1i - s3r)
    return [y0, y1, y2, y3]


def _twiddle(z, e, sign):
    zr, zi = z
    e = e % 16
    if e == 0:
        return z
    if (e * sign) % 16 == 12:
        return (zi, -zr)
    if (e * sign) % 16 == 4:
        return (-zi, zr)
    c = float(np.cos(2 * np.pi * e / 16))
    s = float(sign * np.sin(2 * np.pi * e / 16))
    if abs(abs(c) - abs(s)) < 1e-12:
        r = abs(c)
        u = zr - zi if (c > 0) == (s > 0) else zr + zi
        v = zi + zr if (c > 0) == (s > 0) else zi - zr
        return (u * c, v * c)
    return (zr * c - zi * s, zi * c + zr * s)


def _fft16(xs, sign):
    t = [None] * 16
    for b in range(4):
        col = _fft4([xs[4 * a + b] for a in range(4)], sign)
        for c in range(4):
            t[4 * c + b] = _twiddle(col[c], b * c, sign)
    out = [None] * 16
    for c in range(4):
        col = _fft4([t[4 * c + b] for b in range(4)], sign)
        for e in range(4):
            out[c + 4 * e] = col[e]
    return out


def _kernel(axt_hbm, wrt_hbm, wit_hbm, bxt_hbm, ckv_hbm, wq_hbm, wuk_hbm, wuv_hbm, wot_hbm,
            g1_hbm, rt_hbm, rtt_hbm, g2_hbm, perm_hbm,
            out_hbm,
            axt, wrt, wit, bxt, ckv, wq_w, wuk_w, wuv_w, wot, g1, rt, rtt, g2, perm,
            x1_s, a_s, wr_s, wi_s, b_s, y1_s,
            wqt_s, wk_s, wvt_s, qt_s, k_s, vt_s, acc_s, o_s, s0_s, s1_s, p0_s, p1_s,
            sem, wsem, osem):
    h = pl.program_id(0)

    simple = [(axt_hbm, axt), (g1_hbm, g1), (wrt_hbm, wrt), (wit_hbm, wit), (perm_hbm, perm),
              (rt_hbm, rt), (rtt_hbm, rtt), (g2_hbm, g2), (bxt_hbm, bxt), (ckv_hbm, ckv),
              (wot_hbm.at[0:1], wot.at[0:1]), (wot_hbm.at[1:H], wot.at[1:H])]
    cps = [pltpu.make_async_copy(s, d, sem.at[i]) for i, (s, d) in enumerate(simple)]
    (cp_axt, cp_g1, cp_wrt, cp_wit, cp_perm, cp_rt, cp_rtt, cp_g2, cp_bxt, cp_ckv,
     cp_wot0, cp_wot1) = cps

    def wcopies(widx, w_hbm, w_buf, stage):
        src = w_hbm.bitcast(jnp.uint32)
        g, j0, n = ((0, 0, 1), (0, 1, 3), (1, 0, 4))[stage]
        return [pltpu.make_async_copy(
            src.at[:, p, pl.ds(4 * g + j0, n), pl.ds(128 * t, 128)],
            w_buf.at[g, t, :, pl.ds(4 * p + j0, n), :],
            wsem.at[widx, stage, 2 * t + p]) for t in range(2) for p in range(2)]

    wlist = [(0, wq_hbm, wq_w), (1, wuk_hbm, wuk_w), (2, wuv_hbm, wuv_w)]

    def head_weight(w_buf, rows, hh):
        g = lax.shift_right_logical(hh, 3)
        j = lax.shift_right_logical(hh, 1) & 3
        sh = ((hh & 1) * 16).astype(jnp.uint32)
        halves = []
        for t in range(2):
            w2 = w_buf.at[g, t].reshape(rows * 4, 128)
            a = w2[pl.ds(j, rows, stride=4), :]
            halves.append(pltpu.bitcast((a >> sh) << 16, F32))
        return jnp.concatenate(halves, axis=1)

    def prep_weights(hh):
        wqt_s[...] = head_weight(wq_w, DA, hh).T.astype(BF)
        wk_s[...] = head_weight(wuk_w, C, hh).astype(BF)
        wvt_s[...] = head_weight(wuv_w, C, hh).T.astype(BF)

    @pl.when(h == 0)
    def _prologue():
        for cp in (cp_axt, cp_g1, cp_wrt, cp_wit, cp_perm, cp_rt, cp_rtt, cp_g2, cp_bxt):
            cp.start()
        for cp in wcopies(*wlist[0], 0):
            cp.start()
        cp_ckv.start()
        for cp in wcopies(*wlist[1], 0) + wcopies(*wlist[2], 0):
            cp.start()
        cp_wot0.start()

        acc_s[...] = jnp.zeros_like(acc_s)

        cp_axt.wait()
        cp_g1.wait()

        def step1(c, carry):
            cols = pl.ds(pl.multiple_of(c * 512, 512), 512)
            x1_s[:, cols] = jnp.dot(g1[...], axt[:, cols], preferred_element_type=F32)
            return carry
        lax.fori_loop(0, S // 512, step1, 0)

        for r in range(0, FP, 8):
            xs = [(x1_s[r:r + 8, 128 * s1:128 * (s1 + 1)],
                   x1_s[FP + r:FP + r + 8, 128 * s1:128 * (s1 + 1)]) for s1 in range(N1)]
            ys = _fft16(xs, -1)
            for k1 in range(N1):
                a_s[k1, r:r + 8, 0:128] = ys[k1][0]
                a_s[k1, r:r + 8, 128:256] = ys[k1][1]
        a_s[:, FP:256, :] = jnp.zeros((N1, 256 - FP, 256), F32)

        cp_wrt.wait()
        cp_wit.wait()
        cp_perm.wait()
        zpad = jnp.zeros((128, 256 - DF), F32)
        for a in range(N1):
            for (src, dst) in ((wrt, wr_s), (wit, wi_s)):
                t = lax.dot_general(perm[...], src[:, 128 * a:128 * (a + 1)], NT,
                                    preferred_element_type=F32)
                t = jnp.concatenate([t, zpad], axis=1)
                for k1 in range(N1):
                    dst[k1, 8 * a:8 * (a + 1), :] = t[8 * k1:8 * (k1 + 1), :]

        cp_rt.wait()
        cp_rtt.wait()
        for k1 in range(N1):
            z = lax.dot_general(rt[k1], a_s[k1].astype(BF), NT, preferred_element_type=F32)
            zr, zi = z[0:128], z[128:256]
            wr, wi = wr_s[k1], wi_s[k1]
            y = jnp.concatenate([zr * wr - zi * wi, zr * wi + zi * wr], axis=0).astype(BF)
            b_s[k1] = jnp.dot(rtt[k1], y, preferred_element_type=F32)

        for g in range(N2 // 8):
            for t in range(2):
                xs = [(b_s[k1, 8 * g:8 * g + 8, 128 * t:128 * (t + 1)],
                       b_s[k1, 128 + 8 * g:128 + 8 * g + 8, 128 * t:128 * (t + 1)]) for k1 in range(N1)]
                ys = _fft16(xs, +1)
                for s1 in range(N1):
                    r0 = 128 * s1 + 8 * g
                    y1_s[r0:r0 + 8, 128 * t:128 * (t + 1)] = ys[s1][0]
                    y1_s[r0:r0 + 8, 256 + 128 * t:256 + 128 * (t + 1)] = ys[s1][1]
        cp_g2.wait()

        def step7(c, carry):
            rows = pl.ds(pl.multiple_of(c * 512, 512), 512)
            ya = jnp.dot(y1_s[rows, :].astype(BF), g2[...], preferred_element_type=F32)
            o_s[rows, 0:DA] = ya.astype(BF)
            return carry
        lax.fori_loop(0, S // 512, step7, 0)

        cp_bxt.wait()
        cp_ckv.wait()
        for w in wlist:
            for cp in wcopies(*w, 0):
                cp.wait()
        cp_wot0.wait()
        for stage in (1, 2):
            for w in wlist:
                for cp in wcopies(*w, stage):
                    cp.start()
            if stage == 1:
                cp_wot1.start()
        prep_weights(h)

    @pl.when(h == 1)
    def _():
        for w in wlist:
            for cp in wcopies(*w, 1):
                cp.wait()
        cp_wot1.wait()

    @pl.when(h == 6)
    def _():
        for w in wlist:
            for cp in wcopies(*w, 2):
                cp.wait()

    NB = S // TQ
    key = lax.broadcasted_iota(jnp.int32, (TQ, TQ), 0)
    qry = lax.broadcasted_iota(jnp.int32, (TQ, TQ), 1)
    causal = key <= qry

    def proj(i):
        cs = slice(i * TQ, (i + 1) * TQ)
        qt = jnp.dot(wqt_s[...], bxt[:, cs], preferred_element_type=F32) * (D ** -0.5 * LOG2E)
        qt_s[:, cs] = qt.astype(BF)
        k_s[cs, :] = jnp.dot(ckv[cs, :], wk_s[...], preferred_element_type=F32).astype(BF)
        vt_s[:, cs] = lax.dot_general(wvt_s[...], ckv[cs, :], NT,
                                      preferred_element_type=F32).astype(BF)

    def colreduce(x, op, nacc=4):
        accs = [x[8 * a:8 * a + 8] for a in range(nacc)]
        for r in range(8 * nacc, x.shape[0], 8 * nacc):
            for a in range(nacc):
                accs[a] = op(accs[a], x[r + 8 * a:r + 8 * a + 8])
        while len(accs) > 1:
            accs = [op(accs[2 * a], accs[2 * a + 1]) for a in range(len(accs) // 2)]
        return accs[0]

    def qk_softmax(i):
        L = (i + 1) * TQ
        st = jnp.dot(k_s[0:L, :], qt_s[:, i * TQ:(i + 1) * TQ], preferred_element_type=F32)
        sd = jnp.where(causal, st[L - TQ:, :], MASK_VAL)
        st = jnp.concatenate([st[:L - TQ, :], sd], axis=0) if L > TQ else sd
        m = jnp.max(colreduce(st, jnp.maximum), axis=0, keepdims=True)
        p = jnp.exp2(st - m)
        l = jnp.sum(colreduce(p, jnp.add), axis=0, keepdims=True)
        return p.astype(BF), l

    def pv(i, p):
        L = (i + 1) * TQ
        return jnp.dot(vt_s[:, 0:L], p, preferred_element_type=F32)

    def outproj(i, ot, l, l_next):
        inv = 1.0 / l
        if PIN and l_next is not None:
            inv = jnp.minimum(inv, l_next)
        ot = (ot * inv).astype(BF)
        acc_s[64:512, i * TQ:(i + 1) * TQ] += jnp.dot(wot[h], ot, preferred_element_type=F32)

    ps, ls, ots = {}, {}, {}
    for t in range(-2, NB + 1):
        if 0 <= t + 2 < NB:
            proj(t + 2)
            if t + 2 == NB - 1:
                prep_weights(jnp.minimum(h + 1, H - 1))
        if 0 <= t + 1 < NB:
            ps[t + 1], ls[t + 1] = qk_softmax(t + 1)
        if 0 <= t < NB:
            ots[t] = pv(t, ps.pop(t))
        if 0 <= t - 1 < NB:
            outproj(t - 1, ots.pop(t - 1), ls[t - 1], ls.get(t - 1 + PIN))

    @pl.when(h == H - 1)
    def _epilogue():
        OB = 256
        lane = lax.broadcasted_iota(jnp.int32, (OB, 128), 1)
        outs = []
        for i in range(S // OB):
            rows = slice(i * OB, (i + 1) * OB)
            bt = acc_s[:, rows].T.astype(BF)
            first = jnp.where(lane < 64, o_s[rows, 384:512], bt[:, 0:128])
            o_s[rows, 384:512] = first
            o_s[rows, 512:896] = bt[:, 128:512]
            cp = pltpu.make_async_copy(o_s.at[rows], out_hbm.at[rows], osem.at[i])
            cp.start()
            outs.append(cp)
        for cp in outs:
            cp.wait()


@jax.jit
def pallas_concat_heads__spectral_gfnet__compressed_kv_cla__prompt_kernel(
    A_x, A_w_r, A_w_i, B_x, B_c_kv, B_w_q, B_w_uk, B_w_uv, B_w_o,
):
    g1, rt, rtt, g2, perm = _tables()
    axt = jnp.swapaxes(A_x, 1, 2).reshape(DA, S)
    bxt = jnp.swapaxes(B_x, 1, 2).reshape(DA, S)
    wrt = A_w_r.T
    wit = A_w_i.T
    ckv = B_c_kv.reshape(S, C)
    wq = B_w_q.reshape(DA // 2, 2, H, D)
    wuk = B_w_uk.reshape(C // 2, 2, H, D)
    wuv = B_w_uv.reshape(C // 2, 2, H, D)
    wot = jnp.swapaxes(B_w_o, 1, 2)

    any_spec = pl.BlockSpec(memory_space=pl.ANY)
    V = pltpu.VMEM
    out = pl.pallas_call(
        _kernel,
        grid=(H,),
        in_specs=[any_spec] * 14,
        out_specs=any_spec,
        out_shape=jax.ShapeDtypeStruct((S, 2 * DA), BF),
        scratch_shapes=[
            V((DA, S), BF), V((DF, S), BF), V((DF, S), BF), V((DA, S), BF), V((S, C), BF),
            V((2, 2, DA // 2, 8, 128), jnp.uint32),
            V((2, 2, C // 2, 8, 128), jnp.uint32),
            V((2, 2, C // 2, 8, 128), jnp.uint32),
            V((H, DA, D), BF),
            V((2 * FP, DA), BF), V((N1, 256, 256), BF), V((N1, 256, 256), BF), V((512, DA), BF),
            V((128, 128), BF),
            V((2 * FP, S), F32), V((N1, 256, 256), F32), V((N1, 128, 256), F32),
            V((N1, 128, 256), F32), V((N1, 256, 256), F32), V((S, 512), F32),
            V((D, DA), BF), V((C, D), BF), V((D, C), BF),
            V((D, S), BF), V((S, D), BF), V((D, S), BF), V((512, S), F32), V((S, 2 * DA), BF),
            V((S, TQ), F32), V((S, TQ), F32), V((S, TQ), BF), V((S, TQ), BF),
            pltpu.SemaphoreType.DMA((12,)),
            pltpu.SemaphoreType.DMA((3, 3, 4)),
            pltpu.SemaphoreType.DMA((8,)),
        ],
        compiler_params=pltpu.CompilerParams(
            dimension_semantics=("arbitrary",),
            vmem_limit_bytes=120 * 2**20),
    )(axt, wrt, wit, bxt, ckv, wq, wuk, wuv, wot, g1, rt, rtt, g2, perm)
    return out.reshape(1, S, 2 * DA)
```

```python
import numpy as np
import jax
import jax.numpy as jnp
from jax import lax
import jax.experimental.pallas as pl
import jax.experimental.pallas.tpu as pltpu

S = 2048
DA = 448
DF = DA // 2 + 1
FP = 240
H = 16
D = 256
C = 1024
N1 = 16
N2 = 128
TQ = 256
PIN = 0
LOG2E = 1.4426950408889634
MASK_VAL = -1e9 * LOG2E
BF = jnp.bfloat16
F32 = jnp.float32
NT = (((1,), (1,)), ((), ()))


def _tables():
    f = np.arange(FP)[:, None].astype(np.float64)
    d = np.arange(DA)[None, :].astype(np.float64)
    valid = (np.arange(FP) < DF)[:, None]
    ang = 2 * np.pi * ((f * d) % DA) / DA
    g1 = np.concatenate([np.cos(ang) * valid, -np.sin(ang) * valid], axis=0)
    k2 = np.arange(N2)[:, None]
    s2 = np.arange(N2)[None, :]
    rt = np.zeros((N1, 2 * N2, 2 * N2))
    for k1 in range(N1):
        a = 2 * np.pi * ((s2 * (k1 + N1 * k2)) % S) / S
        mr, mi = np.cos(a), -np.sin(a)
        rt[k1] = np.block([[mr, -mi], [mi, mr]])
    rtt = np.transpose(rt, (0, 2, 1))
    f2 = np.arange(256)[:, None].astype(np.float64)
    cf = np.where((f2 == 0) | (f2 == DA // 2), 1.0, 2.0) * (f2 < DF) / (S * DA)
    ang2 = 2 * np.pi * ((f2 * d) % DA) / DA
    g2 = np.concatenate([np.cos(ang2) * cf, -np.sin(ang2) * cf], axis=0)
    perm = np.zeros((128, 128))
    for k1 in range(N1):
        for j in range(8):
            perm[8 * k1 + j, k1 + 16 * j] = 1.0
    cast = lambda a: jnp.asarray(a.astype(np.float32), dtype=BF)
    return cast(g1), cast(rt), cast(rtt), cast(g2), cast(perm)


def _fft4(xs, sign):
    (ar, ai), (br, bi), (cr, ci), (dr, di) = xs
    s0r, s0i = ar + cr, ai + ci
    s1r, s1i = ar - cr, ai - ci
    s2r, s2i = br + dr, bi + di
    s3r, s3i = br - dr, bi - di
    y0 = (s0r + s2r, s0i + s2i)
    y2 = (s0r - s2r, s0i - s2i)
    if sign < 0:
        y1 = (s1r + s3i, s1i - s3r)
        y3 = (s1r - s3i, s1i + s3r)
    else:
        y1 = (s1r - s3i, s1i + s3r)
        y3 = (s1r + s3i, s1i - s3r)
    return [y0, y1, y2, y3]


def _twiddle(z, e, sign):
    zr, zi = z
    e = e % 16
    if e == 0:
        return z
    if (e * sign) % 16 == 12:
        return (zi, -zr)
    if (e * sign) % 16 == 4:
        return (-zi, zr)
    c = float(np.cos(2 * np.pi * e / 16))
    s = float(sign * np.sin(2 * np.pi * e / 16))
    if abs(abs(c) - abs(s)) < 1e-12:
        r = abs(c)
        u = zr - zi if (c > 0) == (s > 0) else zr + zi
        v = zi + zr if (c > 0) == (s > 0) else zi - zr
        return (u * c, v * c)
    return (zr * c - zi * s, zi * c + zr * s)


def _fft16(xs, sign):
    t = [None] * 16
    for b in range(4):
        col = _fft4([xs[4 * a + b] for a in range(4)], sign)
        for c in range(4):
            t[4 * c + b] = _twiddle(col[c], b * c, sign)
    out = [None] * 16
    for c in range(4):
        col = _fft4([t[4 * c + b] for b in range(4)], sign)
        for e in range(4):
            out[c + 4 * e] = col[e]
    return out


def _kernel(axt_hbm, wrt_hbm, wit_hbm, bxt_hbm, ckv_hbm, wq_hbm, wuk_hbm, wuv_hbm, wot_hbm,
            g1_hbm, rt_hbm, rtt_hbm, g2_hbm, perm_hbm,
            out_hbm,
            axt, wrt, wit, bxt, ckv, wq_w, wuk_w, wuv_w, wot, g1, rt, rtt, g2, perm,
            x1_s, a_s, wr_s, wi_s, b_s, y1_s,
            wqt_s, wk_s, wvt_s, qt_s, k_s, vt_s, acc_s, o_s, s0_s, s1_s, p0_s, p1_s,
            sem, wsem, osem):
    h = pl.program_id(0)

    simple = [(axt_hbm, axt), (g1_hbm, g1), (wrt_hbm, wrt), (wit_hbm, wit), (perm_hbm, perm),
              (rt_hbm, rt), (rtt_hbm, rtt), (g2_hbm, g2), (bxt_hbm, bxt), (ckv_hbm, ckv),
              (wot_hbm.at[0:1], wot.at[0:1]), (wot_hbm.at[1:H], wot.at[1:H])]
    cps = [pltpu.make_async_copy(s, d, sem.at[i]) for i, (s, d) in enumerate(simple)]
    (cp_axt, cp_g1, cp_wrt, cp_wit, cp_perm, cp_rt, cp_rtt, cp_g2, cp_bxt, cp_ckv,
     cp_wot0, cp_wot1) = cps

    def wcopies(widx, w_hbm, w_buf, stage):
        src = w_hbm.bitcast(jnp.uint32)
        g, j0, n = ((0, 0, 1), (0, 1, 3), (1, 0, 4))[stage]
        return [pltpu.make_async_copy(
            src.at[:, p, pl.ds(4 * g + j0, n), pl.ds(128 * t, 128)],
            w_buf.at[g, t, :, pl.ds(4 * p + j0, n), :],
            wsem.at[widx, stage, 2 * t + p]) for t in range(2) for p in range(2)]

    wlist = [(0, wq_hbm, wq_w), (1, wuk_hbm, wuk_w), (2, wuv_hbm, wuv_w)]

    def head_weight(w_buf, rows, hh):
        g = lax.shift_right_logical(hh, 3)
        j = lax.shift_right_logical(hh, 1) & 3
        sh = ((hh & 1) * 16).astype(jnp.uint32)
        halves = []
        for t in range(2):
            w2 = w_buf.at[g, t].reshape(rows * 4, 128)
            a = w2[pl.ds(j, rows, stride=4), :]
            halves.append(pltpu.bitcast((a >> sh) << 16, F32))
        return jnp.concatenate(halves, axis=1)

    def prep_weights(hh):
        wqt_s[...] = head_weight(wq_w, DA, hh).T.astype(BF)
        wk_s[...] = head_weight(wuk_w, C, hh).astype(BF)
        wvt_s[...] = head_weight(wuv_w, C, hh).T.astype(BF)

    @pl.when(h == 0)
    def _prologue():
        for cp in (cp_axt, cp_g1, cp_wrt, cp_wit, cp_perm, cp_rt, cp_rtt, cp_g2, cp_bxt):
            cp.start()
        for cp in wcopies(*wlist[0], 0):
            cp.start()
        cp_ckv.start()
        for cp in wcopies(*wlist[1], 0) + wcopies(*wlist[2], 0):
            cp.start()
        cp_wot0.start()

        acc_s[...] = jnp.zeros_like(acc_s)

        cp_axt.wait()
        cp_g1.wait()

        def step1(c, carry):
            cols = pl.ds(pl.multiple_of(c * 512, 512), 512)
            x1_s[:, cols] = jnp.dot(g1[...], axt[:, cols], preferred_element_type=F32)
            return carry
        lax.fori_loop(0, S // 512, step1, 0)

        for r in range(0, FP, 8):
            xs = [(x1_s[r:r + 8, 128 * s1:128 * (s1 + 1)],
                   x1_s[FP + r:FP + r + 8, 128 * s1:128 * (s1 + 1)]) for s1 in range(N1)]
            ys = _fft16(xs, -1)
            for k1 in range(N1):
                a_s[k1, r:r + 8, 0:128] = ys[k1][0]
                a_s[k1, r:r + 8, 128:256] = ys[k1][1]
        a_s[:, FP:256, :] = jnp.zeros((N1, 256 - FP, 256), F32)

        cp_wrt.wait()
        cp_wit.wait()
        cp_perm.wait()
        zpad = jnp.zeros((128, 256 - DF), F32)
        for a in range(N1):
            for (src, dst) in ((wrt, wr_s), (wit, wi_s)):
                t = lax.dot_general(perm[...], src[:, 128 * a:128 * (a + 1)], NT,
                                    preferred_element_type=F32)
                t = jnp.concatenate([t, zpad], axis=1)
                for k1 in range(N1):
                    dst[k1, 8 * a:8 * (a + 1), :] = t[8 * k1:8 * (k1 + 1), :]

        cp_rt.wait()
        cp_rtt.wait()
        for k1 in range(N1):
            z = lax.dot_general(rt[k1], a_s[k1].astype(BF), NT, preferred_element_type=F32)
            zr, zi = z[0:128], z[128:256]
            wr, wi = wr_s[k1], wi_s[k1]
            y = jnp.concatenate([zr * wr - zi * wi, zr * wi + zi * wr], axis=0).astype(BF)
            b_s[k1] = jnp.dot(rtt[k1], y, preferred_element_type=F32)

        for g in range(N2 // 8):
            for t in range(2):
                xs = [(b_s[k1, 8 * g:8 * g + 8, 128 * t:128 * (t + 1)],
                       b_s[k1, 128 + 8 * g:128 + 8 * g + 8, 128 * t:128 * (t + 1)]) for k1 in range(N1)]
                ys = _fft16(xs, +1)
                for s1 in range(N1):
                    r0 = 128 * s1 + 8 * g
                    y1_s[r0:r0 + 8, 128 * t:128 * (t + 1)] = ys[s1][0]
                    y1_s[r0:r0 + 8, 256 + 128 * t:256 + 128 * (t + 1)] = ys[s1][1]
        cp_g2.wait()

        def step7(c, carry):
            rows = pl.ds(pl.multiple_of(c * 512, 512), 512)
            ya = jnp.dot(y1_s[rows, :].astype(BF), g2[...], preferred_element_type=F32)
            o_s[rows, 0:DA] = ya.astype(BF)
            return carry
        lax.fori_loop(0, S // 512, step7, 0)

        cp_bxt.wait()
        cp_ckv.wait()
        for w in wlist:
            for cp in wcopies(*w, 0):
                cp.wait()
        cp_wot0.wait()
        for stage in (1, 2):
            for w in wlist:
                for cp in wcopies(*w, stage):
                    cp.start()
            if stage == 1:
                cp_wot1.start()
        prep_weights(h)

    @pl.when(h == 1)
    def _():
        for w in wlist:
            for cp in wcopies(*w, 1):
                cp.wait()
        cp_wot1.wait()

    @pl.when(h == 6)
    def _():
        for w in wlist:
            for cp in wcopies(*w, 2):
                cp.wait()

    NB = S // TQ
    key = lax.broadcasted_iota(jnp.int32, (TQ, TQ), 0)
    qry = lax.broadcasted_iota(jnp.int32, (TQ, TQ), 1)
    causal = key <= qry

    def proj(i):
        cs = slice(i * TQ, (i + 1) * TQ)
        qt = jnp.dot(wqt_s[...], bxt[:, cs], preferred_element_type=F32) * (D ** -0.5 * LOG2E)
        qt_s[:, cs] = qt.astype(BF)
        k_s[cs, :] = jnp.dot(ckv[cs, :], wk_s[...], preferred_element_type=F32).astype(BF)
        vt_s[:, cs] = lax.dot_general(wvt_s[...], ckv[cs, :], NT,
                                      preferred_element_type=F32).astype(BF)

    def colreduce(x, op, nacc=2):
        accs = [x[8 * a:8 * a + 8] for a in range(nacc)]
        for r in range(8 * nacc, x.shape[0], 8 * nacc):
            for a in range(nacc):
                accs[a] = op(accs[a], x[r + 8 * a:r + 8 * a + 8])
        while len(accs) > 1:
            accs = [op(accs[2 * a], accs[2 * a + 1]) for a in range(len(accs) // 2)]
        return accs[0]

    def qk_softmax(i):
        L = (i + 1) * TQ
        st = jnp.dot(k_s[0:L, :], qt_s[:, i * TQ:(i + 1) * TQ], preferred_element_type=F32)
        sd = jnp.where(causal, st[L - TQ:, :], MASK_VAL)
        st = jnp.concatenate([st[:L - TQ, :], sd], axis=0) if L > TQ else sd
        m = jnp.max(colreduce(st, jnp.maximum), axis=0, keepdims=True)
        p = jnp.exp2(st - m)
        l = jnp.sum(colreduce(p, jnp.add), axis=0, keepdims=True)
        return p.astype(BF), l

    def pv(i, p):
        L = (i + 1) * TQ
        return jnp.dot(vt_s[:, 0:L], p, preferred_element_type=F32)

    def outproj(i, ot, l, l_next):
        inv = 1.0 / l
        if PIN and l_next is not None:
            inv = jnp.minimum(inv, l_next)
        ot = (ot * inv).astype(BF)
        acc_s[64:512, i * TQ:(i + 1) * TQ] += jnp.dot(wot[h], ot, preferred_element_type=F32)

    ps, ls, ots = {}, {}, {}
    proj(0)
    for t in range(-1, NB + 1):
        if 0 <= t + 1 < NB:
            ps[t + 1], ls[t + 1] = qk_softmax(t + 1)
        if 0 <= t + 2 < NB:
            proj(t + 2)
            if t + 2 == NB - 1:
                prep_weights(jnp.minimum(h + 1, H - 1))
        if 0 <= t < NB:
            ots[t] = pv(t, ps.pop(t))
        if 0 <= t - 1 < NB:
            outproj(t - 1, ots.pop(t - 1), ls[t - 1], ls.get(t - 1 + PIN))

    @pl.when(h == H - 1)
    def _epilogue():
        OB = 256
        lane = lax.broadcasted_iota(jnp.int32, (OB, 128), 1)
        outs = []
        for i in range(S // OB):
            rows = slice(i * OB, (i + 1) * OB)
            bt = acc_s[:, rows].T.astype(BF)
            first = jnp.where(lane < 64, o_s[rows, 384:512], bt[:, 0:128])
            o_s[rows, 384:512] = first
            o_s[rows, 512:896] = bt[:, 128:512]
            cp = pltpu.make_async_copy(o_s.at[rows], out_hbm.at[rows], osem.at[i])
            cp.start()
            outs.append(cp)
        for cp in outs:
            cp.wait()


@jax.jit
def pallas_concat_heads__spectral_gfnet__compressed_kv_cla__prompt_kernel(
    A_x, A_w_r, A_w_i, B_x, B_c_kv, B_w_q, B_w_uk, B_w_uv, B_w_o,
):
    g1, rt, rtt, g2, perm = _tables()
    axt = jnp.swapaxes(A_x, 1, 2).reshape(DA, S)
    bxt = jnp.swapaxes(B_x, 1, 2).reshape(DA, S)
    wrt = A_w_r.T
    wit = A_w_i.T
    ckv = B_c_kv.reshape(S, C)
    wq = B_w_q.reshape(DA // 2, 2, H, D)
    wuk = B_w_uk.reshape(C // 2, 2, H, D)
    wuv = B_w_uv.reshape(C // 2, 2, H, D)
    wot = jnp.swapaxes(B_w_o, 1, 2)

    any_spec = pl.BlockSpec(memory_space=pl.ANY)
    V = pltpu.VMEM
    out = pl.pallas_call(
        _kernel,
        grid=(H,),
        in_specs=[any_spec] * 14,
        out_specs=any_spec,
        out_shape=jax.ShapeDtypeStruct((S, 2 * DA), BF),
        scratch_shapes=[
            V((DA, S), BF), V((DF, S), BF), V((DF, S), BF), V((DA, S), BF), V((S, C), BF),
            V((2, 2, DA // 2, 8, 128), jnp.uint32),
            V((2, 2, C // 2, 8, 128), jnp.uint32),
            V((2, 2, C // 2, 8, 128), jnp.uint32),
            V((H, DA, D), BF),
            V((2 * FP, DA), BF), V((N1, 256, 256), BF), V((N1, 256, 256), BF), V((512, DA), BF),
            V((128, 128), BF),
            V((2 * FP, S), F32), V((N1, 256, 256), F32), V((N1, 128, 256), F32),
            V((N1, 128, 256), F32), V((N1, 256, 256), F32), V((S, 512), F32),
            V((D, DA), BF), V((C, D), BF), V((D, C), BF),
            V((D, S), BF), V((S, D), BF), V((D, S), BF), V((512, S), F32), V((S, 2 * DA), BF),
            V((S, TQ), F32), V((S, TQ), F32), V((S, TQ), BF), V((S, TQ), BF),
            pltpu.SemaphoreType.DMA((12,)),
            pltpu.SemaphoreType.DMA((3, 3, 4)),
            pltpu.SemaphoreType.DMA((8,)),
        ],
        compiler_params=pltpu.CompilerParams(
            dimension_semantics=("arbitrary",),
            vmem_limit_bytes=120 * 2**20),
    )(axt, wrt, wit, bxt, ckv, wq, wuk, wuv, wot, g1, rt, rtt, g2, perm)
    return out.reshape(1, S, 2 * DA)
```

```python
import numpy as np
import jax
import jax.numpy as jnp
from jax import lax
import jax.experimental.pallas as pl
import jax.experimental.pallas.tpu as pltpu

S = 2048
DA = 448
DF = DA // 2 + 1
FP = 240
H = 16
D = 256
C = 1024
N1 = 16
N2 = 128
TQ = 256
HT = 128
PREP_FENCE = 1
LOG2E = 1.4426950408889634
MASK_VAL = -1e9 * LOG2E
BF = jnp.bfloat16
F32 = jnp.float32
NT = (((1,), (1,)), ((), ()))


def _tables():
    f = np.arange(FP)[:, None].astype(np.float64)
    d = np.arange(DA)[None, :].astype(np.float64)
    valid = (np.arange(FP) < DF)[:, None]
    ang = 2 * np.pi * ((f * d) % DA) / DA
    g1 = np.concatenate([np.cos(ang) * valid, -np.sin(ang) * valid], axis=0)
    k2 = np.arange(N2)[:, None]
    s2 = np.arange(N2)[None, :]
    rt = np.zeros((N1, 2 * N2, 2 * N2))
    for k1 in range(N1):
        a = 2 * np.pi * ((s2 * (k1 + N1 * k2)) % S) / S
        mr, mi = np.cos(a), -np.sin(a)
        rt[k1] = np.block([[mr, -mi], [mi, mr]])
    rtt = np.transpose(rt, (0, 2, 1))
    f2 = np.arange(256)[:, None].astype(np.float64)
    cf = np.where((f2 == 0) | (f2 == DA // 2), 1.0, 2.0) * (f2 < DF) / (S * DA)
    ang2 = 2 * np.pi * ((f2 * d) % DA) / DA
    g2 = np.concatenate([np.cos(ang2) * cf, -np.sin(ang2) * cf], axis=0)
    perm = np.zeros((128, 128))
    for k1 in range(N1):
        for j in range(8):
            perm[8 * k1 + j, k1 + 16 * j] = 1.0
    cast = lambda a: jnp.asarray(a.astype(np.float32), dtype=BF)
    return cast(g1), cast(rt), cast(rtt), cast(g2), cast(perm)


def _fft4(xs, sign):
    (ar, ai), (br, bi), (cr, ci), (dr, di) = xs
    s0r, s0i = ar + cr, ai + ci
    s1r, s1i = ar - cr, ai - ci
    s2r, s2i = br + dr, bi + di
    s3r, s3i = br - dr, bi - di
    y0 = (s0r + s2r, s0i + s2i)
    y2 = (s0r - s2r, s0i - s2i)
    if sign < 0:
        y1 = (s1r + s3i, s1i - s3r)
        y3 = (s1r - s3i, s1i + s3r)
    else:
        y1 = (s1r - s3i, s1i + s3r)
        y3 = (s1r + s3i, s1i - s3r)
    return [y0, y1, y2, y3]


def _twiddle(z, e, sign):
    zr, zi = z
    e = e % 16
    if e == 0:
        return z
    if (e * sign) % 16 == 12:
        return (zi, -zr)
    if (e * sign) % 16 == 4:
        return (-zi, zr)
    c = float(np.cos(2 * np.pi * e / 16))
    s = float(sign * np.sin(2 * np.pi * e / 16))
    if abs(abs(c) - abs(s)) < 1e-12:
        r = abs(c)
        u = zr - zi if (c > 0) == (s > 0) else zr + zi
        v = zi + zr if (c > 0) == (s > 0) else zi - zr
        return (u * c, v * c)
    return (zr * c - zi * s, zi * c + zr * s)


def _fft16(xs, sign):
    t = [None] * 16
    for b in range(4):
        col = _fft4([xs[4 * a + b] for a in range(4)], sign)
        for c in range(4):
            t[4 * c + b] = _twiddle(col[c], b * c, sign)
    out = [None] * 16
    for c in range(4):
        col = _fft4([t[4 * c + b] for b in range(4)], sign)
        for e in range(4):
            out[c + 4 * e] = col[e]
    return out


def _kernel(axt_hbm, wrt_hbm, wit_hbm, bxt_hbm, ckv_hbm, wq_hbm, wuk_hbm, wuv_hbm, wot_hbm,
            g1_hbm, rt_hbm, rtt_hbm, g2_hbm, perm_hbm,
            out_hbm,
            axt, wrt, wit, bxt, ckv, wq_w, wuk_w, wuv_w, wot, g1, rt, rtt, g2, perm,
            x1_s, a_s, wr_s, wi_s, b_s, y1_s,
            wqt_s, wk_s, wvt_s, qt_s, k_s, vt_s, acc_s, o_s, p0_s, inv0_s, ot7_s,
            sem, wsem, osem):
    h = pl.program_id(0)

    simple = [(axt_hbm, axt), (g1_hbm, g1), (wrt_hbm, wrt), (wit_hbm, wit), (perm_hbm, perm),
              (rt_hbm, rt), (rtt_hbm, rtt), (g2_hbm, g2), (bxt_hbm, bxt), (ckv_hbm, ckv),
              (wot_hbm.at[0:1], wot.at[0:1]), (wot_hbm.at[1:H], wot.at[1:H])]
    cps = [pltpu.make_async_copy(s, d, sem.at[i]) for i, (s, d) in enumerate(simple)]
    (cp_axt, cp_g1, cp_wrt, cp_wit, cp_perm, cp_rt, cp_rtt, cp_g2, cp_bxt, cp_ckv,
     cp_wot0, cp_wot1) = cps

    def wcopies(widx, w_hbm, w_buf, stage):
        src = w_hbm.bitcast(jnp.uint32)
        g, j0, n = ((0, 0, 1), (0, 1, 3), (1, 0, 4))[stage]
        return [pltpu.make_async_copy(
            src.at[:, p, pl.ds(4 * g + j0, n), pl.ds(128 * t, 128)],
            w_buf.at[g, t, :, pl.ds(4 * p + j0, n), :],
            wsem.at[widx, stage, 2 * t + p]) for t in range(2) for p in range(2)]

    wlist = [(0, wq_hbm, wq_w), (1, wuk_hbm, wuk_w), (2, wuv_hbm, wuv_w)]

    def head_weight(w_buf, rows, hh):
        g = lax.shift_right_logical(hh, 3)
        j = lax.shift_right_logical(hh, 1) & 3
        sh = ((hh & 1) * 16).astype(jnp.uint32)
        halves = []
        for t in range(2):
            w2 = w_buf.at[g, t].reshape(rows * 4, 128)
            a = w2[pl.ds(j, rows, stride=4), :]
            halves.append(pltpu.bitcast((a >> sh) << 16, F32))
        return jnp.concatenate(halves, axis=1)

    def orall(x):
        w = pltpu.bitcast(x, jnp.uint32)
        acc = None
        for r in range(0, w.shape[0], 8):
            for c in range(0, w.shape[1], 128):
                t = w[r:r + 8, c:min(c + 128, w.shape[1])]
                if t.shape[1] < 128:
                    continue
                acc = t if acc is None else acc | t
        return acc

    def prep_weights(hh):
        a = head_weight(wq_w, DA, hh).T.astype(BF)
        b = head_weight(wuk_w, C, hh).astype(BF)
        c = head_weight(wuv_w, C, hh).T.astype(BF)
        wqt_s[...] = a
        wk_s[...] = b
        wvt_s[...] = c
        deps = [orall(a)]
        if PREP_FENCE >= 2:
            deps.append(orall(b))
        if PREP_FENCE >= 3:
            deps.append(orall(c))
        d = deps[0]
        for e in deps[1:]:
            d = d | e
        return pltpu.bitcast(d, F32)

    NB = S // TQ
    key = lax.broadcasted_iota(jnp.int32, (HT, HT), 0)
    qry = lax.broadcasted_iota(jnp.int32, (HT, HT), 1)
    causal = key <= qry

    def proj_qk(i):
        cs = slice(i * TQ, (i + 1) * TQ)
        qt = jnp.dot(wqt_s[...], bxt[:, cs], preferred_element_type=F32) * (D ** -0.5 * LOG2E)
        qt_s[:, cs] = qt.astype(BF)
        k_s[cs, :] = jnp.dot(ckv[cs, :], wk_s[...], preferred_element_type=F32).astype(BF)

    def proj_v(i):
        cs = slice(i * TQ, (i + 1) * TQ)
        vt_s[:, cs] = lax.dot_general(wvt_s[...], ckv[cs, :], NT,
                                      preferred_element_type=F32).astype(BF)

    def colreduce(x, op, nacc=2):
        accs = [x[8 * a:8 * a + 8] for a in range(nacc)]
        for r in range(8 * nacc, x.shape[0], 8 * nacc):
            for a in range(nacc):
                accs[a] = op(accs[a], x[r + 8 * a:r + 8 * a + 8])
        while len(accs) > 1:
            accs = [op(accs[2 * a], accs[2 * a + 1]) for a in range(len(accs) // 2)]
        return accs[0]

    def fence(x, dep):
        never = (dep - dep) < -1.0
        head = pltpu.bitcast(x[0:16, 0:128], jnp.uint32)
        head = pltpu.bitcast(jnp.where(never, jnp.uint32(0), head), BF)
        top = jnp.concatenate([head, x[0:16, 128:]], axis=1)
        return jnp.concatenate([top, x[16:]], axis=0)

    def softmax_cols(st):
        m = jnp.max(colreduce(st, jnp.maximum), axis=0, keepdims=True)
        p = jnp.exp2(st - m)
        l = jnp.sum(colreduce(p, jnp.add), axis=0, keepdims=True)
        return p.astype(BF), 1.0 / l

    def qk_softmax(i, dep=None):
        L = (i + 1) * TQ
        qt = qt_s[:, i * TQ:(i + 1) * TQ]
        if dep is not None:
            qt = fence(qt, dep)
        sa = jnp.dot(k_s[0:L - HT, :], qt, preferred_element_type=F32)
        sb = jnp.dot(k_s[L - HT:L, :], qt[:, HT:], preferred_element_type=F32)
        left = [jnp.where(causal, sa[L - TQ:, :HT], MASK_VAL)]
        if L > TQ:
            left = [sa[:L - TQ, :HT]] + left
        left = jnp.concatenate(left, axis=0)
        right = jnp.concatenate([sa[:, HT:], jnp.where(causal, sb, MASK_VAL)], axis=0)
        pl_, invl = softmax_cols(left)
        pr, invr = softmax_cols(right)
        pa = jnp.concatenate([pl_, pr[:L - HT]], axis=1)
        return pa, pr[L - HT:], jnp.concatenate([invl, invr], axis=1)

    def pv(i, pa, pb, inv):
        L = (i + 1) * TQ
        oa = jnp.dot(vt_s[:, 0:L - HT], pa, preferred_element_type=F32)
        ob = jnp.dot(vt_s[:, L - HT:L], pb, preferred_element_type=F32)
        ot = jnp.concatenate([oa[:, :HT], oa[:, HT:] + ob], axis=1)
        return (ot * inv).astype(BF)

    def outproj(i, ot, hh):
        acc_s[64:512, i * TQ:(i + 1) * TQ] += jnp.dot(wot[hh], ot, preferred_element_type=F32)

    def save_first_block():
        pa, pb, inv = qk_softmax(0)
        p0_s[0:HT, :] = pa
        p0_s[HT:TQ, HT:TQ] = pb
        inv0_s[...] = jnp.broadcast_to(inv, (8, TQ))

    @pl.when(h == 0)
    def _prologue():
        for cp in (cp_axt, cp_g1, cp_wrt, cp_wit, cp_perm, cp_rt, cp_rtt, cp_g2, cp_bxt):
            cp.start()
        for cp in wcopies(*wlist[0], 0):
            cp.start()
        cp_ckv.start()
        for cp in wcopies(*wlist[1], 0) + wcopies(*wlist[2], 0):
            cp.start()
        cp_wot0.start()

        acc_s[...] = jnp.zeros_like(acc_s)

        cp_axt.wait()
        cp_g1.wait()

        def step1(c, carry):
            cols = pl.ds(pl.multiple_of(c * 512, 512), 512)
            x1_s[:, cols] = jnp.dot(g1[...], axt[:, cols], preferred_element_type=F32)
            return carry
        lax.fori_loop(0, S // 512, step1, 0)

        for r in range(0, FP, 8):
            xs = [(x1_s[r:r + 8, 128 * s1:128 * (s1 + 1)],
                   x1_s[FP + r:FP + r + 8, 128 * s1:128 * (s1 + 1)]) for s1 in range(N1)]
            ys = _fft16(xs, -1)
            for k1 in range(N1):
                a_s[k1, r:r + 8, 0:128] = ys[k1][0]
                a_s[k1, r:r + 8, 128:256] = ys[k1][1]
        a_s[:, FP:256, :] = jnp.zeros((N1, 256 - FP, 256), F32)

        cp_wrt.wait()
        cp_wit.wait()
        cp_perm.wait()
        zpad = jnp.zeros((128, 256 - DF), F32)
        for a in range(N1):
            for (src, dst) in ((wrt, wr_s), (wit, wi_s)):
                t = lax.dot_general(perm[...], src[:, 128 * a:128 * (a + 1)], NT,
                                    preferred_element_type=F32)
                t = jnp.concatenate([t, zpad], axis=1)
                for k1 in range(N1):
                    dst[k1, 8 * a:8 * (a + 1), :] = t[8 * k1:8 * (k1 + 1), :]

        cp_rt.wait()
        cp_rtt.wait()
        for k1 in range(N1):
            z = lax.dot_general(rt[k1], a_s[k1].astype(BF), NT, preferred_element_type=F32)
            zr, zi = z[0:128], z[128:256]
            wr, wi = wr_s[k1], wi_s[k1]
            y = jnp.concatenate([zr * wr - zi * wi, zr * wi + zi * wr], axis=0).astype(BF)
            b_s[k1] = jnp.dot(rtt[k1], y, preferred_element_type=F32)

        for g in range(N2 // 8):
            for t in range(2):
                xs = [(b_s[k1, 8 * g:8 * g + 8, 128 * t:128 * (t + 1)],
                       b_s[k1, 128 + 8 * g:128 + 8 * g + 8, 128 * t:128 * (t + 1)]) for k1 in range(N1)]
                ys = _fft16(xs, +1)
                for s1 in range(N1):
                    r0 = 128 * s1 + 8 * g
                    y1_s[r0:r0 + 8, 128 * t:128 * (t + 1)] = ys[s1][0]
                    y1_s[r0:r0 + 8, 256 + 128 * t:256 + 128 * (t + 1)] = ys[s1][1]
        cp_g2.wait()

        def step7(c, carry):
            rows = pl.ds(pl.multiple_of(c * 512, 512), 512)
            ya = jnp.dot(y1_s[rows, :].astype(BF), g2[...], preferred_element_type=F32)
            o_s[rows, 0:DA] = ya.astype(BF)
            return carry
        lax.fori_loop(0, S // 512, step7, 0)

        cp_bxt.wait()
        cp_ckv.wait()
        for w in wlist:
            for cp in wcopies(*w, 0):
                cp.wait()
        cp_wot0.wait()
        for stage in (1, 2):
            for w in wlist:
                for cp in wcopies(*w, stage):
                    cp.start()
            if stage == 1:
                cp_wot1.start()
        prep_weights(h)
        proj_qk(0)
        proj_qk(1)
        proj_v(0)
        proj_v(1)
        save_first_block()
        ot7_s[...] = jnp.zeros_like(ot7_s)

    @pl.when(h == 1)
    def _():
        for w in wlist:
            for cp in wcopies(*w, 1):
                cp.wait()
        cp_wot1.wait()

    @pl.when(h == 6)
    def _():
        for w in wlist:
            for cp in wcopies(*w, 2):
                cp.wait()

    ps = {0: (p0_s[0:HT, :], p0_s[HT:TQ, HT:TQ], inv0_s[0:1, :])}
    ots = {-1: ot7_s[...]}
    for t in range(NB):
        if t + 1 < NB:
            ps[t + 1] = qk_softmax(t + 1, dep if (PREP_FENCE and t + 1 == NB - 1) else None)
        if t + 2 < NB:
            proj_qk(t + 2)
            proj_v(t + 2)
            if t + 2 == NB - 1:
                dep = prep_weights(jnp.minimum(h + 1, H - 1))
        else:
            proj_qk(t + 2 - NB)
        if t == NB - 1:
            save_first_block()
        ots[t] = pv(t, *ps.pop(t))
        if t == 0:
            outproj(NB - 1, ots.pop(-1), jnp.maximum(h - 1, 0))
        else:
            outproj(t - 1, ots.pop(t - 1), h)
    proj_v(0)
    proj_v(1)
    ot7_s[...] = ots.pop(NB - 1)

    @pl.when(h == H - 1)
    def _epilogue():
        outproj(NB - 1, ot7_s[...], H - 1)
        OB = 256
        lane = lax.broadcasted_iota(jnp.int32, (OB, 128), 1)
        outs = []
        for i in range(S // OB):
            rows = slice(i * OB, (i + 1) * OB)
            bt = acc_s[:, rows].T.astype(BF)
            first = jnp.where(lane < 64, o_s[rows, 384:512], bt[:, 0:128])
            o_s[rows, 384:512] = first
            o_s[rows, 512:896] = bt[:, 128:512]
            cp = pltpu.make_async_copy(o_s.at[rows], out_hbm.at[rows], osem.at[i])
            cp.start()
            outs.append(cp)
        for cp in outs:
            cp.wait()


@jax.jit
def pallas_concat_heads__spectral_gfnet__compressed_kv_cla__prompt_kernel(
    A_x, A_w_r, A_w_i, B_x, B_c_kv, B_w_q, B_w_uk, B_w_uv, B_w_o,
):
    g1, rt, rtt, g2, perm = _tables()
    axt = jnp.swapaxes(A_x, 1, 2).reshape(DA, S)
    bxt = jnp.swapaxes(B_x, 1, 2).reshape(DA, S)
    wrt = A_w_r.T
    wit = A_w_i.T
    ckv = B_c_kv.reshape(S, C)
    wq = B_w_q.reshape(DA // 2, 2, H, D)
    wuk = B_w_uk.reshape(C // 2, 2, H, D)
    wuv = B_w_uv.reshape(C // 2, 2, H, D)
    wot = jnp.swapaxes(B_w_o, 1, 2)

    any_spec = pl.BlockSpec(memory_space=pl.ANY)
    V = pltpu.VMEM
    out = pl.pallas_call(
        _kernel,
        grid=(H,),
        in_specs=[any_spec] * 14,
        out_specs=any_spec,
        out_shape=jax.ShapeDtypeStruct((S, 2 * DA), BF),
        scratch_shapes=[
            V((DA, S), BF), V((DF, S), BF), V((DF, S), BF), V((DA, S), BF), V((S, C), BF),
            V((2, 2, DA // 2, 8, 128), jnp.uint32),
            V((2, 2, C // 2, 8, 128), jnp.uint32),
            V((2, 2, C // 2, 8, 128), jnp.uint32),
            V((H, DA, D), BF),
            V((2 * FP, DA), BF), V((N1, 256, 256), BF), V((N1, 256, 256), BF), V((512, DA), BF),
            V((128, 128), BF),
            V((2 * FP, S), F32), V((N1, 256, 256), F32), V((N1, 128, 256), F32),
            V((N1, 128, 256), F32), V((N1, 256, 256), F32), V((S, 512), F32),
            V((D, DA), BF), V((C, D), BF), V((D, C), BF),
            V((D, S), BF), V((S, D), BF), V((D, S), BF), V((512, S), F32), V((S, 2 * DA), BF),
            V((TQ, TQ), BF), V((8, TQ), F32), V((D, TQ), BF),
            pltpu.SemaphoreType.DMA((12,)),
            pltpu.SemaphoreType.DMA((3, 3, 4)),
            pltpu.SemaphoreType.DMA((8,)),
        ],
        compiler_params=pltpu.CompilerParams(
            dimension_semantics=("arbitrary",),
            vmem_limit_bytes=120 * 2**20),
    )(axt, wrt, wit, bxt, ckv, wq, wuk, wuv, wot, g1, rt, rtt, g2, perm)
    return out.reshape(1, S, 2 * DA)
```

```python
import numpy as np
import jax
import jax.numpy as jnp
from jax import lax
import jax.experimental.pallas as pl
import jax.experimental.pallas.tpu as pltpu

S = 2048
DA = 448
DF = DA // 2 + 1
FP = 240
H = 16
D = 256
C = 1024
N1 = 16
N2 = 128
TQ = 256
HT = 128
PREP_FENCE = 1
LOG2E = 1.4426950408889634
MASK_VAL = -1e9 * LOG2E
BF = jnp.bfloat16
F32 = jnp.float32
NT = (((1,), (1,)), ((), ()))
TN = (((0,), (0,)), ((), ()))


def _tables():
    f = np.arange(FP)[:, None].astype(np.float64)
    d = np.arange(DA)[None, :].astype(np.float64)
    valid = (np.arange(FP) < DF)[:, None]
    ang = 2 * np.pi * ((f * d) % DA) / DA
    g1 = np.concatenate([np.cos(ang) * valid, -np.sin(ang) * valid], axis=0)
    k2 = np.arange(N2)[:, None]
    s2 = np.arange(N2)[None, :]
    m2 = np.zeros((N1, 2 * N2, N2))
    for k1 in range(N1):
        a = 2 * np.pi * ((s2 * (k1 + N1 * k2)) % S) / S
        m2[k1] = np.concatenate([np.cos(a), -np.sin(a)], axis=0)
    f2 = np.arange(256)[:, None].astype(np.float64)
    cf = np.where((f2 == 0) | (f2 == DA // 2), 1.0, 2.0) * (f2 < DF) / (S * DA)
    ang2 = 2 * np.pi * ((f2 * d) % DA) / DA
    g2 = np.concatenate([np.cos(ang2) * cf, -np.sin(ang2) * cf], axis=0)
    perm = np.zeros((128, 128))
    for k1 in range(N1):
        for j in range(8):
            perm[8 * k1 + j, k1 + 16 * j] = 1.0
    cast = lambda a: jnp.asarray(a.astype(np.float32), dtype=BF)
    return cast(g1), cast(m2), cast(g2), cast(perm)


def _fft4(xs, sign):
    (ar, ai), (br, bi), (cr, ci), (dr, di) = xs
    s0r, s0i = ar + cr, ai + ci
    s1r, s1i = ar - cr, ai - ci
    s2r, s2i = br + dr, bi + di
    s3r, s3i = br - dr, bi - di
    y0 = (s0r + s2r, s0i + s2i)
    y2 = (s0r - s2r, s0i - s2i)
    if sign < 0:
        y1 = (s1r + s3i, s1i - s3r)
        y3 = (s1r - s3i, s1i + s3r)
    else:
        y1 = (s1r - s3i, s1i + s3r)
        y3 = (s1r + s3i, s1i - s3r)
    return [y0, y1, y2, y3]


def _twiddle(z, e, sign):
    zr, zi = z
    e = e % 16
    if e == 0:
        return z
    if (e * sign) % 16 == 12:
        return (zi, -zr)
    if (e * sign) % 16 == 4:
        return (-zi, zr)
    c = float(np.cos(2 * np.pi * e / 16))
    s = float(sign * np.sin(2 * np.pi * e / 16))
    if abs(abs(c) - abs(s)) < 1e-12:
        r = abs(c)
        u = zr - zi if (c > 0) == (s > 0) else zr + zi
        v = zi + zr if (c > 0) == (s > 0) else zi - zr
        return (u * c, v * c)
    return (zr * c - zi * s, zi * c + zr * s)


def _fft16(xs, sign):
    t = [None] * 16
    for b in range(4):
        col = _fft4([xs[4 * a + b] for a in range(4)], sign)
        for c in range(4):
            t[4 * c + b] = _twiddle(col[c], b * c, sign)
    out = [None] * 16
    for c in range(4):
        col = _fft4([t[4 * c + b] for b in range(4)], sign)
        for e in range(4):
            out[c + 4 * e] = col[e]
    return out


def _kernel(axt_hbm, wrt_hbm, wit_hbm, bxt_hbm, ckv_hbm, wq_hbm, wuk_hbm, wuv_hbm, wot_hbm,
            g1_hbm, m2_hbm, g2_hbm, perm_hbm,
            out_hbm,
            axt, wrt, wit, bxt, ckv, wq_w, wuk_w, wuv_w, wot, g1, m2, g2, perm,
            x1_s, a_s, wr_s, wi_s, b_s, y1_s,
            wqt_s, wk_s, wvt_s, qt_s, k_s, vt_s, acc_s, o_s, p0_s, inv0_s, ot7_s,
            sem, wsem, osem):
    h = pl.program_id(0)

    CK0 = 2 * TQ
    simple = [(axt_hbm, axt), (g1_hbm, g1), (wrt_hbm, wrt), (wit_hbm, wit), (perm_hbm, perm),
              (m2_hbm, m2), (g2_hbm, g2), (bxt_hbm, bxt),
              (ckv_hbm.at[0:CK0], ckv.at[0:CK0]), (ckv_hbm.at[CK0:S], ckv.at[CK0:S]),
              (wot_hbm.at[0:1], wot.at[0:1]), (wot_hbm.at[1:H], wot.at[1:H]),
              (o_s.at[:, 0:384], out_hbm.at[:, 0:384])]
    cps = [pltpu.make_async_copy(s, d, sem.at[i]) for i, (s, d) in enumerate(simple)]
    (cp_axt, cp_g1, cp_wrt, cp_wit, cp_perm, cp_m2, cp_g2, cp_bxt, cp_ckv0, cp_ckv1,
     cp_wot0, cp_wot1, cp_outa) = cps

    def wcopies(widx, w_hbm, w_buf, stage):
        src = w_hbm.bitcast(jnp.uint32)
        g, j0, n = ((0, 0, 1), (0, 1, 3), (1, 0, 4))[stage]
        return [pltpu.make_async_copy(
            src.at[:, p, pl.ds(4 * g + j0, n), pl.ds(128 * t, 128)],
            w_buf.at[g, t, :, pl.ds(4 * p + j0, n), :],
            wsem.at[widx, stage, 2 * t + p]) for t in range(2) for p in range(2)]

    wlist = [(0, wq_hbm, wq_w), (1, wuk_hbm, wuk_w), (2, wuv_hbm, wuv_w)]

    def head_weight(w_buf, rows, hh):
        g = lax.shift_right_logical(hh, 3)
        j = lax.shift_right_logical(hh, 1) & 3
        sh = ((hh & 1) * 16).astype(jnp.uint32)
        halves = []
        for t in range(2):
            w2 = w_buf.at[g, t].reshape(rows * 4, 128)
            a = w2[pl.ds(j, rows, stride=4), :]
            halves.append(pltpu.bitcast((a >> sh) << 16, F32))
        return jnp.concatenate(halves, axis=1)

    def orall(x):
        w = pltpu.bitcast(x, jnp.uint32)
        acc = None
        for r in range(0, w.shape[0], 8):
            for c in range(0, w.shape[1], 128):
                t = w[r:r + 8, c:min(c + 128, w.shape[1])]
                if t.shape[1] < 128:
                    continue
                acc = t if acc is None else acc | t
        return acc

    def prep_weights(hh):
        a = head_weight(wq_w, DA, hh).T.astype(BF)
        b = head_weight(wuk_w, C, hh).astype(BF)
        c = head_weight(wuv_w, C, hh).T.astype(BF)
        wqt_s[...] = a
        wk_s[...] = b
        wvt_s[...] = c
        deps = [orall(a)]
        if PREP_FENCE >= 2:
            deps.append(orall(b))
        if PREP_FENCE >= 3:
            deps.append(orall(c))
        d = deps[0]
        for e in deps[1:]:
            d = d | e
        return pltpu.bitcast(d, F32)

    NB = S // TQ
    key = lax.broadcasted_iota(jnp.int32, (HT, HT), 0)
    qry = lax.broadcasted_iota(jnp.int32, (HT, HT), 1)
    causal = key <= qry

    def proj_qk(i):
        cs = slice(i * TQ, (i + 1) * TQ)
        qt = jnp.dot(wqt_s[...], bxt[:, cs], preferred_element_type=F32) * (D ** -0.5 * LOG2E)
        qt_s[:, cs] = qt.astype(BF)
        k_s[cs, :] = jnp.dot(ckv[cs, :], wk_s[...], preferred_element_type=F32).astype(BF)

    def proj_v(i):
        cs = slice(i * TQ, (i + 1) * TQ)
        vt_s[:, cs] = lax.dot_general(wvt_s[...], ckv[cs, :], NT,
                                      preferred_element_type=F32).astype(BF)

    def colreduce(x, op, nacc=2):
        accs = [x[8 * a:8 * a + 8] for a in range(nacc)]
        for r in range(8 * nacc, x.shape[0], 8 * nacc):
            for a in range(nacc):
                accs[a] = op(accs[a], x[r + 8 * a:r + 8 * a + 8])
        while len(accs) > 1:
            accs = [op(accs[2 * a], accs[2 * a + 1]) for a in range(len(accs) // 2)]
        return accs[0]

    def fence(x, dep):
        never = (dep - dep) < -1.0
        head = pltpu.bitcast(x[0:16, 0:128], jnp.uint32)
        head = pltpu.bitcast(jnp.where(never, jnp.uint32(0), head), BF)
        top = jnp.concatenate([head, x[0:16, 128:]], axis=1)
        return jnp.concatenate([top, x[16:]], axis=0)

    def softmax_cols(st):
        m = jnp.max(colreduce(st, jnp.maximum), axis=0, keepdims=True)
        p = jnp.exp2(st - m)
        l = jnp.sum(colreduce(p, jnp.add), axis=0, keepdims=True)
        return p.astype(BF), 1.0 / l

    def qk_main(i, dep=None):
        L = (i + 1) * TQ
        qt = qt_s[:, i * TQ:(i + 1) * TQ]
        if dep is not None:
            qt = fence(qt, dep)
        return jnp.dot(k_s[0:L - HT, :], qt, preferred_element_type=F32)

    def qk_diag(i):
        L = (i + 1) * TQ
        return jnp.dot(k_s[L - HT:L, :], qt_s[:, L - HT:L], preferred_element_type=F32)

    def softmax(i, sa, sb):
        L = (i + 1) * TQ
        left = [jnp.where(causal, sa[L - TQ:, :HT], MASK_VAL)]
        if L > TQ:
            left = [sa[:L - TQ, :HT]] + left
        left = jnp.concatenate(left, axis=0)
        right = jnp.concatenate([sa[:, HT:], jnp.where(causal, sb, MASK_VAL)], axis=0)
        pl_, invl = softmax_cols(left)
        pr, invr = softmax_cols(right)
        pa = jnp.concatenate([pl_, pr[:L - HT]], axis=1)
        return pa, pr[L - HT:], jnp.concatenate([invl, invr], axis=1)

    def pv_diag(i, pb):
        L = (i + 1) * TQ
        top = jnp.dot(vt_s[0:HT, L - HT:L], pb, preferred_element_type=F32)
        bot = jnp.dot(vt_s[HT:D, L - HT:L], pb, preferred_element_type=F32)
        return jnp.concatenate([top, bot], axis=0)

    def pv(i, pa, ob, inv):
        L = (i + 1) * TQ
        oa = jnp.dot(vt_s[:, 0:L - HT], pa, preferred_element_type=F32)
        ot = jnp.concatenate([oa[:, :HT], oa[:, HT:] + ob], axis=1)
        return (ot * inv).astype(BF)

    def outproj(i, ot, hh):
        acc_s[64:512, i * TQ:(i + 1) * TQ] += jnp.dot(wot[hh], ot, preferred_element_type=F32)

    def save_first_block():
        pa, pb, inv = softmax(0, qk_main(0), qk_diag(0))
        p0_s[0:HT, :] = pa
        p0_s[HT:TQ, HT:TQ] = pb
        inv0_s[...] = jnp.broadcast_to(inv, (8, TQ))

    @pl.when(h == 0)
    def _prologue():
        for cp in (cp_axt, cp_g1, cp_wrt, cp_wit, cp_perm, cp_m2, cp_g2, cp_bxt):
            cp.start()
        for cp in wcopies(*wlist[0], 0):
            cp.start()
        cp_ckv0.start()
        for cp in wcopies(*wlist[1], 0) + wcopies(*wlist[2], 0):
            cp.start()
        cp_wot0.start()
        cp_ckv1.start()

        acc_s[...] = jnp.zeros_like(acc_s)

        cp_axt.wait()
        cp_g1.wait()

        def step1(c, carry):
            cols = pl.ds(pl.multiple_of(c * 512, 512), 512)
            x1_s[:, cols] = jnp.dot(g1[...], axt[:, cols], preferred_element_type=F32)
            return carry
        lax.fori_loop(0, S // 512, step1, 0)

        for r in range(0, FP, 8):
            xs = [(x1_s[r:r + 8, 128 * s1:128 * (s1 + 1)],
                   x1_s[FP + r:FP + r + 8, 128 * s1:128 * (s1 + 1)]) for s1 in range(N1)]
            ys = _fft16(xs, -1)
            for k1 in range(N1):
                a_s[k1, r:r + 8, 0:128] = ys[k1][0]
                a_s[k1, r:r + 8, 128:256] = ys[k1][1]
        a_s[:, FP:256, :] = jnp.zeros((N1, 256 - FP, 256), F32)

        cp_wrt.wait()
        cp_wit.wait()
        cp_perm.wait()
        zpad = jnp.zeros((128, 256 - DF), F32)
        for a in range(N1):
            for (src, dst) in ((wrt, wr_s), (wit, wi_s)):
                t = lax.dot_general(perm[...], src[:, 128 * a:128 * (a + 1)], NT,
                                    preferred_element_type=F32)
                t = jnp.concatenate([t, zpad], axis=1)
                for k1 in range(N1):
                    dst[k1, 8 * a:8 * (a + 1), :] = t[8 * k1:8 * (k1 + 1), :]

        cp_m2.wait()
        for k1 in range(N1):
            mk = m2[k1]
            u = lax.dot_general(mk, a_s[k1, :, 0:128].astype(BF), NT, preferred_element_type=F32)
            v = lax.dot_general(mk, a_s[k1, :, 128:256].astype(BF), NT, preferred_element_type=F32)
            zr = u[0:128] - v[128:256]
            zi = u[128:256] + v[0:128]
            wr, wi = wr_s[k1], wi_s[k1]
            yr = (zr * wr - zi * wi).astype(BF)
            yi = (zr * wi + zi * wr).astype(BF)
            rhs = jnp.concatenate([jnp.concatenate([yr, yi], axis=1),
                                   jnp.concatenate([yi, -yr], axis=1)], axis=0)
            b_s[k1] = lax.dot_general(mk, rhs, TN, preferred_element_type=F32)

        for g in range(N2 // 8):
            for t in range(2):
                xs = [(b_s[k1, 8 * g:8 * g + 8, 128 * t:128 * (t + 1)],
                       b_s[k1, 8 * g:8 * g + 8, 256 + 128 * t:256 + 128 * (t + 1)]) for k1 in range(N1)]
                ys = _fft16(xs, +1)
                for s1 in range(N1):
                    r0 = 128 * s1 + 8 * g
                    y1_s[r0:r0 + 8, 128 * t:128 * (t + 1)] = ys[s1][0]
                    y1_s[r0:r0 + 8, 256 + 128 * t:256 + 128 * (t + 1)] = ys[s1][1]
        cp_g2.wait()

        def step7(c, carry):
            rows = pl.ds(pl.multiple_of(c * 512, 512), 512)
            ya = jnp.dot(y1_s[rows, :].astype(BF), g2[...], preferred_element_type=F32)
            o_s[rows, 0:DA] = ya.astype(BF)
            return carry
        lax.fori_loop(0, S // 512, step7, 0)

        cp_outa.start()

        cp_bxt.wait()
        cp_ckv0.wait()
        for w in wlist:
            for cp in wcopies(*w, 0):
                cp.wait()
        prep_weights(h)
        proj_qk(0)
        proj_qk(1)
        proj_v(0)
        proj_v(1)
        save_first_block()
        ot7_s[...] = jnp.zeros_like(ot7_s)
        cp_wot0.wait()
        cp_ckv1.wait()
        for stage in (1, 2):
            for w in wlist:
                for cp in wcopies(*w, stage):
                    cp.start()
            if stage == 1:
                cp_wot1.start()

    @pl.when(h == 1)
    def _():
        for w in wlist:
            for cp in wcopies(*w, 1):
                cp.wait()
        cp_wot1.wait()
        cp_outa.wait()

    @pl.when(h == 6)
    def _():
        for w in wlist:
            for cp in wcopies(*w, 2):
                cp.wait()

    ps = {0: (p0_s[0:HT, :], p0_s[HT:TQ, HT:TQ], inv0_s[0:1, :])}
    ots = {-1: ot7_s[...]}
    for t in range(NB):
        pa, pb, inv = ps.pop(t)
        if t + 1 < NB:
            sa = qk_main(t + 1, dep if (PREP_FENCE and t + 1 == NB - 1) else None)
        if t + 2 < NB:
            proj_qk(t + 2)
            proj_v(t + 2)
            if t + 2 == NB - 1:
                dep = prep_weights(jnp.minimum(h + 1, H - 1))
        else:
            proj_qk(t + 2 - NB)
        if t + 1 < NB:
            ps[t + 1] = softmax(t + 1, sa, qk_diag(t + 1))
        else:
            save_first_block()
        ob = pv_diag(t, pb)
        ots[t] = pv(t, pa, ob, inv)
        if t == 0:
            outproj(NB - 1, ots.pop(-1), jnp.maximum(h - 1, 0))
        else:
            outproj(t - 1, ots.pop(t - 1), h)
    proj_v(0)
    proj_v(1)
    ot7_s[...] = ots.pop(NB - 1)

    @pl.when(h == H - 1)
    def _epilogue():
        outproj(NB - 1, ot7_s[...], H - 1)
        OB = 256
        lane = lax.broadcasted_iota(jnp.int32, (OB, 128), 1)
        outs = []
        for i in range(S // OB):
            rows = slice(i * OB, (i + 1) * OB)
            bt = acc_s[:, rows].T.astype(BF)
            first = jnp.where(lane < 64, o_s[rows, 384:512], bt[:, 0:128])
            o_s[rows, 384:512] = first
            o_s[rows, 512:896] = bt[:, 128:512]
            cp = pltpu.make_async_copy(o_s.at[rows, 384:896], out_hbm.at[rows, 384:896], osem.at[i])
            cp.start()
            outs.append(cp)
        for cp in outs:
            cp.wait()


@jax.jit
def pallas_concat_heads__spectral_gfnet__compressed_kv_cla__prompt_kernel(
    A_x, A_w_r, A_w_i, B_x, B_c_kv, B_w_q, B_w_uk, B_w_uv, B_w_o,
):
    g1, m2, g2, perm = _tables()
    axt = jnp.swapaxes(A_x, 1, 2).reshape(DA, S)
    bxt = jnp.swapaxes(B_x, 1, 2).reshape(DA, S)
    wrt = A_w_r.T
    wit = A_w_i.T
    ckv = B_c_kv.reshape(S, C)
    wq = B_w_q.reshape(DA // 2, 2, H, D)
    wuk = B_w_uk.reshape(C // 2, 2, H, D)
    wuv = B_w_uv.reshape(C // 2, 2, H, D)
    wot = jnp.swapaxes(B_w_o, 1, 2)

    any_spec = pl.BlockSpec(memory_space=pl.ANY)
    V = pltpu.VMEM
    out = pl.pallas_call(
        _kernel,
        grid=(H,),
        in_specs=[any_spec] * 13,
        out_specs=any_spec,
        out_shape=jax.ShapeDtypeStruct((S, 2 * DA), BF),
        scratch_shapes=[
            V((DA, S), BF), V((DF, S), BF), V((DF, S), BF), V((DA, S), BF), V((S, C), BF),
            V((2, 2, DA // 2, 8, 128), jnp.uint32),
            V((2, 2, C // 2, 8, 128), jnp.uint32),
            V((2, 2, C // 2, 8, 128), jnp.uint32),
            V((H, DA, D), BF),
            V((2 * FP, DA), BF), V((N1, 256, 128), BF), V((512, DA), BF),
            V((128, 128), BF),
            V((2 * FP, S), F32), V((N1, 256, 256), F32), V((N1, 128, 256), F32),
            V((N1, 128, 256), F32), V((N1, 128, 512), F32), V((S, 512), F32),
            V((D, DA), BF), V((C, D), BF), V((D, C), BF),
            V((D, S), BF), V((S, D), BF), V((D, S), BF), V((512, S), F32), V((S, 2 * DA), BF),
            V((TQ, TQ), BF), V((8, TQ), F32), V((D, TQ), BF),
            pltpu.SemaphoreType.DMA((13,)),
            pltpu.SemaphoreType.DMA((3, 3, 4)),
            pltpu.SemaphoreType.DMA((8,)),
        ],
        compiler_params=pltpu.CompilerParams(
            dimension_semantics=("arbitrary",),
            vmem_limit_bytes=120 * 2**20),
    )(axt, wrt, wit, bxt, ckv, wq, wuk, wuv, wot, g1, m2, g2, perm)
    return out.reshape(1, S, 2 * DA)
```

```python
import numpy as np
import jax
import jax.numpy as jnp
from jax import lax
import jax.experimental.pallas as pl
import jax.experimental.pallas.tpu as pltpu

S = 2048
DA = 448
DF = DA // 2 + 1
FP = 240
H = 16
D = 256
C = 1024
N1 = 16
N2 = 128
TQ = 256
HT = 128
PREP_FENCE = 1
LOG2E = 1.4426950408889634
MASK_VAL = -1e9 * LOG2E
BF = jnp.bfloat16
F32 = jnp.float32
NT = (((1,), (1,)), ((), ()))
TN = (((0,), (0,)), ((), ()))


def _tables():
    f = np.arange(FP)[:, None].astype(np.float64)
    d = np.arange(DA)[None, :].astype(np.float64)
    valid = (np.arange(FP) < DF)[:, None]
    ang = 2 * np.pi * ((f * d) % DA) / DA
    g1 = np.concatenate([np.cos(ang) * valid, -np.sin(ang) * valid], axis=0)
    k2 = np.arange(N2)[:, None]
    s2 = np.arange(N2)[None, :]
    m2 = np.zeros((N1, 2 * N2, N2))
    for k1 in range(N1):
        a = 2 * np.pi * ((s2 * (k1 + N1 * k2)) % S) / S
        m2[k1] = np.concatenate([np.cos(a), -np.sin(a)], axis=0)
    f2 = np.arange(256)[:, None].astype(np.float64)
    cf = np.where((f2 == 0) | (f2 == DA // 2), 1.0, 2.0) * (f2 < DF) / (S * DA)
    ang2 = 2 * np.pi * ((f2 * d) % DA) / DA
    g2 = np.concatenate([np.cos(ang2) * cf, -np.sin(ang2) * cf], axis=0)
    perm = np.zeros((128, 128))
    for k1 in range(N1):
        for j in range(8):
            perm[8 * k1 + j, k1 + 16 * j] = 1.0
    cast = lambda a: jnp.asarray(a.astype(np.float32), dtype=BF)
    return cast(g1), cast(m2), cast(g2), cast(perm)


def _fft4(xs, sign):
    (ar, ai), (br, bi), (cr, ci), (dr, di) = xs
    s0r, s0i = ar + cr, ai + ci
    s1r, s1i = ar - cr, ai - ci
    s2r, s2i = br + dr, bi + di
    s3r, s3i = br - dr, bi - di
    y0 = (s0r + s2r, s0i + s2i)
    y2 = (s0r - s2r, s0i - s2i)
    if sign < 0:
        y1 = (s1r + s3i, s1i - s3r)
        y3 = (s1r - s3i, s1i + s3r)
    else:
        y1 = (s1r - s3i, s1i + s3r)
        y3 = (s1r + s3i, s1i - s3r)
    return [y0, y1, y2, y3]


def _twiddle(z, e, sign):
    zr, zi = z
    e = e % 16
    if e == 0:
        return z
    if (e * sign) % 16 == 12:
        return (zi, -zr)
    if (e * sign) % 16 == 4:
        return (-zi, zr)
    c = float(np.cos(2 * np.pi * e / 16))
    s = float(sign * np.sin(2 * np.pi * e / 16))
    if abs(abs(c) - abs(s)) < 1e-12:
        r = abs(c)
        u = zr - zi if (c > 0) == (s > 0) else zr + zi
        v = zi + zr if (c > 0) == (s > 0) else zi - zr
        return (u * c, v * c)
    return (zr * c - zi * s, zi * c + zr * s)


def _fft16(xs, sign):
    t = [None] * 16
    for b in range(4):
        col = _fft4([xs[4 * a + b] for a in range(4)], sign)
        for c in range(4):
            t[4 * c + b] = _twiddle(col[c], b * c, sign)
    out = [None] * 16
    for c in range(4):
        col = _fft4([t[4 * c + b] for b in range(4)], sign)
        for e in range(4):
            out[c + 4 * e] = col[e]
    return out


def _kernel(axt_hbm, wrt_hbm, wit_hbm, bxt_hbm, ckv_hbm, wq_hbm, wuk_hbm, wuv_hbm, wot_hbm,
            g1_hbm, m2_hbm, g2_hbm, perm_hbm,
            out_hbm,
            axt, wrt, wit, bxt, ckv, wq_w, wuk_w, wuv_w, wot, g1, m2, g2, perm,
            x1_s, a_s, wr_s, wi_s, b_s, y1_s,
            wqt_s, wk_s, wvt_s, qt_s, k_s, vt_s, acc_s, o_s, p0_s, inv0_s, ot7_s,
            sem, wsem, osem, asem):
    h = pl.program_id(0)

    CK0 = 2 * TQ
    simple = [(g1_hbm, g1), (wrt_hbm, wrt), (wit_hbm, wit), (perm_hbm, perm),
              (m2_hbm, m2), (g2_hbm, g2), (bxt_hbm, bxt),
              (ckv_hbm.at[0:CK0], ckv.at[0:CK0]), (ckv_hbm.at[CK0:S], ckv.at[CK0:S]),
              (wot_hbm.at[0:1], wot.at[0:1]), (wot_hbm.at[1:H], wot.at[1:H]),
              (o_s.at[:, 0:384], out_hbm.at[:, 0:384])]
    cps = [pltpu.make_async_copy(s, d, sem.at[i]) for i, (s, d) in enumerate(simple)]
    (cp_g1, cp_wrt, cp_wit, cp_perm, cp_m2, cp_g2, cp_bxt, cp_ckv0, cp_ckv1,
     cp_wot0, cp_wot1, cp_outa) = cps

    def axt_copy(c):
        cols = pl.ds(pl.multiple_of(c * 512, 512), 512)
        return pltpu.make_async_copy(axt_hbm.at[:, cols], axt.at[:, cols], asem.at[c])

    def wcopies(widx, w_hbm, w_buf, stage):
        src = w_hbm.bitcast(jnp.uint32)
        g, j0, n = ((0, 0, 1), (0, 1, 3), (1, 0, 4))[stage]
        return [pltpu.make_async_copy(
            src.at[:, p, pl.ds(4 * g + j0, n), pl.ds(128 * t, 128)],
            w_buf.at[g, t, :, pl.ds(4 * p + j0, n), :],
            wsem.at[widx, stage, 2 * t + p]) for t in range(2) for p in range(2)]

    wlist = [(0, wq_hbm, wq_w), (1, wuk_hbm, wuk_w), (2, wuv_hbm, wuv_w)]

    def head_weight(w_buf, rows, hh):
        g = lax.shift_right_logical(hh, 3)
        j = lax.shift_right_logical(hh, 1) & 3
        sh = ((hh & 1) * 16).astype(jnp.uint32)
        halves = []
        for t in range(2):
            w2 = w_buf.at[g, t].reshape(rows * 4, 128)
            a = w2[pl.ds(j, rows, stride=4), :]
            halves.append(pltpu.bitcast((a >> sh) << 16, F32))
        return jnp.concatenate(halves, axis=1)

    def orall(x):
        w = pltpu.bitcast(x, jnp.uint32)
        acc = None
        for r in range(0, w.shape[0], 8):
            for c in range(0, w.shape[1], 128):
                t = w[r:r + 8, c:min(c + 128, w.shape[1])]
                if t.shape[1] < 128:
                    continue
                acc = t if acc is None else acc | t
        return acc

    def prep_weights(hh):
        a = head_weight(wq_w, DA, hh).T.astype(BF)
        b = head_weight(wuk_w, C, hh).astype(BF)
        c = head_weight(wuv_w, C, hh).T.astype(BF)
        wqt_s[...] = a
        wk_s[...] = b
        wvt_s[...] = c
        deps = [orall(a)]
        if PREP_FENCE >= 2:
            deps.append(orall(b))
        if PREP_FENCE >= 3:
            deps.append(orall(c))
        d = deps[0]
        for e in deps[1:]:
            d = d | e
        return pltpu.bitcast(d, F32)

    NB = S // TQ
    key = lax.broadcasted_iota(jnp.int32, (HT, HT), 0)
    qry = lax.broadcasted_iota(jnp.int32, (HT, HT), 1)
    causal = key <= qry

    def proj_qk(i):
        cs = slice(i * TQ, (i + 1) * TQ)
        qt = jnp.dot(wqt_s[...], bxt[:, cs], preferred_element_type=F32) * (D ** -0.5 * LOG2E)
        qt_s[:, cs] = qt.astype(BF)
        k_s[cs, :] = jnp.dot(ckv[cs, :], wk_s[...], preferred_element_type=F32).astype(BF)

    def proj_v(i):
        cs = slice(i * TQ, (i + 1) * TQ)
        vt_s[:, cs] = lax.dot_general(wvt_s[...], ckv[cs, :], NT,
                                      preferred_element_type=F32).astype(BF)

    def colreduce(x, op, nacc=2):
        accs = [x[8 * a:8 * a + 8] for a in range(nacc)]
        for r in range(8 * nacc, x.shape[0], 8 * nacc):
            for a in range(nacc):
                accs[a] = op(accs[a], x[r + 8 * a:r + 8 * a + 8])
        while len(accs) > 1:
            accs = [op(accs[2 * a], accs[2 * a + 1]) for a in range(len(accs) // 2)]
        return accs[0]

    def fence(x, dep):
        never = (dep - dep) < -1.0
        head = pltpu.bitcast(x[0:16, 0:128], jnp.uint32)
        head = pltpu.bitcast(jnp.where(never, jnp.uint32(0), head), BF)
        top = jnp.concatenate([head, x[0:16, 128:]], axis=1)
        return jnp.concatenate([top, x[16:]], axis=0)

    def softmax_cols(st):
        m = jnp.max(colreduce(st, jnp.maximum), axis=0, keepdims=True)
        p = jnp.exp2(st - m)
        l = jnp.sum(colreduce(p, jnp.add), axis=0, keepdims=True)
        return p, 1.0 / l

    def qk_main(i, dep=None):
        L = (i + 1) * TQ
        qt = qt_s[:, i * TQ:(i + 1) * TQ]
        if dep is not None:
            qt = fence(qt, dep)
        return jnp.dot(k_s[0:L - HT, :], qt, preferred_element_type=F32)

    def qk_diag(i):
        L = (i + 1) * TQ
        return jnp.dot(k_s[L - HT:L, :], qt_s[:, L - HT:L], preferred_element_type=F32)

    def softmax(i, sa, sb):
        L = (i + 1) * TQ
        left = [jnp.where(causal, sa[L - TQ:, :HT], MASK_VAL)]
        if L > TQ:
            left = [sa[:L - TQ, :HT]] + left
        left = jnp.concatenate(left, axis=0)
        right = jnp.concatenate([sa[:, HT:], jnp.where(causal, sb, MASK_VAL)], axis=0)
        pl_, invl = softmax_cols(left)
        pr, invr = softmax_cols(right)
        pa = jnp.concatenate([pl_, pr[:L - HT]], axis=1).astype(BF)
        return pa, pr[L - HT:].astype(BF), jnp.concatenate([invl, invr], axis=1)

    def pv_diag(i, pb):
        L = (i + 1) * TQ
        top = jnp.dot(vt_s[0:HT, L - HT:L], pb, preferred_element_type=F32)
        bot = jnp.dot(vt_s[HT:D, L - HT:L], pb, preferred_element_type=F32)
        return jnp.concatenate([top, bot], axis=0)

    def pv(i, pa, ob, inv):
        L = (i + 1) * TQ
        oa = jnp.dot(vt_s[:, 0:L - HT], pa, preferred_element_type=F32)
        ot = jnp.concatenate([oa[:, :HT], oa[:, HT:] + ob], axis=1)
        return (ot * inv).astype(BF)

    def outproj(i, ot, hh):
        acc_s[64:512, i * TQ:(i + 1) * TQ] += jnp.dot(wot[hh], ot, preferred_element_type=F32)

    def save_first_block():
        pa, pb, inv = softmax(0, qk_main(0), qk_diag(0))
        p0_s[0:HT, :] = pa
        p0_s[HT:TQ, HT:TQ] = pb
        inv0_s[...] = jnp.broadcast_to(inv, (8, TQ))

    @pl.when(h == 0)
    def _prologue():
        cp_g1.start()
        for c in range(S // 512):
            axt_copy(c).start()
        for cp in (cp_wrt, cp_wit, cp_perm, cp_m2, cp_bxt):
            cp.start(priority=1)
        for cp in wcopies(*wlist[0], 0):
            cp.start(priority=1)
        cp_ckv0.start(priority=1)
        for cp in wcopies(*wlist[1], 0) + wcopies(*wlist[2], 0):
            cp.start(priority=1)
        cp_g2.start(priority=1)
        cp_wot0.start(priority=1)
        cp_ckv1.start(priority=1)

        acc_s[...] = jnp.zeros_like(acc_s)

        cp_g1.wait()

        def step1(c, carry):
            axt_copy(c).wait()
            cols = pl.ds(pl.multiple_of(c * 512, 512), 512)
            x1_s[:, cols] = jnp.dot(g1[...], axt[:, cols], preferred_element_type=F32)
            return carry
        lax.fori_loop(0, S // 512, step1, 0)

        cp_wrt.wait()
        cp_wit.wait()
        cp_perm.wait()
        zpad = jnp.zeros((128, 256 - DF), F32)
        for a in range(N1):
            for (src, dst) in ((wrt, wr_s), (wit, wi_s)):
                t = lax.dot_general(perm[...], src[:, 128 * a:128 * (a + 1)], NT,
                                    preferred_element_type=F32)
                t = jnp.concatenate([t, zpad], axis=1)
                for k1 in range(N1):
                    dst[k1, 8 * a:8 * (a + 1), :] = t[8 * k1:8 * (k1 + 1), :]

        for r in range(0, FP, 8):
            xs = [(x1_s[r:r + 8, 128 * s1:128 * (s1 + 1)],
                   x1_s[FP + r:FP + r + 8, 128 * s1:128 * (s1 + 1)]) for s1 in range(N1)]
            ys = _fft16(xs, -1)
            for k1 in range(N1):
                a_s[k1, r:r + 8, 0:128] = ys[k1][0]
                a_s[k1, r:r + 8, 128:256] = ys[k1][1]
        a_s[:, FP:256, :] = jnp.zeros((N1, 256 - FP, 256), F32)

        cp_m2.wait()

        def mid_fwd(k1):
            mk = m2[k1]
            u = lax.dot_general(mk, a_s[k1, :, 0:128].astype(BF), NT, preferred_element_type=F32)
            v = lax.dot_general(mk, a_s[k1, :, 128:256].astype(BF), NT, preferred_element_type=F32)
            zr = u[0:128] - v[128:256]
            zi = u[128:256] + v[0:128]
            wr, wi = wr_s[k1], wi_s[k1]
            yr = (zr * wr - zi * wi).astype(BF)
            yi = (zr * wi + zi * wr).astype(BF)
            return jnp.concatenate([jnp.concatenate([yr, yi], axis=1),
                                    jnp.concatenate([yi, -yr], axis=1)], axis=0)

        rhs = {0: mid_fwd(0)}
        for k1 in range(N1):
            if k1 + 1 < N1:
                rhs[k1 + 1] = mid_fwd(k1 + 1)
            b_s[k1] = lax.dot_general(m2[k1], rhs.pop(k1), TN, preferred_element_type=F32)

        cp_bxt.wait()
        cp_ckv0.wait()
        for w in wlist:
            for cp in wcopies(*w, 0):
                cp.wait()
        prep_weights(h)
        proj_qk(0)
        proj_qk(1)
        proj_v(0)
        proj_v(1)
        save_first_block()
        ot7_s[...] = jnp.zeros_like(ot7_s)

        for g in range(N2 // 8):
            for t in range(2):
                xs = [(b_s[k1, 8 * g:8 * g + 8, 128 * t:128 * (t + 1)],
                       b_s[k1, 8 * g:8 * g + 8, 256 + 128 * t:256 + 128 * (t + 1)]) for k1 in range(N1)]
                ys = _fft16(xs, +1)
                for s1 in range(N1):
                    r0 = 128 * s1 + 8 * g
                    y1_s[r0:r0 + 8, 128 * t:128 * (t + 1)] = ys[s1][0]
                    y1_s[r0:r0 + 8, 256 + 128 * t:256 + 128 * (t + 1)] = ys[s1][1]
        cp_g2.wait()

        def step7(c, carry):
            rows = pl.ds(pl.multiple_of(c * 512, 512), 512)
            ya = jnp.dot(y1_s[rows, :].astype(BF), g2[...], preferred_element_type=F32)
            o_s[rows, 0:DA] = ya.astype(BF)
            return carry
        lax.fori_loop(0, S // 512, step7, 0)
        cp_outa.start()

        cp_wot0.wait()
        cp_ckv1.wait()
        for w in wlist:
            for cp in wcopies(*w, 1):
                cp.start()
        cp_wot1.start()

    @pl.when(h == 1)
    def _():
        for w in wlist:
            for cp in wcopies(*w, 1):
                cp.wait()
        cp_wot1.wait()
        cp_outa.wait()
        for w in wlist:
            for cp in wcopies(*w, 2):
                cp.start()

    @pl.when(h == 6)
    def _():
        for w in wlist:
            for cp in wcopies(*w, 2):
                cp.wait()

    ps = {0: (p0_s[0:HT, :], p0_s[HT:TQ, HT:TQ], inv0_s[0:1, :])}
    ots = {-1: ot7_s[...]}
    for t in range(NB):
        pa, pb, inv = ps.pop(t)
        if t + 1 < NB:
            sa = qk_main(t + 1, dep if (PREP_FENCE and t + 1 == NB - 1) else None)
        if t + 2 < NB:
            proj_qk(t + 2)
            proj_v(t + 2)
            if t + 2 == NB - 1:
                dep = prep_weights(jnp.minimum(h + 1, H - 1))
        else:
            proj_qk(t + 2 - NB)
        if t + 1 < NB:
            ps[t + 1] = softmax(t + 1, sa, qk_diag(t + 1))
        else:
            save_first_block()
        ob = pv_diag(t, pb)
        ots[t] = pv(t, pa, ob, inv)
        if t == 0:
            outproj(NB - 1, ots.pop(-1), jnp.maximum(h - 1, 0))
        else:
            outproj(t - 1, ots.pop(t - 1), h)
    proj_v(0)
    proj_v(1)
    ot7_s[...] = ots.pop(NB - 1)

    @pl.when(h == H - 1)
    def _epilogue():
        outproj(NB - 1, ot7_s[...], H - 1)
        OB = 256
        lane = lax.broadcasted_iota(jnp.int32, (OB, 128), 1)
        outs = []
        for i in range(S // OB):
            rows = slice(i * OB, (i + 1) * OB)
            bt = acc_s[:, rows].T.astype(BF)
            first = jnp.where(lane < 64, o_s[rows, 384:512], bt[:, 0:128])
            o_s[rows, 384:512] = first
            o_s[rows, 512:896] = bt[:, 128:512]
            cp = pltpu.make_async_copy(o_s.at[rows, 384:896], out_hbm.at[rows, 384:896], osem.at[i])
            cp.start()
            outs.append(cp)
        for cp in outs:
            cp.wait()


@jax.jit
def pallas_concat_heads__spectral_gfnet__compressed_kv_cla__prompt_kernel(
    A_x, A_w_r, A_w_i, B_x, B_c_kv, B_w_q, B_w_uk, B_w_uv, B_w_o,
):
    g1, m2, g2, perm = _tables()
    axt = jnp.swapaxes(A_x, 1, 2).reshape(DA, S)
    bxt = jnp.swapaxes(B_x, 1, 2).reshape(DA, S)
    wrt = A_w_r.T
    wit = A_w_i.T
    ckv = B_c_kv.reshape(S, C)
    wq = B_w_q.reshape(DA // 2, 2, H, D)
    wuk = B_w_uk.reshape(C // 2, 2, H, D)
    wuv = B_w_uv.reshape(C // 2, 2, H, D)
    wot = jnp.swapaxes(B_w_o, 1, 2)

    any_spec = pl.BlockSpec(memory_space=pl.ANY)
    V = pltpu.VMEM
    out = pl.pallas_call(
        _kernel,
        grid=(H,),
        in_specs=[any_spec] * 13,
        out_specs=any_spec,
        out_shape=jax.ShapeDtypeStruct((S, 2 * DA), BF),
        scratch_shapes=[
            V((DA, S), BF), V((DF, S), BF), V((DF, S), BF), V((DA, S), BF), V((S, C), BF),
            V((2, 2, DA // 2, 8, 128), jnp.uint32),
            V((2, 2, C // 2, 8, 128), jnp.uint32),
            V((2, 2, C // 2, 8, 128), jnp.uint32),
            V((H, DA, D), BF),
            V((2 * FP, DA), BF), V((N1, 256, 128), BF), V((512, DA), BF),
            V((128, 128), BF),
            V((2 * FP, S), F32), V((N1, 256, 256), F32), V((N1, 128, 256), F32),
            V((N1, 128, 256), F32), V((N1, 128, 512), F32), V((S, 512), F32),
            V((D, DA), BF), V((C, D), BF), V((D, C), BF),
            V((D, S), BF), V((S, D), BF), V((D, S), BF), V((512, S), F32), V((S, 2 * DA), BF),
            V((TQ, TQ), BF), V((8, TQ), F32), V((D, TQ), BF),
            pltpu.SemaphoreType.DMA((12,)),
            pltpu.SemaphoreType.DMA((3, 3, 4)),
            pltpu.SemaphoreType.DMA((8,)),
            pltpu.SemaphoreType.DMA((4,)),
        ],
        compiler_params=pltpu.CompilerParams(
            dimension_semantics=("arbitrary",),
            vmem_limit_bytes=120 * 2**20),
    )(axt, wrt, wit, bxt, ckv, wq, wuk, wuv, wot, g1, m2, g2, perm)
    return out.reshape(1, S, 2 * DA)
```

```python
import numpy as np
import jax
import jax.numpy as jnp
from jax import lax
import jax.experimental.pallas as pl
import jax.experimental.pallas.tpu as pltpu

S = 2048
DA = 448
DF = DA // 2 + 1
FP = 240
H = 16
D = 256
C = 1024
N1 = 16
N2 = 128
TQ = 256
HT = 128
QC = 256
QK_LAG = 2
PREP_FENCE = 1
LOG2E = 1.4426950408889634
MASK_VAL = -1e9 * LOG2E
BF = jnp.bfloat16
F32 = jnp.float32
NT = (((1,), (1,)), ((), ()))
TN = (((0,), (0,)), ((), ()))


def _tables():
    f = np.arange(FP)[:, None].astype(np.float64)
    d = np.arange(DA)[None, :].astype(np.float64)
    valid = (np.arange(FP) < DF)[:, None]
    ang = 2 * np.pi * ((f * d) % DA) / DA
    g1 = np.concatenate([np.cos(ang) * valid, -np.sin(ang) * valid], axis=0)
    k2 = np.arange(N2)[:, None]
    s2 = np.arange(N2)[None, :]
    m2 = np.zeros((N1, 2 * N2, N2))
    for k1 in range(N1):
        a = 2 * np.pi * ((s2 * (k1 + N1 * k2)) % S) / S
        m2[k1] = np.concatenate([np.cos(a), -np.sin(a)], axis=0)
    f2 = np.arange(256)[:, None].astype(np.float64)
    cf = np.where((f2 == 0) | (f2 == DA // 2), 1.0, 2.0) * (f2 < DF) / (S * DA)
    ang2 = 2 * np.pi * ((f2 * d) % DA) / DA
    g2 = np.concatenate([np.cos(ang2) * cf, -np.sin(ang2) * cf], axis=0)
    perm = np.zeros((128, 128))
    for k1 in range(N1):
        for j in range(8):
            perm[8 * k1 + j, k1 + 16 * j] = 1.0
    cast = lambda a: jnp.asarray(a.astype(np.float32), dtype=BF)
    return cast(g1), cast(m2), cast(g2), cast(perm)


def _fft4(xs, sign):
    (ar, ai), (br, bi), (cr, ci), (dr, di) = xs
    s0r, s0i = ar + cr, ai + ci
    s1r, s1i = ar - cr, ai - ci
    s2r, s2i = br + dr, bi + di
    s3r, s3i = br - dr, bi - di
    y0 = (s0r + s2r, s0i + s2i)
    y2 = (s0r - s2r, s0i - s2i)
    if sign < 0:
        y1 = (s1r + s3i, s1i - s3r)
        y3 = (s1r - s3i, s1i + s3r)
    else:
        y1 = (s1r - s3i, s1i + s3r)
        y3 = (s1r + s3i, s1i - s3r)
    return [y0, y1, y2, y3]


def _twiddle(z, e, sign):
    zr, zi = z
    e = e % 16
    if e == 0:
        return z
    if (e * sign) % 16 == 12:
        return (zi, -zr)
    if (e * sign) % 16 == 4:
        return (-zi, zr)
    c = float(np.cos(2 * np.pi * e / 16))
    s = float(sign * np.sin(2 * np.pi * e / 16))
    if abs(abs(c) - abs(s)) < 1e-12:
        r = abs(c)
        u = zr - zi if (c > 0) == (s > 0) else zr + zi
        v = zi + zr if (c > 0) == (s > 0) else zi - zr
        return (u * c, v * c)
    return (zr * c - zi * s, zi * c + zr * s)


def _fft16(xs, sign):
    t = [None] * 16
    for b in range(4):
        col = _fft4([xs[4 * a + b] for a in range(4)], sign)
        for c in range(4):
            t[4 * c + b] = _twiddle(col[c], b * c, sign)
    out = [None] * 16
    for c in range(4):
        col = _fft4([t[4 * c + b] for b in range(4)], sign)
        for e in range(4):
            out[c + 4 * e] = col[e]
    return out


def _kernel(axt_hbm, wrt_hbm, wit_hbm, bxt_hbm, ckv_hbm, wq_hbm, wuk_hbm, wuv_hbm, wot_hbm,
            g1_hbm, m2_hbm, g2_hbm, perm_hbm,
            out_hbm,
            axt, wrt, wit, bxt, ckv, wq_w, wuk_w, wuv_w, wot, g1, m2, g2, perm,
            x1_s, a_s, wr_s, wi_s, b_s, y1_s,
            wqt_s, wk_s, wvt_s, qt_s, k_s, vt_s, acc_s, o_s, p0_s, inv0_s, ot7_s,
            sem, wsem, osem, asem):
    h = pl.program_id(0)

    CK0 = 2 * TQ
    simple = [(g1_hbm, g1), (wrt_hbm, wrt), (wit_hbm, wit), (perm_hbm, perm),
              (m2_hbm, m2), (g2_hbm, g2), (bxt_hbm, bxt.at[0:DA]),
              (ckv_hbm.at[0:CK0], ckv.at[0:CK0]), (ckv_hbm.at[CK0:S], ckv.at[CK0:S]),
              (wot_hbm.at[0:1], wot.at[0:1]), (wot_hbm.at[1:H], wot.at[1:H]),
              (o_s.at[:, 0:384], out_hbm.at[:, 0:384])]
    cps = [pltpu.make_async_copy(s, d, sem.at[i]) for i, (s, d) in enumerate(simple)]
    (cp_g1, cp_wrt, cp_wit, cp_perm, cp_m2, cp_g2, cp_bxt, cp_ckv0, cp_ckv1,
     cp_wot0, cp_wot1, cp_outa) = cps

    def axt_copy(c):
        cols = pl.ds(pl.multiple_of(c * 512, 512), 512)
        return pltpu.make_async_copy(axt_hbm.at[:, cols], axt.at[:, cols], asem.at[c])

    def wcopies(widx, w_hbm, w_buf, stage):
        src = w_hbm.bitcast(jnp.uint32)
        g, j0, n = ((0, 0, 1), (0, 1, 3), (1, 0, 4))[stage]
        return [pltpu.make_async_copy(
            src.at[:, p, pl.ds(4 * g + j0, n), pl.ds(128 * t, 128)],
            w_buf.at[g, t, :, pl.ds(4 * p + j0, n), :],
            wsem.at[widx, stage, 2 * t + p]) for t in range(2) for p in range(2)]

    wlist = [(0, wq_hbm, wq_w), (1, wuk_hbm, wuk_w), (2, wuv_hbm, wuv_w)]

    def head_weight(w_buf, rows, hh):
        g = lax.shift_right_logical(hh, 3)
        j = lax.shift_right_logical(hh, 1) & 3
        sh = ((hh & 1) * 16).astype(jnp.uint32)
        halves = []
        for t in range(2):
            w2 = w_buf.at[g, t].reshape(rows * 4, 128)
            a = w2[pl.ds(j, rows, stride=4), :]
            halves.append(pltpu.bitcast((a >> sh) << 16, F32))
        return jnp.concatenate(halves, axis=1)

    def orall(x):
        w = pltpu.bitcast(x, jnp.uint32)
        acc = None
        for r in range(0, w.shape[0], 8):
            for c in range(0, w.shape[1], 128):
                t = w[r:r + 8, c:min(c + 128, w.shape[1])]
                if t.shape[1] < 128:
                    continue
                acc = t if acc is None else acc | t
        return acc

    def prep_weights(hh):
        a = head_weight(wq_w, DA, hh).T.astype(BF)
        b = head_weight(wuk_w, C, hh).astype(BF)
        c = head_weight(wuv_w, C, hh).T.astype(BF)
        wqt_s[:, 0:DA] = a
        wk_s[...] = b
        wvt_s[...] = c
        deps = [orall(a)]
        if PREP_FENCE >= 2:
            deps.append(orall(b))
        if PREP_FENCE >= 3:
            deps.append(orall(c))
        d = deps[0]
        for e in deps[1:]:
            d = d | e
        return pltpu.bitcast(d, F32)

    NB = S // TQ
    key = lax.broadcasted_iota(jnp.int32, (HT, HT), 0)
    qry = lax.broadcasted_iota(jnp.int32, (HT, HT), 1)
    causal = key <= qry

    def proj_qk(i):
        cs = slice(i * TQ, (i + 1) * TQ)
        qt = jnp.dot(wqt_s[...], bxt[:, cs], preferred_element_type=F32) * (D ** -0.5 * LOG2E)
        qt_s[:, cs] = qt.astype(BF)
        k_s[cs, :] = jnp.dot(ckv[cs, :], wk_s[...], preferred_element_type=F32).astype(BF)

    def proj_v(i):
        cs = slice(i * TQ, (i + 1) * TQ)
        vt_s[:, cs] = lax.dot_general(wvt_s[...], ckv[cs, :], NT,
                                      preferred_element_type=F32).astype(BF)

    def colreduce(x, op, nacc=2):
        accs = [x[8 * a:8 * a + 8] for a in range(nacc)]
        for r in range(8 * nacc, x.shape[0], 8 * nacc):
            for a in range(nacc):
                accs[a] = op(accs[a], x[r + 8 * a:r + 8 * a + 8])
        while len(accs) > 1:
            accs = [op(accs[2 * a], accs[2 * a + 1]) for a in range(len(accs) // 2)]
        return accs[0]

    def fence(x, dep):
        never = (dep - dep) < -1.0
        head = pltpu.bitcast(x[0:16, 0:128], jnp.uint32)
        head = pltpu.bitcast(jnp.where(never, jnp.uint32(0), head), BF)
        top = jnp.concatenate([head, x[0:16, 128:]], axis=1)
        return jnp.concatenate([top, x[16:]], axis=0)

    def qk_main(i, dep=None):
        L = (i + 1) * TQ
        qt = qt_s[:, i * TQ:(i + 1) * TQ]
        if dep is not None:
            qt = fence(qt, dep)
        bounds = list(range(0, L - HT, QC)) + [L - HT]
        sts, ms = [], []
        for c in range(len(bounds) - 1):
            kc = k_s[bounds[c]:bounds[c + 1], :]
            if c >= QK_LAG:
                kc = fence(kc, ms[c - QK_LAG][:, 0:HT] + ms[c - QK_LAG][:, HT:])
            st = jnp.dot(kc, qt, preferred_element_type=F32)
            if c == len(bounds) - 2:
                n = st.shape[0]
                dg = jnp.concatenate([jnp.where(causal, st[n - HT:, :HT], MASK_VAL), st[n - HT:, HT:]], axis=1)
                st = jnp.concatenate([st[:n - HT], dg], axis=0) if n > HT else dg
            mc = colreduce(st, jnp.maximum)
            ms.append(mc if c == 0 else jnp.maximum(ms[-1], mc))
            sts.append(st)
        return jnp.concatenate(sts, axis=0), ms[-1]

    def qk_diag(i):
        L = (i + 1) * TQ
        return jnp.dot(k_s[L - HT:L, :], qt_s[:, L - HT:L], preferred_element_type=F32)

    def softmax(i, sa_m8, sb):
        sa, m8 = sa_m8
        L = (i + 1) * TQ
        sb = jnp.where(causal, sb, MASK_VAL)
        ml = jnp.max(m8[:, :HT], axis=0, keepdims=True)
        mr = jnp.max(jnp.maximum(m8[:, HT:], colreduce(sb, jnp.maximum)), axis=0, keepdims=True)
        pa = jnp.exp2(sa - jnp.concatenate([ml, mr], axis=1))
        pb = jnp.exp2(sb - mr)
        l8 = colreduce(pa, jnp.add)
        ll = jnp.sum(l8[:, :HT], axis=0, keepdims=True)
        lr = jnp.sum(l8[:, HT:] + colreduce(pb, jnp.add), axis=0, keepdims=True)
        return pa.astype(BF), pb.astype(BF), 1.0 / jnp.concatenate([ll, lr], axis=1)

    def pv_diag(i, pb):
        L = (i + 1) * TQ
        top = jnp.dot(vt_s[0:HT, L - HT:L], pb, preferred_element_type=F32)
        bot = jnp.dot(vt_s[HT:D, L - HT:L], pb, preferred_element_type=F32)
        return jnp.concatenate([top, bot], axis=0)

    def pv(i, pa, ob, inv):
        L = (i + 1) * TQ
        oa = jnp.dot(vt_s[:, 0:L - HT], pa, preferred_element_type=F32)
        ot = jnp.concatenate([oa[:, :HT], oa[:, HT:] + ob], axis=1)
        return (ot * inv).astype(BF)

    def outproj(i, ot, hh):
        acc_s[64:512, i * TQ:(i + 1) * TQ] += jnp.dot(wot[hh], ot, preferred_element_type=F32)

    def save_first_block():
        pa, pb, inv = softmax(0, qk_main(0), qk_diag(0))
        p0_s[0:HT, :] = pa
        p0_s[HT:TQ, HT:TQ] = pb
        inv0_s[...] = jnp.broadcast_to(inv, (8, TQ))

    @pl.when(h == 0)
    def _prologue():
        cp_g1.start()
        for c in range(S // 512):
            axt_copy(c).start()
        for cp in (cp_wrt, cp_wit, cp_perm, cp_m2, cp_bxt):
            cp.start(priority=1)
        for cp in wcopies(*wlist[0], 0):
            cp.start(priority=1)
        cp_ckv0.start(priority=1)
        for cp in wcopies(*wlist[1], 0) + wcopies(*wlist[2], 0):
            cp.start(priority=1)
        cp_g2.start(priority=1)
        cp_wot0.start(priority=1)
        cp_ckv1.start(priority=1)

        acc_s[...] = jnp.zeros_like(acc_s)
        bxt[DA:512, :] = jnp.zeros((512 - DA, S), BF)
        wqt_s[...] = jnp.zeros_like(wqt_s)

        cp_g1.wait()

        def step1(c, carry):
            axt_copy(c).wait()
            cols = pl.ds(pl.multiple_of(c * 512, 512), 512)
            x1_s[:, cols] = jnp.dot(g1[...], axt[:, cols], preferred_element_type=F32)
            return carry
        lax.fori_loop(0, S // 512, step1, 0)

        cp_wrt.wait()
        cp_wit.wait()
        cp_perm.wait()
        zpad = jnp.zeros((128, 256 - DF), F32)
        for a in range(N1):
            for (src, dst) in ((wrt, wr_s), (wit, wi_s)):
                t = lax.dot_general(perm[...], src[:, 128 * a:128 * (a + 1)], NT,
                                    preferred_element_type=F32)
                t = jnp.concatenate([t, zpad], axis=1)
                for k1 in range(N1):
                    dst[k1, 8 * a:8 * (a + 1), :] = t[8 * k1:8 * (k1 + 1), :]

        for r in range(0, FP, 8):
            xs = [(x1_s[r:r + 8, 128 * s1:128 * (s1 + 1)],
                   x1_s[FP + r:FP + r + 8, 128 * s1:128 * (s1 + 1)]) for s1 in range(N1)]
            ys = _fft16(xs, -1)
            for k1 in range(N1):
                a_s[k1, r:r + 8, 0:128] = ys[k1][0]
                a_s[k1, r:r + 8, 128:256] = ys[k1][1]
        a_s[:, FP:256, :] = jnp.zeros((N1, 256 - FP, 256), F32)

        cp_m2.wait()

        def mid_fwd(k1):
            mk = m2[k1]
            u = lax.dot_general(mk, a_s[k1, :, 0:128].astype(BF), NT, preferred_element_type=F32)
            v = lax.dot_general(mk, a_s[k1, :, 128:256].astype(BF), NT, preferred_element_type=F32)
            zr = u[0:128] - v[128:256]
            zi = u[128:256] + v[0:128]
            wr, wi = wr_s[k1], wi_s[k1]
            yr = (zr * wr - zi * wi).astype(BF)
            yi = (zr * wi + zi * wr).astype(BF)
            return jnp.concatenate([jnp.concatenate([yr, yi], axis=1),
                                    jnp.concatenate([yi, -yr], axis=1)], axis=0)

        rhs = {0: mid_fwd(0)}
        for k1 in range(N1):
            if k1 + 1 < N1:
                rhs[k1 + 1] = mid_fwd(k1 + 1)
            b_s[k1] = lax.dot_general(m2[k1], rhs.pop(k1), TN, preferred_element_type=F32)

        cp_bxt.wait()
        cp_ckv0.wait()
        for w in wlist:
            for cp in wcopies(*w, 0):
                cp.wait()
        prep_weights(h)
        proj_qk(0)
        proj_qk(1)
        proj_v(0)
        proj_v(1)
        save_first_block()
        ot7_s[...] = jnp.zeros_like(ot7_s)

        for g in range(N2 // 8):
            for t in range(2):
                xs = [(b_s[k1, 8 * g:8 * g + 8, 128 * t:128 * (t + 1)],
                       b_s[k1, 8 * g:8 * g + 8, 256 + 128 * t:256 + 128 * (t + 1)]) for k1 in range(N1)]
                ys = _fft16(xs, +1)
                for s1 in range(N1):
                    r0 = 128 * s1 + 8 * g
                    y1_s[r0:r0 + 8, 128 * t:128 * (t + 1)] = ys[s1][0]
                    y1_s[r0:r0 + 8, 256 + 128 * t:256 + 128 * (t + 1)] = ys[s1][1]
        cp_g2.wait()

        def step7(c, carry):
            rows = pl.ds(pl.multiple_of(c * 512, 512), 512)
            ya = jnp.dot(y1_s[rows, :].astype(BF), g2[...], preferred_element_type=F32)
            o_s[rows, 0:DA] = ya.astype(BF)
            return carry
        lax.fori_loop(0, S // 512, step7, 0)
        cp_outa.start()

        cp_wot0.wait()
        cp_ckv1.wait()
        for w in wlist:
            for cp in wcopies(*w, 1):
                cp.start()
        cp_wot1.start()

    @pl.when(h == 1)
    def _():
        for w in wlist:
            for cp in wcopies(*w, 1):
                cp.wait()
        cp_wot1.wait()
        cp_outa.wait()
        for w in wlist:
            for cp in wcopies(*w, 2):
                cp.start()

    @pl.when(h == 6)
    def _():
        for w in wlist:
            for cp in wcopies(*w, 2):
                cp.wait()

    ps = {0: (p0_s[0:HT, :], p0_s[HT:TQ, HT:TQ], inv0_s[0:1, :])}
    ots = {-1: ot7_s[...]}
    for t in range(NB):
        pa, pb, inv = ps.pop(t)
        if t + 1 < NB:
            sa = qk_main(t + 1, dep if (PREP_FENCE and t + 1 == NB - 1) else None)
        if t + 2 < NB:
            proj_qk(t + 2)
            proj_v(t + 2)
            if t + 2 == NB - 1:
                dep = prep_weights(jnp.minimum(h + 1, H - 1))
        else:
            proj_qk(t + 2 - NB)
        if t + 1 < NB:
            ps[t + 1] = softmax(t + 1, sa, qk_diag(t + 1))
        else:
            save_first_block()
        ob = pv_diag(t, pb)
        ots[t] = pv(t, pa, ob, inv)
        if t == 0:
            outproj(NB - 1, ots.pop(-1), jnp.maximum(h - 1, 0))
        else:
            outproj(t - 1, ots.pop(t - 1), h)
    proj_v(0)
    proj_v(1)
    ot7_s[...] = ots.pop(NB - 1)

    @pl.when(h == H - 1)
    def _epilogue():
        outproj(NB - 1, ot7_s[...], H - 1)
        OB = 256
        lane = lax.broadcasted_iota(jnp.int32, (OB, 128), 1)
        outs = []
        for i in range(S // OB):
            rows = slice(i * OB, (i + 1) * OB)
            bt = acc_s[:, rows].T.astype(BF)
            first = jnp.where(lane < 64, o_s[rows, 384:512], bt[:, 0:128])
            o_s[rows, 384:512] = first
            o_s[rows, 512:896] = bt[:, 128:512]
            cp = pltpu.make_async_copy(o_s.at[rows, 384:896], out_hbm.at[rows, 384:896], osem.at[i])
            cp.start()
            outs.append(cp)
        for cp in outs:
            cp.wait()


@jax.jit
def pallas_concat_heads__spectral_gfnet__compressed_kv_cla__prompt_kernel(
    A_x, A_w_r, A_w_i, B_x, B_c_kv, B_w_q, B_w_uk, B_w_uv, B_w_o,
):
    g1, m2, g2, perm = _tables()
    axt = jnp.swapaxes(A_x, 1, 2).reshape(DA, S)
    bxt = jnp.swapaxes(B_x, 1, 2).reshape(DA, S)
    wrt = A_w_r.T
    wit = A_w_i.T
    ckv = B_c_kv.reshape(S, C)
    wq = B_w_q.reshape(DA // 2, 2, H, D)
    wuk = B_w_uk.reshape(C // 2, 2, H, D)
    wuv = B_w_uv.reshape(C // 2, 2, H, D)
    wot = jnp.swapaxes(B_w_o, 1, 2)

    any_spec = pl.BlockSpec(memory_space=pl.ANY)
    V = pltpu.VMEM
    out = pl.pallas_call(
        _kernel,
        grid=(H,),
        in_specs=[any_spec] * 13,
        out_specs=any_spec,
        out_shape=jax.ShapeDtypeStruct((S, 2 * DA), BF),
        scratch_shapes=[
            V((DA, S), BF), V((DF, S), BF), V((DF, S), BF), V((512, S), BF), V((S, C), BF),
            V((2, 2, DA // 2, 8, 128), jnp.uint32),
            V((2, 2, C // 2, 8, 128), jnp.uint32),
            V((2, 2, C // 2, 8, 128), jnp.uint32),
            V((H, DA, D), BF),
            V((2 * FP, DA), BF), V((N1, 256, 128), BF), V((512, DA), BF),
            V((128, 128), BF),
            V((2 * FP, S), F32), V((N1, 256, 256), F32), V((N1, 128, 256), F32),
            V((N1, 128, 256), F32), V((N1, 128, 512), F32), V((S, 512), F32),
            V((D, 512), BF), V((C, D), BF), V((D, C), BF),
            V((D, S), BF), V((S, D), BF), V((D, S), BF), V((512, S), F32), V((S, 2 * DA), BF),
            V((TQ, TQ), BF), V((8, TQ), F32), V((D, TQ), BF),
            pltpu.SemaphoreType.DMA((12,)),
            pltpu.SemaphoreType.DMA((3, 3, 4)),
            pltpu.SemaphoreType.DMA((8,)),
            pltpu.SemaphoreType.DMA((4,)),
        ],
        compiler_params=pltpu.CompilerParams(
            dimension_semantics=("arbitrary",),
            vmem_limit_bytes=120 * 2**20),
    )(axt, wrt, wit, bxt, ckv, wq, wuk, wuv, wot, g1, m2, g2, perm)
    return out.reshape(1, S, 2 * DA)
```

```python
import numpy as np
import jax
import jax.numpy as jnp
from jax import lax
import jax.experimental.pallas as pl
import jax.experimental.pallas.tpu as pltpu

S = 2048
DA = 448
DF = DA // 2 + 1
FP = 240
H = 16
D = 256
C = 1024
N1 = 16
N2 = 128
TQ = 256
HT = 128
QC = 256
QK_LAG = 2
PREP_FENCE = 1
LOG2E = 1.4426950408889634
MASK_VAL = -1e9 * LOG2E
BF = jnp.bfloat16
F32 = jnp.float32
NT = (((1,), (1,)), ((), ()))
TN = (((0,), (0,)), ((), ()))


def _tables():
    f = np.arange(FP)[:, None].astype(np.float64)
    d = np.arange(DA)[None, :].astype(np.float64)
    valid = (np.arange(FP) < DF)[:, None]
    ang = 2 * np.pi * ((f * d) % DA) / DA
    g1 = np.concatenate([np.cos(ang) * valid, -np.sin(ang) * valid], axis=0)
    k2 = np.arange(N2)[:, None]
    s2 = np.arange(N2)[None, :]
    m2 = np.zeros((N1, 2 * N2, N2))
    for k1 in range(N1):
        a = 2 * np.pi * ((s2 * (k1 + N1 * k2)) % S) / S
        m2[k1] = np.concatenate([np.cos(a), -np.sin(a)], axis=0)
    f2 = np.arange(256)[:, None].astype(np.float64)
    cf = np.where((f2 == 0) | (f2 == DA // 2), 1.0, 2.0) * (f2 < DF) / (S * DA)
    ang2 = 2 * np.pi * ((f2 * d) % DA) / DA
    g2 = np.concatenate([np.cos(ang2) * cf, -np.sin(ang2) * cf], axis=0)
    perm = np.zeros((128, 128))
    for k1 in range(N1):
        for j in range(8):
            perm[8 * k1 + j, k1 + 16 * j] = 1.0
    cast = lambda a: jnp.asarray(a.astype(np.float32), dtype=BF)
    return cast(g1), cast(m2), cast(g2), cast(perm)


def _fft4(xs, sign):
    (ar, ai), (br, bi), (cr, ci), (dr, di) = xs
    s0r, s0i = ar + cr, ai + ci
    s1r, s1i = ar - cr, ai - ci
    s2r, s2i = br + dr, bi + di
    s3r, s3i = br - dr, bi - di
    y0 = (s0r + s2r, s0i + s2i)
    y2 = (s0r - s2r, s0i - s2i)
    if sign < 0:
        y1 = (s1r + s3i, s1i - s3r)
        y3 = (s1r - s3i, s1i + s3r)
    else:
        y1 = (s1r - s3i, s1i + s3r)
        y3 = (s1r + s3i, s1i - s3r)
    return [y0, y1, y2, y3]


def _twiddle(z, e, sign):
    zr, zi = z
    e = e % 16
    if e == 0:
        return z
    if (e * sign) % 16 == 12:
        return (zi, -zr)
    if (e * sign) % 16 == 4:
        return (-zi, zr)
    c = float(np.cos(2 * np.pi * e / 16))
    s = float(sign * np.sin(2 * np.pi * e / 16))
    if abs(abs(c) - abs(s)) < 1e-12:
        r = abs(c)
        u = zr - zi if (c > 0) == (s > 0) else zr + zi
        v = zi + zr if (c > 0) == (s > 0) else zi - zr
        return (u * c, v * c)
    return (zr * c - zi * s, zi * c + zr * s)


def _fft16(xs, sign):
    t = [None] * 16
    for b in range(4):
        col = _fft4([xs[4 * a + b] for a in range(4)], sign)
        for c in range(4):
            t[4 * c + b] = _twiddle(col[c], b * c, sign)
    out = [None] * 16
    for c in range(4):
        col = _fft4([t[4 * c + b] for b in range(4)], sign)
        for e in range(4):
            out[c + 4 * e] = col[e]
    return out


def _kernel(axt_hbm, wrt_hbm, wit_hbm, bxt_hbm, ckv_hbm, wq_hbm, wuk_hbm, wuv_hbm, wot_hbm,
            g1_hbm, m2_hbm, g2_hbm, perm_hbm,
            out_hbm,
            axt, wrt, wit, bxt, ckv, wq_w, wuk_w, wuv_w, wot, g1, m2, g2, perm,
            x1_s, a_s, wr_s, wi_s, b_s, y1_s,
            wqt_s, wk_s, wvt_s, qt_s, k_s, vt_s, acc_s, o_s, p0_s, inv0_s, ot7_s,
            sem, wsem, osem, asem):
    h = pl.program_id(0)

    CK0 = 2 * TQ
    simple = [(g1_hbm, g1), (wrt_hbm, wrt), (wit_hbm, wit), (perm_hbm, perm),
              (m2_hbm, m2), (g2_hbm, g2), (bxt_hbm, bxt.at[0:DA]),
              (ckv_hbm.at[0:CK0], ckv.at[0:CK0]), (ckv_hbm.at[CK0:S], ckv.at[CK0:S]),
              (wot_hbm.at[0:1], wot.at[0:1]), (wot_hbm.at[1:H], wot.at[1:H]),
              (o_s.at[:, 0:384], out_hbm.at[:, 0:384])]
    cps = [pltpu.make_async_copy(s, d, sem.at[i]) for i, (s, d) in enumerate(simple)]
    (cp_g1, cp_wrt, cp_wit, cp_perm, cp_m2, cp_g2, cp_bxt, cp_ckv0, cp_ckv1,
     cp_wot0, cp_wot1, cp_outa) = cps

    def axt_copy(c):
        cols = pl.ds(pl.multiple_of(c * 512, 512), 512)
        return pltpu.make_async_copy(axt_hbm.at[:, cols], axt.at[:, cols], asem.at[c])

    def wcopies(widx, w_hbm, w_buf, stage):
        src = w_hbm.bitcast(jnp.uint32)
        g, j0, n = ((0, 0, 1), (0, 1, 3), (1, 0, 4))[stage]
        return [pltpu.make_async_copy(
            src.at[:, p, pl.ds(4 * g + j0, n), pl.ds(128 * t, 128)],
            w_buf.at[g, t, :, pl.ds(4 * p + j0, n), :],
            wsem.at[widx, stage, 2 * t + p]) for t in range(2) for p in range(2)]

    wlist = [(0, wq_hbm, wq_w), (1, wuk_hbm, wuk_w), (2, wuv_hbm, wuv_w)]

    def head_weight(w_buf, rows, hh):
        g = lax.shift_right_logical(hh, 3)
        j = lax.shift_right_logical(hh, 1) & 3
        sh = ((hh & 1) * 16).astype(jnp.uint32)
        halves = []
        for t in range(2):
            w2 = w_buf.at[g, t].reshape(rows * 4, 128)
            a = w2[pl.ds(j, rows, stride=4), :]
            halves.append(pltpu.bitcast((a >> sh) << 16, F32))
        return jnp.concatenate(halves, axis=1)

    def orall(x):
        w = pltpu.bitcast(x, jnp.uint32)
        acc = None
        for r in range(0, w.shape[0], 8):
            for c in range(0, w.shape[1], 128):
                t = w[r:r + 8, c:min(c + 128, w.shape[1])]
                if t.shape[1] < 128:
                    continue
                acc = t if acc is None else acc | t
        return acc

    def prep_weights(hh):
        a = head_weight(wq_w, DA, hh).T.astype(BF)
        b = head_weight(wuk_w, C, hh).astype(BF)
        c = head_weight(wuv_w, C, hh).T.astype(BF)
        wqt_s[:, 0:DA] = a
        wk_s[...] = b
        wvt_s[...] = c
        deps = [orall(a)]
        if PREP_FENCE >= 2:
            deps.append(orall(b))
        if PREP_FENCE >= 3:
            deps.append(orall(c))
        d = deps[0]
        for e in deps[1:]:
            d = d | e
        return pltpu.bitcast(d, F32)

    NB = S // TQ
    key = lax.broadcasted_iota(jnp.int32, (HT, HT), 0)
    qry = lax.broadcasted_iota(jnp.int32, (HT, HT), 1)
    causal = key <= qry

    def proj_qk(i):
        cs = slice(i * TQ, (i + 1) * TQ)
        qt = jnp.dot(wqt_s[...], bxt[:, cs], preferred_element_type=F32) * (D ** -0.5 * LOG2E)
        qt_s[:, cs] = qt.astype(BF)
        k_s[cs, :] = jnp.dot(ckv[cs, :], wk_s[...], preferred_element_type=F32).astype(BF)

    def proj_v(i):
        cs = slice(i * TQ, (i + 1) * TQ)
        vt_s[:, cs] = lax.dot_general(wvt_s[...], ckv[cs, :], NT,
                                      preferred_element_type=F32).astype(BF)

    def colreduce(x, op, nacc=2):
        accs = [x[8 * a:8 * a + 8] for a in range(nacc)]
        for r in range(8 * nacc, x.shape[0], 8 * nacc):
            for a in range(nacc):
                accs[a] = op(accs[a], x[r + 8 * a:r + 8 * a + 8])
        while len(accs) > 1:
            accs = [op(accs[2 * a], accs[2 * a + 1]) for a in range(len(accs) // 2)]
        return accs[0]

    def fence(x, dep):
        never = (dep - dep) < -1.0
        head = pltpu.bitcast(x[0:16, 0:128], jnp.uint32)
        head = pltpu.bitcast(jnp.where(never, jnp.uint32(0), head), BF)
        top = jnp.concatenate([head, x[0:16, 128:]], axis=1)
        return jnp.concatenate([top, x[16:]], axis=0)

    def qk_main(i, dep=None):
        L = (i + 1) * TQ
        qt = qt_s[:, i * TQ:(i + 1) * TQ]
        if dep is not None:
            qt = fence(qt, dep)
        bounds = list(range(0, L - HT, QC)) + [L - HT]
        sts, ms = [], []
        for c in range(len(bounds) - 1):
            kc = k_s[bounds[c]:bounds[c + 1], :]
            if c >= QK_LAG:
                kc = fence(kc, ms[c - QK_LAG][:, 0:HT] + ms[c - QK_LAG][:, HT:])
            st = jnp.dot(kc, qt, preferred_element_type=F32)
            if c == len(bounds) - 2:
                n = st.shape[0]
                dg = jnp.concatenate([jnp.where(causal, st[n - HT:, :HT], MASK_VAL), st[n - HT:, HT:]], axis=1)
                st = jnp.concatenate([st[:n - HT], dg], axis=0) if n > HT else dg
            mc = colreduce(st, jnp.maximum)
            ms.append(mc if c == 0 else jnp.maximum(ms[-1], mc))
            sts.append(st)
        return jnp.concatenate(sts, axis=0), ms[-1]

    def qk_diag(i):
        L = (i + 1) * TQ
        return jnp.dot(k_s[L - HT:L, :], qt_s[:, L - HT:L], preferred_element_type=F32)

    def softmax(i, sa_m8, sb):
        sa, m8 = sa_m8
        L = (i + 1) * TQ
        sb = jnp.where(causal, sb, MASK_VAL)
        ml = jnp.max(m8[:, :HT], axis=0, keepdims=True)
        mr = jnp.max(jnp.maximum(m8[:, HT:], colreduce(sb, jnp.maximum)), axis=0, keepdims=True)
        pa = jnp.exp2(sa - jnp.concatenate([ml, mr], axis=1))
        pb = jnp.exp2(sb - mr)
        l8 = colreduce(pa, jnp.add)
        ll = jnp.sum(l8[:, :HT], axis=0, keepdims=True)
        lr = jnp.sum(l8[:, HT:] + colreduce(pb, jnp.add), axis=0, keepdims=True)
        return pa.astype(BF), pb.astype(BF), 1.0 / jnp.concatenate([ll, lr], axis=1)

    def pv_diag(i, pb):
        L = (i + 1) * TQ
        top = jnp.dot(vt_s[0:HT, L - HT:L], pb, preferred_element_type=F32)
        bot = jnp.dot(vt_s[HT:D, L - HT:L], pb, preferred_element_type=F32)
        return jnp.concatenate([top, bot], axis=0)

    def pv(i, pa, ob, inv):
        L = (i + 1) * TQ
        oa = jnp.dot(vt_s[:, 0:L - HT], pa, preferred_element_type=F32)
        ot = jnp.concatenate([oa[:, :HT], oa[:, HT:] + ob], axis=1)
        return (ot * inv).astype(BF)

    def outproj(i, ot, hh):
        acc_s[64:512, i * TQ:(i + 1) * TQ] += jnp.dot(wot[hh], ot, preferred_element_type=F32)

    def save_first_block():
        pa, pb, inv = softmax(0, qk_main(0), qk_diag(0))
        p0_s[0:HT, :] = pa
        p0_s[HT:TQ, HT:TQ] = pb
        inv0_s[...] = jnp.broadcast_to(inv, (8, TQ))

    @pl.when(h == 0)
    def _prologue():
        cp_g1.start()
        for c in range(S // 512):
            axt_copy(c).start()
        for cp in (cp_wrt, cp_wit, cp_perm, cp_m2, cp_bxt):
            cp.start(priority=1)
        for cp in wcopies(*wlist[0], 0):
            cp.start(priority=1)
        cp_ckv0.start(priority=1)
        for cp in wcopies(*wlist[1], 0) + wcopies(*wlist[2], 0):
            cp.start(priority=1)
        cp_g2.start(priority=1)
        cp_wot0.start(priority=1)
        cp_ckv1.start(priority=1)

        acc_s[...] = jnp.zeros_like(acc_s)
        bxt[DA:512, :] = jnp.zeros((512 - DA, S), BF)
        wqt_s[...] = jnp.zeros_like(wqt_s)

        cp_g1.wait()

        def step1(c, carry):
            axt_copy(c).wait()
            cols = pl.ds(pl.multiple_of(c * 512, 512), 512)
            x1_s[:, cols] = jnp.dot(g1[...], axt[:, cols], preferred_element_type=F32)
            return carry
        lax.fori_loop(0, S // 512, step1, 0)

        cp_wrt.wait()
        cp_wit.wait()
        cp_perm.wait()
        zpad = jnp.zeros((128, 256 - DF), F32)
        for a in range(N1):
            for (src, dst) in ((wrt, wr_s), (wit, wi_s)):
                t = lax.dot_general(perm[...], src[:, 128 * a:128 * (a + 1)], NT,
                                    preferred_element_type=F32)
                t = jnp.concatenate([t, zpad], axis=1)
                for k1 in range(N1):
                    dst[k1, 8 * a:8 * (a + 1), :] = t[8 * k1:8 * (k1 + 1), :]

        for r in range(0, FP, 8):
            xs = [(x1_s[r:r + 8, 128 * s1:128 * (s1 + 1)],
                   x1_s[FP + r:FP + r + 8, 128 * s1:128 * (s1 + 1)]) for s1 in range(N1)]
            ys = _fft16(xs, -1)
            for k1 in range(N1):
                a_s[k1, r:r + 8, 0:128] = ys[k1][0]
                a_s[k1, r:r + 8, 128:256] = ys[k1][1]
        a_s[:, FP:256, :] = jnp.zeros((N1, 256 - FP, 256), F32)

        cp_m2.wait()

        def mid_fwd(k1):
            mk = m2[k1]
            u = lax.dot_general(mk, a_s[k1, :, 0:128].astype(BF), NT, preferred_element_type=F32)
            v = lax.dot_general(mk, a_s[k1, :, 128:256].astype(BF), NT, preferred_element_type=F32)
            zr = u[0:128] - v[128:256]
            zi = u[128:256] + v[0:128]
            wr, wi = wr_s[k1], wi_s[k1]
            yr = (zr * wr - zi * wi).astype(BF)
            yi = (zr * wi + zi * wr).astype(BF)
            return jnp.concatenate([jnp.concatenate([yr, yi], axis=1),
                                    jnp.concatenate([yi, -yr], axis=1)], axis=0)

        rhs = {0: mid_fwd(0)}
        for k1 in range(N1):
            if k1 + 1 < N1:
                rhs[k1 + 1] = mid_fwd(k1 + 1)
            b_s[k1] = lax.dot_general(m2[k1], rhs.pop(k1), TN, preferred_element_type=F32)

        cp_bxt.wait()
        cp_ckv0.wait()
        for w in wlist:
            for cp in wcopies(*w, 0):
                cp.wait()
        prep_weights(h)
        proj_qk(0)
        proj_qk(1)
        proj_v(0)
        proj_v(1)
        save_first_block()
        ot7_s[...] = jnp.zeros_like(ot7_s)

        for g in range(N2 // 8):
            for t in range(2):
                xs = [(b_s[k1, 8 * g:8 * g + 8, 128 * t:128 * (t + 1)],
                       b_s[k1, 8 * g:8 * g + 8, 256 + 128 * t:256 + 128 * (t + 1)]) for k1 in range(N1)]
                ys = _fft16(xs, +1)
                for s1 in range(N1):
                    r0 = 128 * s1 + 8 * g
                    y1_s[r0:r0 + 8, 128 * t:128 * (t + 1)] = ys[s1][0]
                    y1_s[r0:r0 + 8, 256 + 128 * t:256 + 128 * (t + 1)] = ys[s1][1]
        cp_g2.wait()

        def step7(c, carry):
            rows = pl.ds(pl.multiple_of(c * 512, 512), 512)
            ya = jnp.dot(y1_s[rows, :].astype(BF), g2[...], preferred_element_type=F32)
            o_s[rows, 0:DA] = ya.astype(BF)
            return carry
        lax.fori_loop(0, S // 512, step7, 0)
        cp_outa.start()

        cp_wot0.wait()
        cp_ckv1.wait()
        for w in wlist:
            for cp in wcopies(*w, 1):
                cp.start()
        cp_wot1.start()

    def at_head(hh, fn):
        def body(i, carry):
            fn()
            return carry
        lax.fori_loop(0, (h == hh).astype(jnp.int32), body, 0)

    def _stage1():
        for w in wlist:
            for cp in wcopies(*w, 1):
                cp.wait()
        cp_wot1.wait()
        cp_outa.wait()
        for w in wlist:
            for cp in wcopies(*w, 2):
                cp.start()

    def _stage2():
        for w in wlist:
            for cp in wcopies(*w, 2):
                cp.wait()

    at_head(1, _stage1)
    at_head(6, _stage2)

    ps = {0: (p0_s[0:HT, :], p0_s[HT:TQ, HT:TQ], inv0_s[0:1, :])}
    ots = {-1: ot7_s[...]}
    for t in range(NB):
        pa, pb, inv = ps.pop(t)
        if t + 1 < NB:
            sa = qk_main(t + 1, dep if (PREP_FENCE and t + 1 == NB - 1) else None)
        if t + 2 < NB:
            proj_qk(t + 2)
            proj_v(t + 2)
            if t + 2 == NB - 1:
                dep = prep_weights(jnp.minimum(h + 1, H - 1))
        else:
            proj_qk(t + 2 - NB)
        if t + 1 < NB:
            ps[t + 1] = softmax(t + 1, sa, qk_diag(t + 1))
        else:
            save_first_block()
        ob = pv_diag(t, pb)
        ots[t] = pv(t, pa, ob, inv)
        if t == 0:
            outproj(NB - 1, ots.pop(-1), jnp.maximum(h - 1, 0))
        else:
            outproj(t - 1, ots.pop(t - 1), h)
    proj_v(0)
    proj_v(1)
    ot7_s[...] = ots.pop(NB - 1)

    @pl.when(h == H - 1)
    def _epilogue():
        outproj(NB - 1, ot7_s[...], H - 1)
        OB = 256
        lane = lax.broadcasted_iota(jnp.int32, (OB, 128), 1)
        outs = []
        for i in range(S // OB):
            rows = slice(i * OB, (i + 1) * OB)
            bt = acc_s[:, rows].T.astype(BF)
            first = jnp.where(lane < 64, o_s[rows, 384:512], bt[:, 0:128])
            o_s[rows, 384:512] = first
            o_s[rows, 512:896] = bt[:, 128:512]
            cp = pltpu.make_async_copy(o_s.at[rows, 384:896], out_hbm.at[rows, 384:896], osem.at[i])
            cp.start()
            outs.append(cp)
        for cp in outs:
            cp.wait()


@jax.jit
def pallas_concat_heads__spectral_gfnet__compressed_kv_cla__prompt_kernel(
    A_x, A_w_r, A_w_i, B_x, B_c_kv, B_w_q, B_w_uk, B_w_uv, B_w_o,
):
    g1, m2, g2, perm = _tables()
    axt = jnp.swapaxes(A_x, 1, 2).reshape(DA, S)
    bxt = jnp.swapaxes(B_x, 1, 2).reshape(DA, S)
    wrt = A_w_r.T
    wit = A_w_i.T
    ckv = B_c_kv.reshape(S, C)
    wq = B_w_q.reshape(DA // 2, 2, H, D)
    wuk = B_w_uk.reshape(C // 2, 2, H, D)
    wuv = B_w_uv.reshape(C // 2, 2, H, D)
    wot = jnp.swapaxes(B_w_o, 1, 2)

    any_spec = pl.BlockSpec(memory_space=pl.ANY)
    V = pltpu.VMEM
    out = pl.pallas_call(
        _kernel,
        grid=(H,),
        in_specs=[any_spec] * 13,
        out_specs=any_spec,
        out_shape=jax.ShapeDtypeStruct((S, 2 * DA), BF),
        scratch_shapes=[
            V((DA, S), BF), V((DF, S), BF), V((DF, S), BF), V((512, S), BF), V((S, C), BF),
            V((2, 2, DA // 2, 8, 128), jnp.uint32),
            V((2, 2, C // 2, 8, 128), jnp.uint32),
            V((2, 2, C // 2, 8, 128), jnp.uint32),
            V((H, DA, D), BF),
            V((2 * FP, DA), BF), V((N1, 256, 128), BF), V((512, DA), BF),
            V((128, 128), BF),
            V((2 * FP, S), F32), V((N1, 256, 256), F32), V((N1, 128, 256), F32),
            V((N1, 128, 256), F32), V((N1, 128, 512), F32), V((S, 512), F32),
            V((D, 512), BF), V((C, D), BF), V((D, C), BF),
            V((D, S), BF), V((S, D), BF), V((D, S), BF), V((512, S), F32), V((S, 2 * DA), BF),
            V((TQ, TQ), BF), V((8, TQ), F32), V((D, TQ), BF),
            pltpu.SemaphoreType.DMA((12,)),
            pltpu.SemaphoreType.DMA((3, 3, 4)),
            pltpu.SemaphoreType.DMA((8,)),
            pltpu.SemaphoreType.DMA((4,)),
        ],
        compiler_params=pltpu.CompilerParams(
            dimension_semantics=("arbitrary",),
            vmem_limit_bytes=120 * 2**20),
    )(axt, wrt, wit, bxt, ckv, wq, wuk, wuv, wot, g1, m2, g2, perm)
    return out.reshape(1, S, 2 * DA)
```

```python
import numpy as np
import jax
import jax.numpy as jnp
from jax import lax
import jax.experimental.pallas as pl
import jax.experimental.pallas.tpu as pltpu

S = 2048
DA = 448
DF = DA // 2 + 1
FP = 240
H = 16
D = 256
C = 1024
N1 = 16
N2 = 128
TQ = 256
HT = 128
QC = 256
QK_LAG = 2
PREP_FENCE = 1
LOG2E = 1.4426950408889634
MASK_VAL = -1e9 * LOG2E
BF = jnp.bfloat16
F32 = jnp.float32
NT = (((1,), (1,)), ((), ()))
TN = (((0,), (0,)), ((), ()))


def _tables():
    f = np.arange(FP)[:, None].astype(np.float64)
    d = np.arange(DA)[None, :].astype(np.float64)
    valid = (np.arange(FP) < DF)[:, None]
    ang = 2 * np.pi * ((f * d) % DA) / DA
    g1 = np.concatenate([np.cos(ang) * valid, -np.sin(ang) * valid], axis=0)
    k2 = np.arange(N2)[:, None]
    s2 = np.arange(N2)[None, :]
    m2 = np.zeros((N1, 2 * N2, N2))
    for k1 in range(N1):
        a = 2 * np.pi * ((s2 * (k1 + N1 * k2)) % S) / S
        m2[k1] = np.concatenate([np.cos(a), -np.sin(a)], axis=0)
    f2 = np.arange(256)[:, None].astype(np.float64)
    cf = np.where((f2 == 0) | (f2 == DA // 2), 1.0, 2.0) * (f2 < DF) / (S * DA)
    ang2 = 2 * np.pi * ((f2 * d) % DA) / DA
    g2 = np.concatenate([np.cos(ang2) * cf, -np.sin(ang2) * cf], axis=0)
    perm = np.zeros((128, 128))
    for k1 in range(N1):
        for j in range(8):
            perm[8 * k1 + j, k1 + 16 * j] = 1.0
    cast = lambda a: jnp.asarray(a.astype(np.float32), dtype=BF)
    return cast(g1), cast(m2), cast(g2), cast(perm)


def _fft4(xs, sign):
    (ar, ai), (br, bi), (cr, ci), (dr, di) = xs
    s0r, s0i = ar + cr, ai + ci
    s1r, s1i = ar - cr, ai - ci
    s2r, s2i = br + dr, bi + di
    s3r, s3i = br - dr, bi - di
    y0 = (s0r + s2r, s0i + s2i)
    y2 = (s0r - s2r, s0i - s2i)
    if sign < 0:
        y1 = (s1r + s3i, s1i - s3r)
        y3 = (s1r - s3i, s1i + s3r)
    else:
        y1 = (s1r - s3i, s1i + s3r)
        y3 = (s1r + s3i, s1i - s3r)
    return [y0, y1, y2, y3]


def _twiddle(z, e, sign):
    zr, zi = z
    e = e % 16
    if e == 0:
        return z
    if (e * sign) % 16 == 12:
        return (zi, -zr)
    if (e * sign) % 16 == 4:
        return (-zi, zr)
    c = float(np.cos(2 * np.pi * e / 16))
    s = float(sign * np.sin(2 * np.pi * e / 16))
    if abs(abs(c) - abs(s)) < 1e-12:
        r = abs(c)
        u = zr - zi if (c > 0) == (s > 0) else zr + zi
        v = zi + zr if (c > 0) == (s > 0) else zi - zr
        return (u * c, v * c)
    return (zr * c - zi * s, zi * c + zr * s)


def _fft16(xs, sign):
    t = [None] * 16
    for b in range(4):
        col = _fft4([xs[4 * a + b] for a in range(4)], sign)
        for c in range(4):
            t[4 * c + b] = _twiddle(col[c], b * c, sign)
    out = [None] * 16
    for c in range(4):
        col = _fft4([t[4 * c + b] for b in range(4)], sign)
        for e in range(4):
            out[c + 4 * e] = col[e]
    return out


def _kernel(axt_hbm, wrt_hbm, wit_hbm, bxt_hbm, ckv_hbm, wq_hbm, wuk_hbm, wuv_hbm, wot_hbm,
            g1_hbm, m2_hbm, g2_hbm, perm_hbm,
            out_hbm,
            axt, wrt, wit, bxt, ckv, wq_w, wuk_w, wuv_w, wot, g1, m2, g2, perm,
            x1_s, a_s, wr_s, wi_s, b_s, y1_s,
            wqt_s, wk_s, wvt_s, qt_s, k_s, vt_s, acc_s, o_s, p0_s, inv0_s, ot7_s,
            sem, wsem, osem, asem):
    h = pl.program_id(0)

    CK0 = 2 * TQ
    simple = [(g1_hbm, g1), (wrt_hbm, wrt), (wit_hbm, wit), (perm_hbm, perm),
              (m2_hbm, m2), (g2_hbm, g2), (bxt_hbm, bxt.at[0:DA]),
              (ckv_hbm.at[0:CK0], ckv.at[0:CK0]), (ckv_hbm.at[CK0:S], ckv.at[CK0:S]),
              (wot_hbm.at[0:1], wot.at[0:1]), (wot_hbm.at[1:H], wot.at[1:H]),
              (o_s.at[:, 0:384], out_hbm.at[:, 0:384])]
    cps = [pltpu.make_async_copy(s, d, sem.at[i]) for i, (s, d) in enumerate(simple)]
    (cp_g1, cp_wrt, cp_wit, cp_perm, cp_m2, cp_g2, cp_bxt, cp_ckv0, cp_ckv1,
     cp_wot0, cp_wot1, cp_outa) = cps

    def axt_copy(c):
        cols = pl.ds(pl.multiple_of(c * 512, 512), 512)
        return pltpu.make_async_copy(axt_hbm.at[:, cols], axt.at[:, cols], asem.at[c])

    def wcopies(widx, w_hbm, w_buf, stage):
        src = w_hbm.bitcast(jnp.uint32)
        g, j0, n = ((0, 0, 1), (0, 1, 3), (1, 0, 4))[stage]
        return [pltpu.make_async_copy(
            src.at[:, p, pl.ds(4 * g + j0, n), pl.ds(128 * t, 128)],
            w_buf.at[g, t, :, pl.ds(4 * p + j0, n), :],
            wsem.at[widx, stage, 2 * t + p]) for t in range(2) for p in range(2)]

    wlist = [(0, wq_hbm, wq_w), (1, wuk_hbm, wuk_w), (2, wuv_hbm, wuv_w)]

    def head_weight(w_buf, rows, hh):
        g = lax.shift_right_logical(hh, 3)
        j = lax.shift_right_logical(hh, 1) & 3
        sh = ((hh & 1) * 16).astype(jnp.uint32)
        halves = []
        for t in range(2):
            w2 = w_buf.at[g, t].reshape(rows * 4, 128)
            a = w2[pl.ds(j, rows, stride=4), :]
            halves.append(pltpu.bitcast((a >> sh) << 16, F32))
        return jnp.concatenate(halves, axis=1)

    def orall(x):
        w = pltpu.bitcast(x, jnp.uint32)
        acc = None
        for r in range(0, w.shape[0], 8):
            for c in range(0, w.shape[1], 128):
                t = w[r:r + 8, c:min(c + 128, w.shape[1])]
                if t.shape[1] < 128:
                    continue
                acc = t if acc is None else acc | t
        return acc

    def prep_weights(hh):
        a = head_weight(wq_w, DA, hh).T.astype(BF)
        b = head_weight(wuk_w, C, hh).astype(BF)
        c = head_weight(wuv_w, C, hh).T.astype(BF)
        wqt_s[:, 0:DA] = a
        wk_s[...] = b
        wvt_s[...] = c
        deps = [orall(a)]
        if PREP_FENCE >= 2:
            deps.append(orall(b))
        if PREP_FENCE >= 3:
            deps.append(orall(c))
        d = deps[0]
        for e in deps[1:]:
            d = d | e
        return pltpu.bitcast(d, F32)

    NB = S // TQ
    key = lax.broadcasted_iota(jnp.int32, (HT, HT), 0)
    qry = lax.broadcasted_iota(jnp.int32, (HT, HT), 1)
    causal = key <= qry

    def proj_q(i):
        cs = slice(i * TQ, (i + 1) * TQ)
        qt = jnp.dot(wqt_s[...], bxt[:, cs], preferred_element_type=F32) * (D ** -0.5 * LOG2E)
        qt_s[:, cs] = qt.astype(BF)

    def proj_k(i):
        cs = slice(i * TQ, (i + 1) * TQ)
        k_s[cs, :] = jnp.dot(ckv[cs, :], wk_s[...], preferred_element_type=F32).astype(BF)

    def proj_v(i):
        cs = slice(i * TQ, (i + 1) * TQ)
        vt_s[:, cs] = lax.dot_general(wvt_s[...], ckv[cs, :], NT,
                                      preferred_element_type=F32).astype(BF)

    def colreduce(x, op, nacc=4):
        accs = [x[8 * a:8 * a + 8] for a in range(nacc)]
        for r in range(8 * nacc, x.shape[0], 8 * nacc):
            for a in range(nacc):
                accs[a] = op(accs[a], x[r + 8 * a:r + 8 * a + 8])
        while len(accs) > 1:
            accs = [op(accs[2 * a], accs[2 * a + 1]) for a in range(len(accs) // 2)]
        return accs[0]

    def fence(x, dep):
        never = (dep - dep) < -1.0
        head = pltpu.bitcast(x[0:16, 0:128], jnp.uint32)
        head = pltpu.bitcast(jnp.where(never, jnp.uint32(0), head), BF)
        top = jnp.concatenate([head, x[0:16, 128:]], axis=1)
        return jnp.concatenate([top, x[16:]], axis=0)

    def qk_main(i, dep=None):
        L = (i + 1) * TQ
        qt = qt_s[:, i * TQ:(i + 1) * TQ]
        if dep is not None:
            qt = fence(qt, dep)
        bounds = list(range(0, L - HT, QC)) + [L - HT]
        sts, ms = [], []
        for c in range(len(bounds) - 1):
            kc = k_s[bounds[c]:bounds[c + 1], :]
            if c >= QK_LAG:
                kc = fence(kc, ms[c - QK_LAG][:, 0:HT] + ms[c - QK_LAG][:, HT:])
            st = jnp.dot(kc, qt, preferred_element_type=F32)
            if c == len(bounds) - 2:
                n = st.shape[0]
                dg = jnp.concatenate([jnp.where(causal, st[n - HT:, :HT], MASK_VAL), st[n - HT:, HT:]], axis=1)
                st = jnp.concatenate([st[:n - HT], dg], axis=0) if n > HT else dg
            mc = colreduce(st, jnp.maximum)
            ms.append(mc if c == 0 else jnp.maximum(ms[-1], mc))
            sts.append(st)
        return jnp.concatenate(sts, axis=0), ms[-1]

    def qk_diag(i):
        L = (i + 1) * TQ
        return jnp.dot(k_s[L - HT:L, :], qt_s[:, L - HT:L], preferred_element_type=F32)

    def softmax(i, sa_m8, sb):
        sa, m8 = sa_m8
        L = (i + 1) * TQ
        sb = jnp.where(causal, sb, MASK_VAL)
        ml = jnp.max(m8[:, :HT], axis=0, keepdims=True)
        mr = jnp.max(jnp.maximum(m8[:, HT:], colreduce(sb, jnp.maximum)), axis=0, keepdims=True)
        pa = jnp.exp2(sa - jnp.concatenate([ml, mr], axis=1))
        pb = jnp.exp2(sb - mr)
        l8 = colreduce(pa, jnp.add)
        ll = jnp.sum(l8[:, :HT], axis=0, keepdims=True)
        lr = jnp.sum(l8[:, HT:] + colreduce(pb, jnp.add), axis=0, keepdims=True)
        return pa.astype(BF), pb.astype(BF), 1.0 / jnp.concatenate([ll, lr], axis=1)

    def pv_diag(i, pb):
        L = (i + 1) * TQ
        top = jnp.dot(vt_s[0:HT, L - HT:L], pb, preferred_element_type=F32)
        bot = jnp.dot(vt_s[HT:D, L - HT:L], pb, preferred_element_type=F32)
        return jnp.concatenate([top, bot], axis=0)

    def pv(i, pa, ob, inv):
        L = (i + 1) * TQ
        oa = jnp.dot(vt_s[:, 0:L - HT], pa, preferred_element_type=F32)
        ot = jnp.concatenate([oa[:, :HT], oa[:, HT:] + ob], axis=1)
        return (ot * inv).astype(BF)

    def outproj(i, ot, hh):
        acc_s[64:512, i * TQ:(i + 1) * TQ] += jnp.dot(wot[hh], ot, preferred_element_type=F32)

    def save_first_block():
        pa, pb, inv = softmax(0, qk_main(0), qk_diag(0))
        p0_s[0:HT, :] = pa
        p0_s[HT:TQ, HT:TQ] = pb
        inv0_s[...] = jnp.broadcast_to(inv, (8, TQ))

    @pl.when(h == 0)
    def _prologue():
        cp_g1.start()
        for c in range(S // 512):
            axt_copy(c).start()
        for cp in (cp_wrt, cp_wit, cp_perm, cp_m2, cp_bxt):
            cp.start(priority=1)
        for cp in wcopies(*wlist[0], 0):
            cp.start(priority=1)
        cp_ckv0.start(priority=1)
        for cp in wcopies(*wlist[1], 0) + wcopies(*wlist[2], 0):
            cp.start(priority=1)
        cp_g2.start(priority=1)
        cp_wot0.start(priority=1)
        cp_ckv1.start(priority=1)

        acc_s[...] = jnp.zeros_like(acc_s)
        bxt[DA:512, :] = jnp.zeros((512 - DA, S), BF)
        wqt_s[...] = jnp.zeros_like(wqt_s)

        cp_g1.wait()

        def step1(c, carry):
            axt_copy(c).wait()
            cols = pl.ds(pl.multiple_of(c * 512, 512), 512)
            x1_s[:, cols] = jnp.dot(g1[...], axt[:, cols], preferred_element_type=F32)
            return carry
        lax.fori_loop(0, S // 512, step1, 0)

        cp_wrt.wait()
        cp_wit.wait()
        cp_perm.wait()
        zpad = jnp.zeros((128, 256 - DF), F32)
        for a in range(N1):
            for (src, dst) in ((wrt, wr_s), (wit, wi_s)):
                t = lax.dot_general(perm[...], src[:, 128 * a:128 * (a + 1)], NT,
                                    preferred_element_type=F32)
                t = jnp.concatenate([t, zpad], axis=1)
                for k1 in range(N1):
                    dst[k1, 8 * a:8 * (a + 1), :] = t[8 * k1:8 * (k1 + 1), :]

        for r in range(0, FP, 8):
            xs = [(x1_s[r:r + 8, 128 * s1:128 * (s1 + 1)],
                   x1_s[FP + r:FP + r + 8, 128 * s1:128 * (s1 + 1)]) for s1 in range(N1)]
            ys = _fft16(xs, -1)
            for k1 in range(N1):
                a_s[k1, r:r + 8, 0:128] = ys[k1][0]
                a_s[k1, r:r + 8, 128:256] = ys[k1][1]
        a_s[:, FP:256, :] = jnp.zeros((N1, 256 - FP, 256), F32)

        cp_m2.wait()

        def mid_fwd(k1):
            mk = m2[k1]
            u = lax.dot_general(mk, a_s[k1, :, 0:128].astype(BF), NT, preferred_element_type=F32)
            v = lax.dot_general(mk, a_s[k1, :, 128:256].astype(BF), NT, preferred_element_type=F32)
            zr = u[0:128] - v[128:256]
            zi = u[128:256] + v[0:128]
            wr, wi = wr_s[k1], wi_s[k1]
            yr = (zr * wr - zi * wi).astype(BF)
            yi = (zr * wi + zi * wr).astype(BF)
            return jnp.concatenate([jnp.concatenate([yr, yi], axis=1),
                                    jnp.concatenate([yi, -yr], axis=1)], axis=0)

        rhs = {0: mid_fwd(0)}
        for k1 in range(N1):
            if k1 + 1 < N1:
                rhs[k1 + 1] = mid_fwd(k1 + 1)
            b_s[k1] = lax.dot_general(m2[k1], rhs.pop(k1), TN, preferred_element_type=F32)

        cp_bxt.wait()
        cp_ckv0.wait()
        for w in wlist:
            for cp in wcopies(*w, 0):
                cp.wait()
        def ifft(idx):
            g, t = idx // 2, idx % 2
            xs = [(b_s[k1, 8 * g:8 * g + 8, 128 * t:128 * (t + 1)],
                   b_s[k1, 8 * g:8 * g + 8, 256 + 128 * t:256 + 128 * (t + 1)]) for k1 in range(N1)]
            xs[0] = (jnp.where(never, 0.0, xs[0][0]), xs[0][1])
            ys = _fft16(xs, +1)
            for s1 in range(N1):
                r0 = 128 * s1 + 8 * g
                y1_s[r0:r0 + 8, 128 * t:128 * (t + 1)] = ys[s1][0]
                y1_s[r0:r0 + 8, 256 + 128 * t:256 + 128 * (t + 1)] = ys[s1][1]

        dep = pltpu.bitcast(bxt[0:16, 0:128], F32)
        never = (dep - dep) < -1.0
        prep_weights(h)
        stages = [lambda: (proj_q(0), proj_k(0)), lambda: (proj_q(1), proj_k(1)),
                  lambda: proj_v(0), lambda: proj_v(1)]
        for n, st in enumerate(stages):
            st()
            for idx in range(8 * n, 8 * n + 8):
                ifft(idx)
        save_first_block()
        ot7_s[...] = jnp.zeros_like(ot7_s)
        cp_g2.wait()

        def step7(c, carry):
            rows = pl.ds(pl.multiple_of(c * 512, 512), 512)
            ya = jnp.dot(y1_s[rows, :].astype(BF), g2[...], preferred_element_type=F32)
            o_s[rows, 0:DA] = ya.astype(BF)
            return carry
        lax.fori_loop(0, S // 512, step7, 0)
        cp_outa.start()

        cp_wot0.wait()
        cp_ckv1.wait()
        for w in wlist:
            for cp in wcopies(*w, 1):
                cp.start()
        cp_wot1.start()

    def at_head(hh, fn):
        def body(i, carry):
            fn()
            return carry
        lax.fori_loop(0, (h == hh).astype(jnp.int32), body, 0)

    def _stage1():
        for w in wlist:
            for cp in wcopies(*w, 1):
                cp.wait()
        cp_wot1.wait()
        cp_outa.wait()
        for w in wlist:
            for cp in wcopies(*w, 2):
                cp.start()

    def _stage2():
        for w in wlist:
            for cp in wcopies(*w, 2):
                cp.wait()

    at_head(1, _stage1)
    at_head(6, _stage2)

    ps = {0: (p0_s[0:HT, :], p0_s[HT:TQ, HT:TQ], inv0_s[0:1, :])}
    ots = {-1: ot7_s[...]}
    for t in range(NB):
        pa, pb, inv = ps.pop(t)
        nxt = (t + 2) % NB
        if t + 1 < NB:
            sa = qk_main(t + 1, dep if (PREP_FENCE and t + 1 == NB - 1) else None)
        if t + 2 < NB:
            proj_v(nxt)
        proj_q(nxt)
        if t + 1 < NB:
            ps[t + 1] = softmax(t + 1, sa, qk_diag(t + 1))
        else:
            save_first_block()
        proj_k(nxt)
        if t + 2 == NB - 1:
            dep = prep_weights(jnp.minimum(h + 1, H - 1))
        ob = pv_diag(t, pb)
        ots[t] = pv(t, pa, ob, inv)
        if t == 0:
            outproj(NB - 1, ots.pop(-1), jnp.maximum(h - 1, 0))
        else:
            outproj(t - 1, ots.pop(t - 1), h)
    proj_v(0)
    proj_v(1)
    ot7_s[...] = ots.pop(NB - 1)

    @pl.when(h == H - 1)
    def _epilogue():
        outproj(NB - 1, ot7_s[...], H - 1)
        OB = 256
        lane = lax.broadcasted_iota(jnp.int32, (OB, 128), 1)
        outs = []
        for i in range(S // OB):
            rows = slice(i * OB, (i + 1) * OB)
            bt = acc_s[:, rows].T.astype(BF)
            first = jnp.where(lane < 64, o_s[rows, 384:512], bt[:, 0:128])
            o_s[rows, 384:512] = first
            o_s[rows, 512:896] = bt[:, 128:512]
            cp = pltpu.make_async_copy(o_s.at[rows, 384:896], out_hbm.at[rows, 384:896], osem.at[i])
            cp.start()
            outs.append(cp)
        for cp in outs:
            cp.wait()


@jax.jit
def pallas_concat_heads__spectral_gfnet__compressed_kv_cla__prompt_kernel(
    A_x, A_w_r, A_w_i, B_x, B_c_kv, B_w_q, B_w_uk, B_w_uv, B_w_o,
):
    g1, m2, g2, perm = _tables()
    axt = jnp.swapaxes(A_x, 1, 2).reshape(DA, S)
    bxt = jnp.swapaxes(B_x, 1, 2).reshape(DA, S)
    wrt = A_w_r.T
    wit = A_w_i.T
    ckv = B_c_kv.reshape(S, C)
    wq = B_w_q.reshape(DA // 2, 2, H, D)
    wuk = B_w_uk.reshape(C // 2, 2, H, D)
    wuv = B_w_uv.reshape(C // 2, 2, H, D)
    wot = jnp.swapaxes(B_w_o, 1, 2)

    any_spec = pl.BlockSpec(memory_space=pl.ANY)
    V = pltpu.VMEM
    out = pl.pallas_call(
        _kernel,
        grid=(H,),
        in_specs=[any_spec] * 13,
        out_specs=any_spec,
        out_shape=jax.ShapeDtypeStruct((S, 2 * DA), BF),
        scratch_shapes=[
            V((DA, S), BF), V((DF, S), BF), V((DF, S), BF), V((512, S), BF), V((S, C), BF),
            V((2, 2, DA // 2, 8, 128), jnp.uint32),
            V((2, 2, C // 2, 8, 128), jnp.uint32),
            V((2, 2, C // 2, 8, 128), jnp.uint32),
            V((H, DA, D), BF),
            V((2 * FP, DA), BF), V((N1, 256, 128), BF), V((512, DA), BF),
            V((128, 128), BF),
            V((2 * FP, S), F32), V((N1, 256, 256), F32), V((N1, 128, 256), F32),
            V((N1, 128, 256), F32), V((N1, 128, 512), F32), V((S, 512), F32),
            V((D, 512), BF), V((C, D), BF), V((D, C), BF),
            V((D, S), BF), V((S, D), BF), V((D, S), BF), V((512, S), F32), V((S, 2 * DA), BF),
            V((TQ, TQ), BF), V((8, TQ), F32), V((D, TQ), BF),
            pltpu.SemaphoreType.DMA((12,)),
            pltpu.SemaphoreType.DMA((3, 3, 4)),
            pltpu.SemaphoreType.DMA((8,)),
            pltpu.SemaphoreType.DMA((4,)),
        ],
        compiler_params=pltpu.CompilerParams(
            dimension_semantics=("arbitrary",),
            vmem_limit_bytes=120 * 2**20),
    )(axt, wrt, wit, bxt, ckv, wq, wuk, wuv, wot, g1, m2, g2, perm)
    return out.reshape(1, S, 2 * DA)
```

```python
import numpy as np
import jax
import jax.numpy as jnp
from jax import lax
import jax.experimental.pallas as pl
import jax.experimental.pallas.tpu as pltpu

S = 2048
DA = 448
DF = DA // 2 + 1
FP = 240
H = 16
D = 256
C = 1024
N1 = 16
N2 = 128
TQ = 256
HT = 128
EMIT_BLOCKS = 7
QC = 256
QK_LAG = 2
PREP_FENCE = 1
LOG2E = 1.4426950408889634
MASK_VAL = -1e9 * LOG2E
BF = jnp.bfloat16
F32 = jnp.float32
NT = (((1,), (1,)), ((), ()))
TN = (((0,), (0,)), ((), ()))


def _tables():
    f = np.arange(FP)[:, None].astype(np.float64)
    d = np.arange(DA)[None, :].astype(np.float64)
    valid = (np.arange(FP) < DF)[:, None]
    ang = 2 * np.pi * ((f * d) % DA) / DA
    g1 = np.concatenate([np.cos(ang) * valid, -np.sin(ang) * valid], axis=0)
    k2 = np.arange(N2)[:, None]
    s2 = np.arange(N2)[None, :]
    m2 = np.zeros((N1, 2 * N2, N2))
    for k1 in range(N1):
        a = 2 * np.pi * ((s2 * (k1 + N1 * k2)) % S) / S
        m2[k1] = np.concatenate([np.cos(a), -np.sin(a)], axis=0)
    f2 = np.arange(256)[:, None].astype(np.float64)
    cf = np.where((f2 == 0) | (f2 == DA // 2), 1.0, 2.0) * (f2 < DF) / (S * DA)
    ang2 = 2 * np.pi * ((f2 * d) % DA) / DA
    g2 = np.concatenate([np.cos(ang2) * cf, -np.sin(ang2) * cf], axis=0)
    perm = np.zeros((128, 128))
    for k1 in range(N1):
        for j in range(8):
            perm[8 * k1 + j, k1 + 16 * j] = 1.0
    cast = lambda a: jnp.asarray(a.astype(np.float32), dtype=BF)
    return cast(g1), cast(m2), cast(g2), cast(perm)


def _fft4(xs, sign):
    (ar, ai), (br, bi), (cr, ci), (dr, di) = xs
    s0r, s0i = ar + cr, ai + ci
    s1r, s1i = ar - cr, ai - ci
    s2r, s2i = br + dr, bi + di
    s3r, s3i = br - dr, bi - di
    y0 = (s0r + s2r, s0i + s2i)
    y2 = (s0r - s2r, s0i - s2i)
    if sign < 0:
        y1 = (s1r + s3i, s1i - s3r)
        y3 = (s1r - s3i, s1i + s3r)
    else:
        y1 = (s1r - s3i, s1i + s3r)
        y3 = (s1r + s3i, s1i - s3r)
    return [y0, y1, y2, y3]


def _twiddle(z, e, sign):
    zr, zi = z
    e = e % 16
    if e == 0:
        return z
    if (e * sign) % 16 == 12:
        return (zi, -zr)
    if (e * sign) % 16 == 4:
        return (-zi, zr)
    c = float(np.cos(2 * np.pi * e / 16))
    s = float(sign * np.sin(2 * np.pi * e / 16))
    if abs(abs(c) - abs(s)) < 1e-12:
        r = abs(c)
        u = zr - zi if (c > 0) == (s > 0) else zr + zi
        v = zi + zr if (c > 0) == (s > 0) else zi - zr
        return (u * c, v * c)
    return (zr * c - zi * s, zi * c + zr * s)


def _fft16(xs, sign):
    t = [None] * 16
    for b in range(4):
        col = _fft4([xs[4 * a + b] for a in range(4)], sign)
        for c in range(4):
            t[4 * c + b] = _twiddle(col[c], b * c, sign)
    out = [None] * 16
    for c in range(4):
        col = _fft4([t[4 * c + b] for b in range(4)], sign)
        for e in range(4):
            out[c + 4 * e] = col[e]
    return out


def _kernel(axt_hbm, wrt_hbm, wit_hbm, bxt_hbm, ckv_hbm, wq_hbm, wuk_hbm, wuv_hbm, wot_hbm,
            g1_hbm, m2_hbm, g2_hbm, perm_hbm,
            out_hbm,
            axt, wrt, wit, bxt, ckv, wq_w, wuk_w, wuv_w, wot, g1, m2, g2, perm,
            x1_s, a_s, wr_s, wi_s, b_s, y1_s,
            wqt_s, wk_s, wvt_s, qt_s, k_s, vt_s, acc_s, o_s, p0_s, inv0_s, ot7_s,
            sem, wsem, osem, asem):
    h = pl.program_id(0)

    CK0 = 2 * TQ
    simple = [(g1_hbm, g1), (wrt_hbm, wrt), (wit_hbm, wit), (perm_hbm, perm),
              (m2_hbm, m2), (g2_hbm, g2), (bxt_hbm, bxt.at[0:DA]),
              (ckv_hbm.at[0:CK0], ckv.at[0:CK0]), (ckv_hbm.at[CK0:S], ckv.at[CK0:S]),
              (wot_hbm.at[0:1], wot.at[0:1]), (wot_hbm.at[1:H], wot.at[1:H]),
              (o_s.at[:, 0:384], out_hbm.at[:, 0:384])]
    cps = [pltpu.make_async_copy(s, d, sem.at[i]) for i, (s, d) in enumerate(simple)]
    (cp_g1, cp_wrt, cp_wit, cp_perm, cp_m2, cp_g2, cp_bxt, cp_ckv0, cp_ckv1,
     cp_wot0, cp_wot1, cp_outa) = cps

    def axt_copy(c):
        cols = pl.ds(pl.multiple_of(c * 512, 512), 512)
        return pltpu.make_async_copy(axt_hbm.at[:, cols], axt.at[:, cols], asem.at[c])

    def wcopies(widx, w_hbm, w_buf, stage):
        src = w_hbm.bitcast(jnp.uint32)
        g, j0, n = ((0, 0, 1), (0, 1, 3), (1, 0, 4))[stage]
        return [pltpu.make_async_copy(
            src.at[:, p, pl.ds(4 * g + j0, n), pl.ds(128 * t, 128)],
            w_buf.at[g, t, :, pl.ds(4 * p + j0, n), :],
            wsem.at[widx, stage, 2 * t + p]) for t in range(2) for p in range(2)]

    wlist = [(0, wq_hbm, wq_w), (1, wuk_hbm, wuk_w), (2, wuv_hbm, wuv_w)]

    def head_weight(w_buf, rows, hh):
        g = lax.shift_right_logical(hh, 3)
        j = lax.shift_right_logical(hh, 1) & 3
        sh = ((hh & 1) * 16).astype(jnp.uint32)
        halves = []
        for t in range(2):
            w2 = w_buf.at[g, t].reshape(rows * 4, 128)
            a = w2[pl.ds(j, rows, stride=4), :]
            halves.append(pltpu.bitcast((a >> sh) << 16, F32))
        return jnp.concatenate(halves, axis=1)

    def orall(x):
        w = pltpu.bitcast(x, jnp.uint32)
        acc = None
        for r in range(0, w.shape[0], 8):
            for c in range(0, w.shape[1], 128):
                t = w[r:r + 8, c:min(c + 128, w.shape[1])]
                if t.shape[1] < 128:
                    continue
                acc = t if acc is None else acc | t
        return acc

    def prep_weights(hh):
        a = head_weight(wq_w, DA, hh).T.astype(BF)
        b = head_weight(wuk_w, C, hh).astype(BF)
        c = head_weight(wuv_w, C, hh).T.astype(BF)
        wqt_s[:, 0:DA] = a
        wk_s[...] = b
        wvt_s[...] = c
        deps = [orall(a)]
        if PREP_FENCE >= 2:
            deps.append(orall(b))
        if PREP_FENCE >= 3:
            deps.append(orall(c))
        d = deps[0]
        for e in deps[1:]:
            d = d | e
        return pltpu.bitcast(d, F32)

    NB = S // TQ
    key = lax.broadcasted_iota(jnp.int32, (HT, HT), 0)
    qry = lax.broadcasted_iota(jnp.int32, (HT, HT), 1)
    causal = key <= qry

    def proj_q(i):
        cs = slice(i * TQ, (i + 1) * TQ)
        qt = jnp.dot(wqt_s[...], bxt[:, cs], preferred_element_type=F32) * (D ** -0.5 * LOG2E)
        qt_s[:, cs] = qt.astype(BF)

    def proj_k(i):
        cs = slice(i * TQ, (i + 1) * TQ)
        k_s[cs, :] = jnp.dot(ckv[cs, :], wk_s[...], preferred_element_type=F32).astype(BF)

    def proj_v(i):
        cs = slice(i * TQ, (i + 1) * TQ)
        vt_s[:, cs] = lax.dot_general(wvt_s[...], ckv[cs, :], NT,
                                      preferred_element_type=F32).astype(BF)

    def colreduce(x, op, nacc=4):
        accs = [x[8 * a:8 * a + 8] for a in range(nacc)]
        for r in range(8 * nacc, x.shape[0], 8 * nacc):
            for a in range(nacc):
                accs[a] = op(accs[a], x[r + 8 * a:r + 8 * a + 8])
        while len(accs) > 1:
            accs = [op(accs[2 * a], accs[2 * a + 1]) for a in range(len(accs) // 2)]
        return accs[0]

    def fence(x, dep):
        never = (dep - dep) < -1.0
        head = pltpu.bitcast(x[0:16, 0:128], jnp.uint32)
        head = pltpu.bitcast(jnp.where(never, jnp.uint32(0), head), BF)
        top = jnp.concatenate([head, x[0:16, 128:]], axis=1)
        return jnp.concatenate([top, x[16:]], axis=0)

    def qk_main(i, dep=None):
        L = (i + 1) * TQ
        qt = qt_s[:, i * TQ:(i + 1) * TQ]
        if dep is not None:
            qt = fence(qt, dep)
        bounds = list(range(0, L - HT, QC)) + [L - HT]
        sts, ms = [], []
        for c in range(len(bounds) - 1):
            kc = k_s[bounds[c]:bounds[c + 1], :]
            if c >= QK_LAG:
                kc = fence(kc, ms[c - QK_LAG][:, 0:HT] + ms[c - QK_LAG][:, HT:])
            st = jnp.dot(kc, qt, preferred_element_type=F32)
            if c == len(bounds) - 2:
                n = st.shape[0]
                dg = jnp.concatenate([jnp.where(causal, st[n - HT:, :HT], MASK_VAL), st[n - HT:, HT:]], axis=1)
                st = jnp.concatenate([st[:n - HT], dg], axis=0) if n > HT else dg
            mc = colreduce(st, jnp.maximum)
            ms.append(mc if c == 0 else jnp.maximum(ms[-1], mc))
            sts.append(st)
        return jnp.concatenate(sts, axis=0), ms[-1]

    def qk_diag(i):
        L = (i + 1) * TQ
        return jnp.dot(k_s[L - HT:L, :], qt_s[:, L - HT:L], preferred_element_type=F32)

    def softmax(i, sa_m8, sb):
        sa, m8 = sa_m8
        L = (i + 1) * TQ
        sb = jnp.where(causal, sb, MASK_VAL)
        ml = jnp.max(m8[:, :HT], axis=0, keepdims=True)
        mr = jnp.max(jnp.maximum(m8[:, HT:], colreduce(sb, jnp.maximum)), axis=0, keepdims=True)
        pa = jnp.exp2(sa - jnp.concatenate([ml, mr], axis=1))
        pb = jnp.exp2(sb - mr)
        l8 = colreduce(pa, jnp.add)
        ll = jnp.sum(l8[:, :HT], axis=0, keepdims=True)
        lr = jnp.sum(l8[:, HT:] + colreduce(pb, jnp.add), axis=0, keepdims=True)
        return pa.astype(BF), pb.astype(BF), 1.0 / jnp.concatenate([ll, lr], axis=1)

    def pv_diag(i, pb):
        L = (i + 1) * TQ
        top = jnp.dot(vt_s[0:HT, L - HT:L], pb, preferred_element_type=F32)
        bot = jnp.dot(vt_s[HT:D, L - HT:L], pb, preferred_element_type=F32)
        return jnp.concatenate([top, bot], axis=0)

    def pv(i, pa, ob, inv):
        L = (i + 1) * TQ
        oa = jnp.dot(vt_s[:, 0:L - HT], pa, preferred_element_type=F32)
        ot = jnp.concatenate([oa[:, :HT], oa[:, HT:] + ob], axis=1)
        return (ot * inv).astype(BF)

    def out_copy(i):
        rows = slice(i * TQ, (i + 1) * TQ)
        return pltpu.make_async_copy(o_s.at[rows, 384:896], out_hbm.at[rows, 384:896], osem.at[i])

    def emit_block(i, acc):
        rows = slice(i * TQ, (i + 1) * TQ)
        lane = lax.broadcasted_iota(jnp.int32, (TQ, 128), 1)
        bt = jnp.concatenate([jnp.zeros((64, TQ), F32), acc], axis=0).T.astype(BF)
        o_s[rows, 384:512] = jnp.where(lane < 64, o_s[rows, 384:512], bt[:, 0:128])
        o_s[rows, 512:896] = bt[:, 128:512]

    def outproj(i, ot, hh, emit=False):
        cols = slice(i * TQ, (i + 1) * TQ)
        acc = acc_s[64:512, cols] + jnp.dot(wot[hh], ot, preferred_element_type=F32)
        acc_s[64:512, cols] = acc
        if emit:
            emit_block(i, acc)

            @pl.when(h == H - 1)
            def _():
                out_copy(i).start()

    def save_first_block():
        pa, pb, inv = softmax(0, qk_main(0), qk_diag(0))
        p0_s[0:HT, :] = pa
        p0_s[HT:TQ, HT:TQ] = pb
        inv0_s[...] = jnp.broadcast_to(inv, (8, TQ))

    @pl.when(h == 0)
    def _prologue():
        cp_g1.start()
        for c in range(S // 512):
            axt_copy(c).start()
        for cp in (cp_wrt, cp_wit, cp_perm, cp_m2, cp_bxt):
            cp.start(priority=1)
        for cp in wcopies(*wlist[0], 0):
            cp.start(priority=1)
        cp_ckv0.start(priority=1)
        for cp in wcopies(*wlist[1], 0) + wcopies(*wlist[2], 0):
            cp.start(priority=1)
        cp_g2.start(priority=1)
        cp_wot0.start(priority=1)
        cp_ckv1.start(priority=1)

        acc_s[...] = jnp.zeros_like(acc_s)
        bxt[DA:512, :] = jnp.zeros((512 - DA, S), BF)
        wqt_s[...] = jnp.zeros_like(wqt_s)

        cp_g1.wait()

        def step1(c, carry):
            axt_copy(c).wait()
            cols = pl.ds(pl.multiple_of(c * 512, 512), 512)
            x1_s[:, cols] = jnp.dot(g1[...], axt[:, cols], preferred_element_type=F32)
            return carry
        lax.fori_loop(0, S // 512, step1, 0)

        cp_wrt.wait()
        cp_wit.wait()
        cp_perm.wait()
        zpad = jnp.zeros((128, 256 - DF), F32)
        for a in range(N1):
            for (src, dst) in ((wrt, wr_s), (wit, wi_s)):
                t = lax.dot_general(perm[...], src[:, 128 * a:128 * (a + 1)], NT,
                                    preferred_element_type=F32)
                t = jnp.concatenate([t, zpad], axis=1)
                for k1 in range(N1):
                    dst[k1, 8 * a:8 * (a + 1), :] = t[8 * k1:8 * (k1 + 1), :]

        for r in range(0, FP, 8):
            xs = [(x1_s[r:r + 8, 128 * s1:128 * (s1 + 1)],
                   x1_s[FP + r:FP + r + 8, 128 * s1:128 * (s1 + 1)]) for s1 in range(N1)]
            ys = _fft16(xs, -1)
            for k1 in range(N1):
                a_s[k1, r:r + 8, 0:128] = ys[k1][0]
                a_s[k1, r:r + 8, 128:256] = ys[k1][1]
        a_s[:, FP:256, :] = jnp.zeros((N1, 256 - FP, 256), F32)

        cp_m2.wait()

        def mid_fwd(k1):
            mk = m2[k1]
            u = lax.dot_general(mk, a_s[k1, :, 0:128].astype(BF), NT, preferred_element_type=F32)
            v = lax.dot_general(mk, a_s[k1, :, 128:256].astype(BF), NT, preferred_element_type=F32)
            zr = u[0:128] - v[128:256]
            zi = u[128:256] + v[0:128]
            wr, wi = wr_s[k1], wi_s[k1]
            yr = (zr * wr - zi * wi).astype(BF)
            yi = (zr * wi + zi * wr).astype(BF)
            return jnp.concatenate([jnp.concatenate([yr, yi], axis=1),
                                    jnp.concatenate([yi, -yr], axis=1)], axis=0)

        rhs = {0: mid_fwd(0)}
        for k1 in range(N1):
            if k1 + 1 < N1:
                rhs[k1 + 1] = mid_fwd(k1 + 1)
            b_s[k1] = lax.dot_general(m2[k1], rhs.pop(k1), TN, preferred_element_type=F32)

        cp_bxt.wait()
        cp_ckv0.wait()
        for w in wlist:
            for cp in wcopies(*w, 0):
                cp.wait()
        def ifft(idx):
            g, t = idx // 2, idx % 2
            xs = [(b_s[k1, 8 * g:8 * g + 8, 128 * t:128 * (t + 1)],
                   b_s[k1, 8 * g:8 * g + 8, 256 + 128 * t:256 + 128 * (t + 1)]) for k1 in range(N1)]
            xs[0] = (jnp.where(never, 0.0, xs[0][0]), xs[0][1])
            ys = _fft16(xs, +1)
            for s1 in range(N1):
                r0 = 128 * s1 + 8 * g
                y1_s[r0:r0 + 8, 128 * t:128 * (t + 1)] = ys[s1][0]
                y1_s[r0:r0 + 8, 256 + 128 * t:256 + 128 * (t + 1)] = ys[s1][1]

        dep = pltpu.bitcast(bxt[0:16, 0:128], F32)
        never = (dep - dep) < -1.0
        prep_weights(h)
        stages = [lambda: (proj_q(0), proj_k(0)), lambda: (proj_q(1), proj_k(1)),
                  lambda: proj_v(0), lambda: proj_v(1)]
        for n, st in enumerate(stages):
            st()
            for idx in range(8 * n, 8 * n + 8):
                ifft(idx)
        save_first_block()
        ot7_s[...] = jnp.zeros_like(ot7_s)
        cp_g2.wait()

        def step7(c, carry):
            rows = pl.ds(pl.multiple_of(c * 512, 512), 512)
            ya = jnp.dot(y1_s[rows, :].astype(BF), g2[...], preferred_element_type=F32)
            o_s[rows, 0:DA] = ya.astype(BF)
            return carry
        lax.fori_loop(0, S // 512, step7, 0)
        cp_outa.start()

        cp_wot0.wait()
        cp_ckv1.wait()
        for w in wlist:
            for cp in wcopies(*w, 1):
                cp.start()
        cp_wot1.start()

    def at_head(hh, fn):
        def body(i, carry):
            fn()
            return carry
        lax.fori_loop(0, (h == hh).astype(jnp.int32), body, 0)

    def _stage1():
        for w in wlist:
            for cp in wcopies(*w, 1):
                cp.wait()
        cp_wot1.wait()
        cp_outa.wait()
        for w in wlist:
            for cp in wcopies(*w, 2):
                cp.start()

    def _stage2():
        for w in wlist:
            for cp in wcopies(*w, 2):
                cp.wait()

    at_head(1, _stage1)
    at_head(6, _stage2)

    ps = {0: (p0_s[0:HT, :], p0_s[HT:TQ, HT:TQ], inv0_s[0:1, :])}
    ots = {-1: ot7_s[...]}
    for t in range(NB):
        pa, pb, inv = ps.pop(t)
        nxt = (t + 2) % NB
        if t + 1 < NB:
            sa = qk_main(t + 1, dep if (PREP_FENCE and t + 1 == NB - 1) else None)
        if t + 2 < NB:
            proj_v(nxt)
        proj_q(nxt)
        if t + 1 < NB:
            ps[t + 1] = softmax(t + 1, sa, qk_diag(t + 1))
        else:
            save_first_block()
        proj_k(nxt)
        if t + 2 == NB - 1:
            dep = prep_weights(jnp.minimum(h + 1, H - 1))
        ob = pv_diag(t, pb)
        ots[t] = pv(t, pa, ob, inv)
        if t == 0:
            outproj(NB - 1, ots.pop(-1), jnp.maximum(h - 1, 0))
        else:
            outproj(t - 1, ots.pop(t - 1), h, emit=(t - 1) < EMIT_BLOCKS)
    proj_v(0)
    proj_v(1)
    ot7_s[...] = ots.pop(NB - 1)

    @pl.when(h == H - 1)
    def _epilogue():
        outproj(NB - 1, ot7_s[...], H - 1)
        for i in range(EMIT_BLOCKS, NB):
            emit_block(i, acc_s[64:512, i * TQ:(i + 1) * TQ])
            out_copy(i).start()
        for i in range(NB):
            out_copy(i).wait()


@jax.jit
def pallas_concat_heads__spectral_gfnet__compressed_kv_cla__prompt_kernel(
    A_x, A_w_r, A_w_i, B_x, B_c_kv, B_w_q, B_w_uk, B_w_uv, B_w_o,
):
    g1, m2, g2, perm = _tables()
    axt = jnp.swapaxes(A_x, 1, 2).reshape(DA, S)
    bxt = jnp.swapaxes(B_x, 1, 2).reshape(DA, S)
    wrt = A_w_r.T
    wit = A_w_i.T
    ckv = B_c_kv.reshape(S, C)
    wq = B_w_q.reshape(DA // 2, 2, H, D)
    wuk = B_w_uk.reshape(C // 2, 2, H, D)
    wuv = B_w_uv.reshape(C // 2, 2, H, D)
    wot = jnp.swapaxes(B_w_o, 1, 2)

    any_spec = pl.BlockSpec(memory_space=pl.ANY)
    V = pltpu.VMEM
    out = pl.pallas_call(
        _kernel,
        grid=(H,),
        in_specs=[any_spec] * 13,
        out_specs=any_spec,
        out_shape=jax.ShapeDtypeStruct((S, 2 * DA), BF),
        scratch_shapes=[
            V((DA, S), BF), V((DF, S), BF), V((DF, S), BF), V((512, S), BF), V((S, C), BF),
            V((2, 2, DA // 2, 8, 128), jnp.uint32),
            V((2, 2, C // 2, 8, 128), jnp.uint32),
            V((2, 2, C // 2, 8, 128), jnp.uint32),
            V((H, DA, D), BF),
            V((2 * FP, DA), BF), V((N1, 256, 128), BF), V((512, DA), BF),
            V((128, 128), BF),
            V((2 * FP, S), F32), V((N1, 256, 256), F32), V((N1, 128, 256), F32),
            V((N1, 128, 256), F32), V((N1, 128, 512), F32), V((S, 512), F32),
            V((D, 512), BF), V((C, D), BF), V((D, C), BF),
            V((D, S), BF), V((S, D), BF), V((D, S), BF), V((512, S), F32), V((S, 2 * DA), BF),
            V((TQ, TQ), BF), V((8, TQ), F32), V((D, TQ), BF),
            pltpu.SemaphoreType.DMA((12,)),
            pltpu.SemaphoreType.DMA((3, 3, 4)),
            pltpu.SemaphoreType.DMA((8,)),
            pltpu.SemaphoreType.DMA((4,)),
        ],
        compiler_params=pltpu.CompilerParams(
            dimension_semantics=("arbitrary",),
            vmem_limit_bytes=120 * 2**20),
    )(axt, wrt, wit, bxt, ckv, wq, wuk, wuv, wot, g1, m2, g2, perm)
    return out.reshape(1, S, 2 * DA)
```

```python
import numpy as np
import jax
import jax.numpy as jnp
from jax import lax
import jax.experimental.pallas as pl
import jax.experimental.pallas.tpu as pltpu

S = 2048
DA = 448
DF = DA // 2 + 1
FP = 240
H = 16
D = 256
C = 1024
N1 = 16
N2 = 128
TQ = 256
HT = 128
EMIT_BLOCKS = 7
QC = 256
QK_LAG = 2
STEP_ORDER = ['MWVqdkeXPO'] + ['MVqdkePO'] * 5 + ['MqdkePO', 'dePOkq']
LOG2E = 1.4426950408889634
MASK_VAL = -1e9 * LOG2E
BF = jnp.bfloat16
F32 = jnp.float32
NT = (((1,), (1,)), ((), ()))
TN = (((0,), (0,)), ((), ()))


def _tables():
    f = np.arange(FP)[:, None].astype(np.float64)
    d = np.arange(DA)[None, :].astype(np.float64)
    valid = (np.arange(FP) < DF)[:, None]
    ang = 2 * np.pi * ((f * d) % DA) / DA
    g1 = np.concatenate([np.cos(ang) * valid, -np.sin(ang) * valid], axis=0)
    k2 = np.arange(N2)[:, None]
    s2 = np.arange(N2)[None, :]
    m2 = np.zeros((N1, 2 * N2, N2))
    for k1 in range(N1):
        a = 2 * np.pi * ((s2 * (k1 + N1 * k2)) % S) / S
        m2[k1] = np.concatenate([np.cos(a), -np.sin(a)], axis=0)
    f2 = np.arange(256)[:, None].astype(np.float64)
    cf = np.where((f2 == 0) | (f2 == DA // 2), 1.0, 2.0) * (f2 < DF) / (S * DA)
    ang2 = 2 * np.pi * ((f2 * d) % DA) / DA
    g2 = np.concatenate([np.cos(ang2) * cf, -np.sin(ang2) * cf], axis=0)
    perm = np.zeros((128, 128))
    for k1 in range(N1):
        for j in range(8):
            perm[8 * k1 + j, k1 + 16 * j] = 1.0
    cast = lambda a: jnp.asarray(a.astype(np.float32), dtype=BF)
    return cast(g1), cast(m2), cast(g2), cast(perm)


def _fft4(xs, sign):
    (ar, ai), (br, bi), (cr, ci), (dr, di) = xs
    s0r, s0i = ar + cr, ai + ci
    s1r, s1i = ar - cr, ai - ci
    s2r, s2i = br + dr, bi + di
    s3r, s3i = br - dr, bi - di
    y0 = (s0r + s2r, s0i + s2i)
    y2 = (s0r - s2r, s0i - s2i)
    if sign < 0:
        y1 = (s1r + s3i, s1i - s3r)
        y3 = (s1r - s3i, s1i + s3r)
    else:
        y1 = (s1r - s3i, s1i + s3r)
        y3 = (s1r + s3i, s1i - s3r)
    return [y0, y1, y2, y3]


def _twiddle(z, e, sign):
    zr, zi = z
    e = e % 16
    if e == 0:
        return z
    if (e * sign) % 16 == 12:
        return (zi, -zr)
    if (e * sign) % 16 == 4:
        return (-zi, zr)
    c = float(np.cos(2 * np.pi * e / 16))
    s = float(sign * np.sin(2 * np.pi * e / 16))
    if abs(abs(c) - abs(s)) < 1e-12:
        r = abs(c)
        u = zr - zi if (c > 0) == (s > 0) else zr + zi
        v = zi + zr if (c > 0) == (s > 0) else zi - zr
        return (u * c, v * c)
    return (zr * c - zi * s, zi * c + zr * s)


def _fft16(xs, sign):
    t = [None] * 16
    for b in range(4):
        col = _fft4([xs[4 * a + b] for a in range(4)], sign)
        for c in range(4):
            t[4 * c + b] = _twiddle(col[c], b * c, sign)
    out = [None] * 16
    for c in range(4):
        col = _fft4([t[4 * c + b] for b in range(4)], sign)
        for e in range(4):
            out[c + 4 * e] = col[e]
    return out


def _kernel(axt_hbm, wrt_hbm, wit_hbm, bxt_hbm, ckv_hbm, wq_hbm, wuk_hbm, wuv_hbm, wot_hbm,
            g1_hbm, m2_hbm, g2_hbm, perm_hbm,
            out_hbm,
            axt, wrt, wit, bxt, ckv, wq_w, wuk_w, wuv_w, wot, g1, m2, g2, perm,
            x1_s, a_s, wr_s, wi_s, b_s, y1_s,
            wqt_s, wk_s, wvt_s, qt_s, k_s, vt_s, acc_s, o_s, p0_s, inv0_s, ot7_s,
            sem, wsem, osem, asem):
    h = pl.program_id(0)

    CK0 = 2 * TQ
    simple = [(g1_hbm, g1), (wrt_hbm, wrt), (wit_hbm, wit), (perm_hbm, perm),
              (m2_hbm, m2), (g2_hbm, g2), (bxt_hbm, bxt.at[0:DA]),
              (ckv_hbm.at[0:CK0], ckv.at[0:CK0]), (ckv_hbm.at[CK0:S], ckv.at[CK0:S]),
              (wot_hbm.at[0:1], wot.at[0:1]), (wot_hbm.at[1:H], wot.at[1:H]),
              (o_s.at[:, 0:384], out_hbm.at[:, 0:384])]
    cps = [pltpu.make_async_copy(s, d, sem.at[i]) for i, (s, d) in enumerate(simple)]
    (cp_g1, cp_wrt, cp_wit, cp_perm, cp_m2, cp_g2, cp_bxt, cp_ckv0, cp_ckv1,
     cp_wot0, cp_wot1, cp_outa) = cps

    def axt_copy(c):
        cols = pl.ds(pl.multiple_of(c * 512, 512), 512)
        return pltpu.make_async_copy(axt_hbm.at[:, cols], axt.at[:, cols], asem.at[c])

    def wcopies(widx, w_hbm, w_buf, stage):
        src = w_hbm.bitcast(jnp.uint32)
        g, j0, n = ((0, 0, 1), (0, 1, 3), (1, 0, 4))[stage]
        return [pltpu.make_async_copy(
            src.at[:, p, pl.ds(4 * g + j0, n), pl.ds(128 * t, 128)],
            w_buf.at[g, t, :, pl.ds(4 * p + j0, n), :],
            wsem.at[widx, stage, 2 * t + p]) for t in range(2) for p in range(2)]

    wlist = [(0, wq_hbm, wq_w), (1, wuk_hbm, wuk_w), (2, wuv_hbm, wuv_w)]

    def head_weight(w_buf, rows, hh):
        g = lax.shift_right_logical(hh, 3)
        j = lax.shift_right_logical(hh, 1) & 3
        sh = ((hh & 1) * 16).astype(jnp.uint32)
        halves = []
        for t in range(2):
            w2 = w_buf.at[g, t].reshape(rows * 4, 128)
            a = w2[pl.ds(j, rows, stride=4), :]
            halves.append(pltpu.bitcast((a >> sh) << 16, F32))
        return jnp.concatenate(halves, axis=1)

    def orall(x):
        w = pltpu.bitcast(x, jnp.uint32)
        acc = None
        for r in range(0, w.shape[0], 8):
            for c in range(0, w.shape[1], 128):
                t = w[r:r + 8, c:min(c + 128, w.shape[1])]
                if t.shape[1] < 128:
                    continue
                acc = t if acc is None else acc | t
        return acc

    def prep_weights(hh):
        a = head_weight(wq_w, DA, hh).T.astype(BF)
        b = head_weight(wuk_w, C, hh).astype(BF)
        c = head_weight(wuv_w, C, hh).T.astype(BF)
        wqt_s[:, 0:DA] = a
        wk_s[...] = b
        wvt_s[...] = c
        return pltpu.bitcast(orall(a), F32)

    NB = S // TQ
    key = lax.broadcasted_iota(jnp.int32, (HT, HT), 0)
    qry = lax.broadcasted_iota(jnp.int32, (HT, HT), 1)
    causal = key <= qry

    def proj_q(i):
        cs = slice(i * TQ, (i + 1) * TQ)
        qt = jnp.dot(wqt_s[...], bxt[:, cs], preferred_element_type=F32) * (D ** -0.5 * LOG2E)
        qt_s[:, cs] = qt.astype(BF)

    def proj_k(i):
        cs = slice(i * TQ, (i + 1) * TQ)
        k_s[cs, :] = jnp.dot(ckv[cs, :], wk_s[...], preferred_element_type=F32).astype(BF)

    def proj_v(i):
        cs = slice(i * TQ, (i + 1) * TQ)
        vt_s[:, cs] = lax.dot_general(wvt_s[...], ckv[cs, :], NT,
                                      preferred_element_type=F32).astype(BF)

    def colreduce(x, op, nacc=4):
        accs = [x[8 * a:8 * a + 8] for a in range(nacc)]
        for r in range(8 * nacc, x.shape[0], 8 * nacc):
            for a in range(nacc):
                accs[a] = op(accs[a], x[r + 8 * a:r + 8 * a + 8])
        while len(accs) > 1:
            accs = [op(accs[2 * a], accs[2 * a + 1]) for a in range(len(accs) // 2)]
        return accs[0]

    def fence(x, dep):
        never = (dep - dep) < -1.0
        head = pltpu.bitcast(x[0:16, 0:128], jnp.uint32)
        head = pltpu.bitcast(jnp.where(never, jnp.uint32(0), head), BF)
        top = jnp.concatenate([head, x[0:16, 128:]], axis=1)
        return jnp.concatenate([top, x[16:]], axis=0)

    def qk_main(i, dep=None):
        L = (i + 1) * TQ
        qt = qt_s[:, i * TQ:(i + 1) * TQ]
        if dep is not None:
            qt = fence(qt, dep)
        bounds = list(range(0, L - HT, QC)) + [L - HT]
        sts, ms = [], []
        for c in range(len(bounds) - 1):
            kc = k_s[bounds[c]:bounds[c + 1], :]
            if c >= QK_LAG:
                kc = fence(kc, ms[c - QK_LAG][:, 0:HT] + ms[c - QK_LAG][:, HT:])
            st = jnp.dot(kc, qt, preferred_element_type=F32)
            if c == len(bounds) - 2:
                n = st.shape[0]
                dg = jnp.concatenate([jnp.where(causal, st[n - HT:, :HT], MASK_VAL), st[n - HT:, HT:]], axis=1)
                st = jnp.concatenate([st[:n - HT], dg], axis=0) if n > HT else dg
            mc = colreduce(st, jnp.maximum, 8)
            ms.append(mc if c == 0 else jnp.maximum(ms[-1], mc))
            sts.append(st)
        return jnp.concatenate(sts, axis=0), ms[-1]

    def qk_diag(i):
        L = (i + 1) * TQ
        return jnp.dot(k_s[L - HT:L, :], qt_s[:, L - HT:L], preferred_element_type=F32)

    def softmax(i, sa_m8, sb):
        sa, m8 = sa_m8
        L = (i + 1) * TQ
        sb = jnp.where(causal, sb, MASK_VAL)
        ml = jnp.max(m8[:, :HT], axis=0, keepdims=True)
        mr = jnp.max(jnp.maximum(m8[:, HT:], colreduce(sb, jnp.maximum, 8)), axis=0, keepdims=True)
        pa = jnp.exp2(sa - jnp.concatenate([ml, mr], axis=1))
        pb = jnp.exp2(sb - mr)
        l8 = colreduce(pa, jnp.add)
        ll = jnp.sum(l8[:, :HT], axis=0, keepdims=True)
        lr = jnp.sum(l8[:, HT:] + colreduce(pb, jnp.add), axis=0, keepdims=True)
        return pa.astype(BF), pb.astype(BF), 1.0 / jnp.concatenate([ll, lr], axis=1)

    def pv_diag(i, pb):
        L = (i + 1) * TQ
        top = jnp.dot(vt_s[0:HT, L - HT:L], pb, preferred_element_type=F32)
        bot = jnp.dot(vt_s[HT:D, L - HT:L], pb, preferred_element_type=F32)
        return jnp.concatenate([top, bot], axis=0)

    def pv(i, pa, ob, inv):
        L = (i + 1) * TQ
        oa = jnp.dot(vt_s[:, 0:L - HT], pa, preferred_element_type=F32)
        ot = jnp.concatenate([oa[:, :HT], oa[:, HT:] + ob], axis=1)
        return (ot * inv).astype(BF)

    def out_copy(i):
        rows = slice(i * TQ, (i + 1) * TQ)
        return pltpu.make_async_copy(o_s.at[rows, 384:896], out_hbm.at[rows, 384:896], osem.at[i])

    def emit_block(i, acc):
        rows = slice(i * TQ, (i + 1) * TQ)
        lane = lax.broadcasted_iota(jnp.int32, (TQ, 128), 1)
        bt = jnp.concatenate([jnp.zeros((64, TQ), F32), acc], axis=0).T.astype(BF)
        o_s[rows, 384:512] = jnp.where(lane < 64, o_s[rows, 384:512], bt[:, 0:128])
        o_s[rows, 512:896] = bt[:, 128:512]

    def outproj(i, ot, hh, emit=False):
        cols = slice(i * TQ, (i + 1) * TQ)
        acc = acc_s[64:512, cols] + jnp.dot(wot[hh], ot, preferred_element_type=F32)
        acc_s[64:512, cols] = acc
        if emit:
            emit_block(i, acc)

            @pl.when(h == H - 1)
            def _():
                out_copy(i).start()

    def save_first_block():
        pa, pb, inv = softmax(0, qk_main(0), qk_diag(0))
        p0_s[0:HT, :] = pa
        p0_s[HT:TQ, HT:TQ] = pb
        inv0_s[...] = jnp.broadcast_to(inv, (8, TQ))

    @pl.when(h == 0)
    def _prologue():
        cp_g1.start()
        for c in range(S // 512):
            axt_copy(c).start()
        for cp in (cp_wrt, cp_wit, cp_perm, cp_m2, cp_bxt):
            cp.start(priority=1)
        for cp in wcopies(*wlist[0], 0):
            cp.start(priority=1)
        cp_ckv0.start(priority=1)
        for cp in wcopies(*wlist[1], 0) + wcopies(*wlist[2], 0):
            cp.start(priority=1)
        cp_g2.start(priority=1)
        cp_wot0.start(priority=1)
        cp_ckv1.start(priority=1)

        acc_s[...] = jnp.zeros_like(acc_s)
        bxt[DA:512, :] = jnp.zeros((512 - DA, S), BF)
        wqt_s[...] = jnp.zeros_like(wqt_s)

        cp_g1.wait()

        def step1(c, carry):
            axt_copy(c).wait()
            cols = pl.ds(pl.multiple_of(c * 512, 512), 512)
            x1_s[:, cols] = jnp.dot(g1[...], axt[:, cols], preferred_element_type=F32)
            return carry
        lax.fori_loop(0, S // 512, step1, 0)

        cp_wrt.wait()
        cp_wit.wait()
        cp_perm.wait()
        zpad = jnp.zeros((128, 256 - DF), F32)
        for a in range(N1):
            for (src, dst) in ((wrt, wr_s), (wit, wi_s)):
                t = lax.dot_general(perm[...], src[:, 128 * a:128 * (a + 1)], NT,
                                    preferred_element_type=F32)
                t = jnp.concatenate([t, zpad], axis=1)
                for k1 in range(N1):
                    dst[k1, 8 * a:8 * (a + 1), :] = t[8 * k1:8 * (k1 + 1), :]

        for r in range(0, FP, 8):
            xs = [(x1_s[r:r + 8, 128 * s1:128 * (s1 + 1)],
                   x1_s[FP + r:FP + r + 8, 128 * s1:128 * (s1 + 1)]) for s1 in range(N1)]
            ys = _fft16(xs, -1)
            for k1 in range(N1):
                a_s[k1, r:r + 8, 0:128] = ys[k1][0]
                a_s[k1, r:r + 8, 128:256] = ys[k1][1]
        a_s[:, FP:256, :] = jnp.zeros((N1, 256 - FP, 256), F32)

        cp_m2.wait()

        def mid_fwd(k1):
            mk = m2[k1]
            u = lax.dot_general(mk, a_s[k1, :, 0:128].astype(BF), NT, preferred_element_type=F32)
            v = lax.dot_general(mk, a_s[k1, :, 128:256].astype(BF), NT, preferred_element_type=F32)
            zr = u[0:128] - v[128:256]
            zi = u[128:256] + v[0:128]
            wr, wi = wr_s[k1], wi_s[k1]
            yr = (zr * wr - zi * wi).astype(BF)
            yi = (zr * wi + zi * wr).astype(BF)
            return jnp.concatenate([jnp.concatenate([yr, yi], axis=1),
                                    jnp.concatenate([yi, -yr], axis=1)], axis=0)

        rhs = {0: mid_fwd(0)}
        for k1 in range(N1):
            if k1 + 1 < N1:
                rhs[k1 + 1] = mid_fwd(k1 + 1)
            b_s[k1] = lax.dot_general(m2[k1], rhs.pop(k1), TN, preferred_element_type=F32)

        cp_bxt.wait()
        cp_ckv0.wait()
        for w in wlist:
            for cp in wcopies(*w, 0):
                cp.wait()
        def ifft(idx):
            g, t = idx // 2, idx % 2
            xs = [(b_s[k1, 8 * g:8 * g + 8, 128 * t:128 * (t + 1)],
                   b_s[k1, 8 * g:8 * g + 8, 256 + 128 * t:256 + 128 * (t + 1)]) for k1 in range(N1)]
            xs[0] = (jnp.where(never, 0.0, xs[0][0]), xs[0][1])
            ys = _fft16(xs, +1)
            for s1 in range(N1):
                r0 = 128 * s1 + 8 * g
                y1_s[r0:r0 + 8, 128 * t:128 * (t + 1)] = ys[s1][0]
                y1_s[r0:r0 + 8, 256 + 128 * t:256 + 128 * (t + 1)] = ys[s1][1]

        dep = pltpu.bitcast(bxt[0:16, 0:128], F32)
        never = (dep - dep) < -1.0
        prep_weights(h)
        stages = [lambda: proj_q(0), lambda: proj_k(0), lambda: proj_q(1), lambda: proj_k(1)]
        for n, st in enumerate(stages):
            st()
            for idx in range(8 * n, 8 * n + 8):
                ifft(idx)
        save_first_block()
        ot7_s[...] = jnp.zeros_like(ot7_s)
        cp_g2.wait()

        def step7(c, carry):
            rows = pl.ds(pl.multiple_of(c * 512, 512), 512)
            ya = jnp.dot(y1_s[rows, :].astype(BF), g2[...], preferred_element_type=F32)
            o_s[rows, 0:DA] = ya.astype(BF)
            return carry
        lax.fori_loop(0, S // 512, step7, 0)
        cp_outa.start()

        cp_wot0.wait()
        cp_ckv1.wait()
        for w in wlist:
            for cp in wcopies(*w, 1):
                cp.start()
        cp_wot1.start()

    def at_head(hh, fn):
        def body(i, carry):
            fn()
            return carry
        lax.fori_loop(0, (h == hh).astype(jnp.int32), body, 0)

    def _stage1():
        for w in wlist:
            for cp in wcopies(*w, 1):
                cp.wait()
        cp_wot1.wait()
        cp_outa.wait()
        for w in wlist:
            for cp in wcopies(*w, 2):
                cp.start()

    def _stage2():
        for w in wlist:
            for cp in wcopies(*w, 2):
                cp.wait()

    at_head(1, _stage1)
    at_head(6, _stage2)

    ps = {0: (p0_s[0:HT, :], p0_s[HT:TQ, HT:TQ], inv0_s[0:1, :])}
    ots = {-1: ot7_s[...]}
    for t in range(NB):
        pa, pb, inv = ps.pop(t)
        nxt = (t + 2) % NB
        st = {}

        def qk_next():
            st['sa'] = qk_main(t + 1, dep if t + 1 == NB - 1 else None)

        def softmax_next():
            if t + 1 < NB:
                ps[t + 1] = softmax(t + 1, st['sa'], qk_diag(t + 1))
            else:
                save_first_block()

        def pv_diag_cur():
            st['ob'] = pv_diag(t, pb)

        def pv_cur():
            ots[t] = pv(t, pa, st['ob'], inv)

        def out_prev():
            if t == 0:
                outproj(NB - 1, ots.pop(-1), jnp.maximum(h - 1, 0))
            else:
                outproj(t - 1, ots.pop(t - 1), h, emit=(t - 1) < EMIT_BLOCKS)

        ops = {'M': qk_next, 'd': softmax_next, 'e': pv_diag_cur, 'P': pv_cur, 'O': out_prev,
               'q': lambda: proj_q(nxt), 'k': lambda: proj_k(nxt), 'V': lambda: proj_v(nxt),
               'W': lambda: proj_v(0), 'X': lambda: proj_v(1)}
        for op in STEP_ORDER[t]:
            ops[op]()
            if t + 2 == NB - 1 and op == 'k':
                dep = prep_weights(jnp.minimum(h + 1, H - 1))
    ot7_s[...] = ots.pop(NB - 1)

    @pl.when(h == H - 1)
    def _epilogue():
        outproj(NB - 1, ot7_s[...], H - 1)
        for i in range(EMIT_BLOCKS, NB):
            emit_block(i, acc_s[64:512, i * TQ:(i + 1) * TQ])
            out_copy(i).start()
        for i in range(NB):
            out_copy(i).wait()


@jax.jit
def pallas_concat_heads__spectral_gfnet__compressed_kv_cla__prompt_kernel(
    A_x, A_w_r, A_w_i, B_x, B_c_kv, B_w_q, B_w_uk, B_w_uv, B_w_o,
):
    g1, m2, g2, perm = _tables()
    axt = jnp.swapaxes(A_x, 1, 2).reshape(DA, S)
    bxt = jnp.swapaxes(B_x, 1, 2).reshape(DA, S)
    wrt = A_w_r.T
    wit = A_w_i.T
    ckv = B_c_kv.reshape(S, C)
    wq = B_w_q.reshape(DA // 2, 2, H, D)
    wuk = B_w_uk.reshape(C // 2, 2, H, D)
    wuv = B_w_uv.reshape(C // 2, 2, H, D)
    wot = jnp.swapaxes(B_w_o, 1, 2)

    any_spec = pl.BlockSpec(memory_space=pl.ANY)
    V = pltpu.VMEM
    out = pl.pallas_call(
        _kernel,
        grid=(H,),
        in_specs=[any_spec] * 13,
        out_specs=any_spec,
        out_shape=jax.ShapeDtypeStruct((S, 2 * DA), BF),
        scratch_shapes=[
            V((DA, S), BF), V((DF, S), BF), V((DF, S), BF), V((512, S), BF), V((S, C), BF),
            V((2, 2, DA // 2, 8, 128), jnp.uint32),
            V((2, 2, C // 2, 8, 128), jnp.uint32),
            V((2, 2, C // 2, 8, 128), jnp.uint32),
            V((H, DA, D), BF),
            V((2 * FP, DA), BF), V((N1, 256, 128), BF), V((512, DA), BF),
            V((128, 128), BF),
            V((2 * FP, S), F32), V((N1, 256, 256), F32), V((N1, 128, 256), F32),
            V((N1, 128, 256), F32), V((N1, 128, 512), F32), V((S, 512), F32),
            V((D, 512), BF), V((C, D), BF), V((D, C), BF),
            V((D, S), BF), V((S, D), BF), V((D, S), BF), V((512, S), F32), V((S, 2 * DA), BF),
            V((TQ, TQ), BF), V((8, TQ), F32), V((D, TQ), BF),
            pltpu.SemaphoreType.DMA((12,)),
            pltpu.SemaphoreType.DMA((3, 3, 4)),
            pltpu.SemaphoreType.DMA((8,)),
            pltpu.SemaphoreType.DMA((4,)),
        ],
        compiler_params=pltpu.CompilerParams(
            dimension_semantics=("arbitrary",),
            vmem_limit_bytes=120 * 2**20),
    )(axt, wrt, wit, bxt, ckv, wq, wuk, wuv, wot, g1, m2, g2, perm)
    return out.reshape(1, S, 2 * DA)
```
